```python
import jax
import jax.numpy as jnp

def _softmax(x, axis=-1):
    return jax.nn.softmax(x, axis=axis)

def _gelu(x):
    return jax.nn.gelu(x, approximate=True)

def _silu(x):
    return jax.nn.silu(x)

def _sigmoid(x):
    return jax.nn.sigmoid(x)

def _layernorm(x, axis=-1, eps=1e-05):
    m = jnp.mean(x, axis=axis, keepdims=True)
    v = jnp.var(x, axis=axis, keepdims=True)
    return (x - m) / jnp.sqrt(v + eps)

def _scatter_add(tgt, idx, src, axis=0):
    return tgt.at[idx].add(src)

def _segment_sum(src, seg, n):
    return jax.ops.segment_sum(src, seg, n)

class _Rng:

    def __init__(self, key):
        self._k = key

    def _next(self):
        self._k, sub = jax.random.split(self._k)
        return sub

    def normal(self, shape):
        return jax.random.normal(self._next(), shape, dtype=jnp.bfloat16)

    def randint(self, lo, hi, shape):
        return jax.random.randint(self._next(), shape, lo, hi, dtype=jnp.int32)

    def uniform(self, shape, lo=0.0, hi=1.0):
        return jax.random.uniform(self._next(), shape, jnp.bfloat16, lo, hi)

    def permutation(self, n):
        return jax.random.permutation(self._next(), n)
kernel_name = 'concat_heads__sliding_local_dilated__memory_aug_recurrent_mem_tr__prompt'

def setup_inputs():
    _rng = _Rng(jax.random.key(int.from_bytes(__import__("os").urandom(4), "little")))
    _w = lambda a: (lambda t: t.astype(jnp.bfloat16) if jnp.issubdtype(t.dtype, jnp.floating) else t)(jnp.asarray(a))

    def _A_setup():
        B, S, D = (1, 2048, 640)
        return {'x': _w((lambda *s: _rng.normal(s) * 0.05)(B, S, D)), 'wqkv': _w((lambda *s: _rng.normal(s) * 0.05)(D, 3 * D)), 'wo': _w((lambda *s: _rng.normal(s) * 0.05)(D, D))}
    _A_in = _A_setup()

    def _B_setup():
        B, S, Dm = (1, 2048, 640)
        H, Dh = (32, 192)
        M, seg = (8, 32)
        seg = min(seg, S)
        S = S // seg * seg
        return {'x': _w((lambda *s: _rng.normal(s) * 0.05)(B, S, Dm)), 'mem0': _w((lambda *s: _rng.normal(s) * 0.05)(B, M, Dm)), 'Wq': _w((lambda *s: _rng.normal(s) * 0.05)(Dm, H, Dh) * Dm ** (-0.5)), 'Wk': _w((lambda *s: _rng.normal(s) * 0.05)(Dm, H, Dh) * Dm ** (-0.5)), 'Wv': _w((lambda *s: _rng.normal(s) * 0.05)(Dm, H, Dh) * Dm ** (-0.5)), 'Wo': _w((lambda *s: _rng.normal(s) * 0.05)(H, Dh, Dm) * (H * Dh) ** (-0.5)), 'seg_len': seg}
    _B_in = _B_setup()
    return {'A_x': _A_in['x'], 'A_wqkv': _A_in['wqkv'], 'A_wo': _A_in['wo'], 'B_x': _B_in['x'], 'B_mem0': _B_in['mem0'], 'B_Wq': _B_in['Wq'], 'B_Wk': _B_in['Wk'], 'B_Wv': _B_in['Wv'], 'B_Wo': _B_in['Wo'], 'B_seg_len': _B_in['seg_len']}

def reference(A_x, A_wqkv, A_wo, B_x, B_mem0, B_Wq, B_Wk, B_Wv, B_Wo, B_seg_len):

    def _A_ref(x, wqkv, wo):
        B, S, D = x.shape
        H = 32
        Dh = D // H
        W, dil = (8, 2)
        qkv = (lambda x, *d: x.transpose(*d))((x @ wqkv).reshape(B, S, 3, H, Dh), 2, 0, 3, 1, 4)
        q, k, v = (qkv[0], qkv[1], qkv[2])
        scale = Dh ** (-0.5)
        pos = jnp.arange(S)
        off = jnp.arange(W) * dil
        idx = pos[:, None] - off[None, :]
        mask = idx >= 0
        idx_c = jnp.where(mask, idx, 0).reshape(-1)
        kg = k[:, :, idx_c, :].reshape(B, H, S, W, Dh)
        vg = v[:, :, idx_c, :].reshape(B, H, S, W, Dh)
        logits = jnp.einsum('bhsd,bhswd->bhsw', q, kg) * scale
        logits = jnp.where(mask[None, None, :, :], logits, -1000000000.0)
        attn = _softmax(logits, axis=-1)
        o = jnp.einsum('bhsw,bhswd->bhsd', attn, vg)
        return (lambda x, *d: x.transpose(*d))(o, 0, 2, 1, 3).reshape(B, S, D) @ wo

    def _B_ref(x, mem0, Wq, Wk, Wv, Wo, seg_len):
        B, S, Dm = x.shape
        H, Dh = (Wq.shape[1], Wq.shape[2])
        M = mem0.shape[1]
        scale = Dh ** (-0.5)
        n_seg = S // seg_len
        L = M + seg_len
        idx = jnp.arange(L)
        mask = (idx[:, None] < M) | (idx[:, None] >= idx[None, :])
        mem = mem0
        outs = []
        for s in range(n_seg):
            xs = x[:, s * seg_len:(s + 1) * seg_len, :].copy()
            h = jnp.concatenate([mem, xs], axis=1)
            q = jnp.einsum('btd,dhe->bhte', h, Wq)
            k = jnp.einsum('btd,dhe->bhte', h, Wk)
            v = jnp.einsum('btd,dhe->bhte', h, Wv)
            scores = jnp.einsum('bhqe,bhke->bhqk', q, k) * scale
            scores = jnp.where(mask[None, None], scores, -1000000000.0)
            p = _softmax(scores, axis=-1)
            o = jnp.einsum('bhqk,bhke->bhqe', p, v)
            o = jnp.einsum('bhte,hed->btd', o, Wo)
            mem = o[:, :M, :].copy()
            outs.append(o[:, M:, :])
        return jnp.concatenate(outs, axis=1)
    a = _A_ref(A_x, A_wqkv, A_wo)
    b = _B_ref(B_x, B_mem0, B_Wq, B_Wk, B_Wv, B_Wo, B_seg_len)
    return jnp.concatenate([a, b], axis=-1)
```

```python
import functools

import jax
import jax.numpy as jnp
from jax import lax
import jax.experimental.pallas as pl
import jax.experimental.pallas.tpu as pltpu

f32, bf16, u32 = jnp.float32, jnp.bfloat16, jnp.uint32

S, D = 2048, 640
NT = D // 128
HA, DH, WIN, DIL = 32, 20, 8, 2
PAD = 16
RB = 128
NB = S // RB
HB, E, MEM, SEG = 32, 192, 8, 32
NP = HB // 2
PW = 2 * E
L = MEM + SEG
NG = S // (4 * SEG)
NPRE = 4
NSLOT = NPRE + 1
NWO = 12
WOC = HB * E // NWO
NEG = -1000000000.0


def _dot(a, b):
    return jnp.dot(a, b, preferred_element_type=f32)


def _dot_nt(a, b):
    return lax.dot_general(a, b, (((1,), (1,)), ((), ())), preferred_element_type=f32)


def _kernel(xa_h, wqkv_h, woa_h, xb_h, mem0_h, wq_h, wk_h, wv_h, wob_h, out_h,
            xa_s, wqkv_s, woa_s, xb_s, wst_s, wost_s,
            t1_s, wpt_s, wop_s, qa_s, ka_s, va_s, oa_s, outa_s,
            w_s, wo_s, mem_s, dq_s, do_s, outb_s,
            sem_a, sem_l, sem_b, sem_wo, sem_out):
    w_h = (wq_h, wk_h, wv_h)

    def cp_xa(blk, nblk, sem):
        rows = pl.ds(blk * RB, nblk * RB)
        return pltpu.make_async_copy(xa_h.at[rows], xa_s.at[rows], sem)

    def cp_w(i, j, sem):
        rows = pl.ds(j * PW, PW)
        return pltpu.make_async_copy(w_h[i].at[rows], wst_s.at[i, rows], sem)

    def cp_loop(k):
        sem = sem_l.at[k]
        return [cp_xa(4 + 2 * k, 2, sem)] + [cp_w(i, 2 * k + dj, sem) for dj in range(2) for i in range(3)]

    def cp_wo(c):
        rows = pl.ds(c * WOC, WOC)
        return pltpu.make_async_copy(wob_h.at[rows], wost_s.at[rows], sem_wo.at[c])

    def cp_outb(g):
        rows = pl.ds(g * 4 * SEG, 4 * SEG)
        return pltpu.make_async_copy(outb_s.at[rows], out_h.at[rows, pl.ds(D, D)], sem_out.at[g])

    cp_x01 = cp_xa(0, 2, sem_a.at[0])
    cp_wqkv = [pltpu.make_async_copy(wqkv_h.at[:, pl.ds(i * D, D)], wqkv_s.at[:, pl.ds(i * D, D)], sem_a.at[1 + i])
               for i in range(3)]
    cp_woa = pltpu.make_async_copy(woa_h, woa_s, sem_a.at[4])
    cp_x23 = cp_xa(2, 2, sem_a.at[5])
    cp_xb = pltpu.make_async_copy(xb_h, xb_s, sem_b.at[0])
    cp_mem = pltpu.make_async_copy(mem0_h, mem_s, sem_b.at[1])
    cp_wlast = {j: [cp_w(i, j, sem_b.at[2 + j - 12]) for i in range(3)] for j in range(12, NP)}
    cp_outa = pltpu.make_async_copy(outa_s, out_h.at[:, pl.ds(0, D)], sem_out.at[NG])

    NLOOP = (NB - 4) // 2
    for c in [cp_x01] + cp_wqkv + [cp_woa, cp_x23]:
        c.start()
    for k in range(NLOOP):
        for c in cp_loop(k):
            c.start()
    cp_xb.start()
    cp_mem.start()
    for j in range(12, NP):
        for c in cp_wlast[j]:
            c.start()
    for c in range(NWO):
        cp_wo(c).start()

    lo16, hi16 = jnp.uint32(0xFFFF), jnp.uint32(0xFFFF0000)

    def permute_rows(base, dst_ref):
        for dp in range(DH // 2):
            for hb in range(2):
                for c in range(NT):
                    a = t1_s[c, pl.ds(base + hb * 160 + dp, 8, stride=DH), :]
                    b = t1_s[c, pl.ds(base + hb * 160 + DH // 2 + dp, 8, stride=DH), :]
                    r = (base if dst_ref is wpt_s else 0) + 2 * dp * 16 + hb * 8
                    dst_ref[r:r + 8, c * 128:(c + 1) * 128] = (a & lo16) | (b << 16)
                    dst_ref[r + 16:r + 24, c * 128:(c + 1) * 128] = (a >> 16) | (b & hi16)

    def to_t1(val_u32, base):
        for c in range(NT):
            t1_s[c, base:base + D // 2, :] = val_u32[:, c * 128:(c + 1) * 128]

    scale_a = DH ** (-0.5)

    def store_part(i, y, p):
        for c in range(NT):
            yc = y[:, c * 128:(c + 1) * 128]
            if i == 0:
                qa_s[p, c] = yc * scale_a
            else:
                ref = ka_s if i == 1 else va_s
                ref[p, c, PAD:, :] = yc
                ref[1 - p, c, 0:PAD, :] = yc[RB - PAD:]

    def wpt_part(i):
        return pltpu.bitcast(wpt_s[i * (D // 2):(i + 1) * (D // 2), :], bf16)

    def qkv(b, p):
        x = xa_s[pl.ds(pl.multiple_of(b * RB, RB), RB), :]
        for i in range(3):
            store_part(i, _dot_nt(x, wpt_part(i)), p)

    def attn(p, first=False):
        rows = lax.broadcasted_iota(jnp.int32, (8, 128), 0)
        for gi in range(RB // 8):
            r0 = gi * 8
            q = [qa_s[p, c, r0:r0 + 8, :] for c in range(NT)]
            lg = []
            for w in range(WIN):
                o = r0 + PAD - DIL * w
                t = q[0] * ka_s[p, 0, o:o + 8, :]
                for c in range(1, NT):
                    t = t + q[c] * ka_s[p, c, o:o + 8, :]
                t = t + pltpu.roll(t, 64, 1)
                t = t + pltpu.roll(t, 32, 1)
                if first and r0 < DIL * w:
                    t = jnp.where(rows + r0 >= DIL * w, t, NEG)
                lg.append(t)
            m = functools.reduce(jnp.maximum, lg)
            e = [jnp.exp(t - m) for t in lg]
            rinv = 1.0 / functools.reduce(lambda a, b: a + b, e)
            for c in range(NT):
                a = None
                for w in range(WIN):
                    o = r0 + PAD - DIL * w
                    u = e[w] * va_s[p, c, o:o + 8, :]
                    a = u if a is None else a + u
                oa_s[p, r0:r0 + 8, c * 128:(c + 1) * 128] = a * rinv

    def proj(b, p):
        y = _dot(oa_s[p].astype(bf16), pltpu.bitcast(wop_s[...], bf16))
        outa_s[pl.ds(pl.multiple_of(b * RB, RB), RB), :] = y.astype(bf16)

    def transpose_pair(j):
        r0 = j * PW if isinstance(j, int) else pl.multiple_of(j * PW, PW)
        for i in range(3):
            w_s[j, :, i * PW:(i + 1) * PW] = pltpu.bitcast(wst_s[i, pl.ds(r0, PW), :].T, u32)

    zpad = jnp.zeros((NT, PAD, 128), f32)
    ka_s[0, :, 0:PAD, :] = zpad
    va_s[0, :, 0:PAD, :] = zpad
    do_s[...] = jnp.zeros(do_s.shape, f32)
    cp_x01.wait()
    for i in range(3):
        cp_wqkv[i].wait()
        to_t1(pltpu.bitcast(wqkv_s[:, i * D:(i + 1) * D].T, u32), i * (D // 2))
        permute_rows(i * (D // 2), wpt_s)
        y = _dot_nt(xa_s[0:2 * RB, :], wpt_part(i))
        for c in range(NT):
            yc = y[:, c * 128:(c + 1) * 128]
            if i == 0:
                qa_s[0, c] = yc[:RB] * scale_a
                qa_s[1, c] = yc[RB:] * scale_a
            else:
                ref = ka_s if i == 1 else va_s
                ref[0, c, PAD:, :] = yc[:RB]
                ref[1, c] = yc[RB - PAD:]
    cp_woa.wait()
    cp_x23.wait()
    to_t1(pltpu.bitcast(woa_s[...], u32), 3 * (D // 2))
    permute_rows(3 * (D // 2), wop_s)
    attn(0, first=True)
    for ref in (ka_s, va_s):
        ref[0, :, 0:PAD, :] = ref[1, :, RB:RB + PAD, :]
    proj(0, 0); attn(1); qkv(2, 0)
    proj(1, 1); attn(0); qkv(3, 1)

    def a_body(k, carry):
        for c in cp_loop(k):
            c.wait()
        t = 4 + 2 * k
        proj(t - 2, 0); attn(1); qkv(t, 0); transpose_pair(2 * k)
        proj(t - 1, 1); attn(0); qkv(t + 1, 1); transpose_pair(2 * k + 1)
        return carry

    lax.fori_loop(0, NLOOP, a_body, 0)

    def wpair(j):
        return pltpu.bitcast(w_s[j], bf16)

    def deferred_rows(g, n):
        return jnp.concatenate(
            [xb_s[pl.ds(pl.multiple_of((4 * g + i) * SEG, SEG), 8), :] for i in range(4 * n)], axis=0)

    def pre_f(j):
        y = _dot(deferred_rows(0, NPRE), wpair(j))
        for g in range(NPRE):
            dq_s[g, j] = y[g * 32:(g + 1) * 32]

    def wo_convert(c):
        r0 = pl.multiple_of(c * WOC, WOC)
        wo_s[pl.ds(pl.multiple_of(c * (WOC // 2), WOC // 2), WOC // 2), :] = pltpu.bitcast(wost_s[pl.ds(r0, WOC), :], u32)

    cp_xb.wait()
    cp_mem.wait()
    proj(NB - 2, 0); attn(1); pre_f(0); pre_f(1)
    proj(NB - 1, 1); pre_f(2); pre_f(3)
    cp_outa.start()
    for j in range(12, NP):
        for c in cp_wlast[j]:
            c.wait()
        pre_f(j - 8); transpose_pair(j)

    def p_body(c, carry):
        cp_wo(c).wait()
        pre_f(8 + c); wo_convert(c)
        return carry

    lax.fori_loop(0, NP - 8, p_body, 0)
    for c in range(NP - 8, NWO):
        cp_wo(c).wait()
        wo_convert(c)

    scale_b = E ** (-0.5)
    ri = lax.broadcasted_iota(jnp.int32, (L, 2 * L), 0)
    ci = lax.broadcasted_iota(jnp.int32, (L, 2 * L), 1)
    is_even = ci < L
    cj = jnp.where(is_even, ci, ci - L)
    pos = lambda r: jnp.where(r < MEM, r, jnp.where(r < 32, r + 8, r - 24))
    mask = (ri < MEM) | (pos(ri) >= pos(cj))
    ev384 = lax.broadcasted_iota(jnp.int32, (L, PW), 1) < E

    def wo_rows(j):
        r0 = j * E if isinstance(j, int) else pl.multiple_of(j * E, 8)
        return pltpu.bitcast(wo_s[pl.ds(r0, E), :], bf16)

    def group(g, with_f):
        slot = lax.rem(g, NSLOT)
        fslot = lax.rem(g + NPRE, NSLOT)
        par = lax.rem(g, 2)
        fl = deferred_rows(g + NPRE, 1) if with_f else None
        gacc = [None]

        def step(i):
            r0 = pl.multiple_of((g * 4 + i) * SEG, SEG)
            h = jnp.concatenate([mem_s[...], xb_s[pl.ds(r0 + 8, 24), :]], axis=0)
            qk, vm, pp, oo, acc = {}, {}, {}, {}, [None]

            def P(j):
                y = _dot(h, wpair(j))
                y = jnp.concatenate([y, dq_s[slot, j, i * 8:(i + 1) * 8, :]], axis=0)
                k, v = y[:, PW:2 * PW], y[:, 2 * PW:]
                blk = lambda a: jnp.concatenate(
                    [jnp.where(ev384, a, 0.0), jnp.where(ev384, 0.0, a)], axis=0).astype(bf16)
                qk[j] = (y[:, :PW].astype(bf16), blk(k))
                vm[j] = blk(v)

            def Sx(j):
                q, km = qk.pop(j)
                sc = jnp.where(mask, _dot_nt(q, km) * scale_b, NEG)
                m_e = jnp.max(jnp.where(is_even, sc, -jnp.inf), axis=1, keepdims=True)
                m_o = jnp.max(jnp.where(is_even, -jnp.inf, sc), axis=1, keepdims=True)
                e = jnp.exp(sc - jnp.where(is_even, m_e, m_o))
                l_e = jnp.sum(jnp.where(is_even, e, 0.0), axis=1, keepdims=True)
                l_o = jnp.sum(jnp.where(is_even, 0.0, e), axis=1, keepdims=True)
                pp[j] = (e * jnp.where(is_even, 1.0 / l_e, 1.0 / l_o)).astype(bf16)

            def V(j):
                o = _dot(pp.pop(j), vm.pop(j))
                do_s[par, i * 8:(i + 1) * 8, j * PW:(j + 1) * PW] = o[32:]
                oo[j] = o[:32].astype(bf16)

            def O(j):
                r = _dot(oo.pop(j), wo_rows(j))
                acc[0] = r if acc[0] is None else acc[0] + r

            def F(j):
                dq_s[fslot, j] = _dot(fl, wpair(j))

            def G(j):
                r = _dot(do_s[1 - par, :, j * PW:(j + 1) * PW].astype(bf16), wo_rows(j))
                gacc[0] = r if gacc[0] is None else gacc[0] + r

            fills = [functools.partial(F, i * 4 + t) for t in range(4)] if with_f else []
            fills += [functools.partial(G, i * 4 + t) for t in range(4)]
            d1, d2, d3 = 1, 2, 1
            for t in range(NP + d1 + d2 + d3):
                if t < NP:
                    P(t)
                elif fills:
                    fills.pop(0)()
                if 0 <= t - d1 < NP:
                    Sx(t - d1)
                if 0 <= t - d1 - d2 < NP:
                    V(t - d1 - d2)
                if 0 <= t - d1 - d2 - d3 < NP:
                    O(t - d1 - d2 - d3)
            for fn in fills:
                fn()
            out = acc[0].astype(bf16)
            mem_s[...] = out[:MEM]
            outb_s[pl.ds(r0 + 8, 24), :] = out[MEM:]

        for i in range(4):
            step(i)
        write_deferred(jnp.maximum(g - 1, 0), gacc[0])

        @pl.when(g > 0)
        def _():
            cp_outb(g - 1).start()

    def write_deferred(g, val):
        r = val.astype(bf16)
        for i in range(4):
            outb_s[pl.ds(pl.multiple_of((g * 4 + i) * SEG, SEG), 8), :] = r[i * 8:(i + 1) * 8]

    def g_with_f(g, carry):
        group(g, True)
        return carry

    def g_no_f(g, carry):
        group(g, False)
        return carry

    lax.fori_loop(0, NG - NPRE, g_with_f, 0)
    lax.fori_loop(NG - NPRE, NG, g_no_f, 0)

    gl = NG - 1
    write_deferred(gl, _dot(do_s[gl % 2].astype(bf16), pltpu.bitcast(wo_s[...], bf16)))
    cp_outb(gl).start()
    cp_outa.wait()
    for g in range(NG):
        cp_outb(g).wait()


@functools.partial(jax.jit, static_argnames=("B_seg_len",))
def pallas_concat_heads__sliding_local_dilated__memory_aug_recurrent_mem_tr__prompt_kernel(
    A_x, A_wqkv, A_wo, B_x, B_mem0, B_Wq, B_Wk, B_Wv, B_Wo, B_seg_len,
):
    assert int(B_seg_len) == SEG
    assert A_x.shape == (1, S, D) and B_x.shape == (1, S, D) and B_mem0.shape == (1, MEM, D)
    assert B_Wq.shape == (D, HB, E) and B_Wo.shape == (HB, E, D)
    wt = lambda w: w.transpose(1, 2, 0).reshape(HB * E, D)
    V = pltpu.VMEM
    scratch = [
        V((S, D), bf16), V((D, 3 * D), bf16), V((D, D), bf16), V((S, D), bf16),
        V((3, HB * E, D), bf16), V((HB * E, D), bf16),
        V((NT, 4 * (D // 2), 128), u32), V((3 * D // 2, D), u32), V((D // 2, D), u32),
        V((2, NT, RB, 128), f32), V((2, NT, PAD + RB, 128), f32), V((2, NT, PAD + RB, 128), f32),
        V((2, RB, D), f32), V((S, D), bf16),
        V((NP, D // 2, 3 * PW), u32), V((HB * E // 2, D), u32), V((MEM, D), bf16),
        V((NSLOT, NP, 32, 3 * PW), f32), V((2, 32, HB * E), f32), V((S, D), bf16),
        pltpu.SemaphoreType.DMA((6,)), pltpu.SemaphoreType.DMA(((NB - 4) // 2,)),
        pltpu.SemaphoreType.DMA((6,)), pltpu.SemaphoreType.DMA((NWO,)), pltpu.SemaphoreType.DMA((NG + 1,)),
    ]
    out = pl.pallas_call(
        _kernel,
        out_shape=jax.ShapeDtypeStruct((S, 2 * D), bf16),
        in_specs=[pl.BlockSpec(memory_space=pl.ANY)] * 9,
        out_specs=pl.BlockSpec(memory_space=pl.ANY),
        scratch_shapes=scratch,
        compiler_params=pltpu.CompilerParams(vmem_limit_bytes=120 * 1024 * 1024),
    )(A_x.reshape(S, D), A_wqkv, A_wo, B_x.reshape(S, D), B_mem0.reshape(MEM, D),
      wt(B_Wq), wt(B_Wk), wt(B_Wv), B_Wo.reshape(HB * E, D))
    return out.reshape(1, S, 2 * D)
```

```python
import functools
CFG = lambda k, d: d

import jax
import jax.numpy as jnp
from jax import lax
import jax.experimental.pallas as pl
import jax.experimental.pallas.tpu as pltpu

f32, bf16, u32 = jnp.float32, jnp.bfloat16, jnp.uint32

S, D = 2048, 640
NT = D // 128
HA, DH, WIN, DIL = 32, 20, 8, 2
PAD = 16
RB = 128
NB = S // RB
ORD = CFG('ORD', 1)
GR = CFG('GR', 8)
HB, E, MEM, SEG = 32, 192, 8, 32
NP = HB // 2
PW = 2 * E
L = MEM + SEG
NG = S // (4 * SEG)
NPRE = 4
NSLOT = NPRE + 1
NWO = 4
WOC = HB * E // NWO
NEG = -1000000000.0


def _dot(a, b):
    return jnp.dot(a, b, preferred_element_type=f32)


def _dot_nt(a, b):
    return lax.dot_general(a, b, (((1,), (1,)), ((), ())), preferred_element_type=f32)


def _kernel(xa_h, wqkv_h, woa_h, xb_h, mem0_h, wq_h, wk_h, wv_h, wob_h, out_h,
            xa_s, wqkv_s, woa_s, xb_s, wst_s, wost_s,
            t1_s, wpt_s, wop_s, qa_s, ka_s, va_s, oa_s, outa_s,
            w_s, wo_s, mem_s, dq_s, do_s, gacc_s, outb_s, pl_s,
            sem_a, sem_l, sem_b, sem_wo, sem_out):
    w_h = (wq_h, wk_h, wv_h)

    def cp_xa(blk, nblk, sem):
        rows = pl.ds(blk * RB, nblk * RB)
        return pltpu.make_async_copy(xa_h.at[rows], xa_s.at[rows], sem)

    def cp_w(i, j, sem):
        rows = pl.ds(j * PW, PW)
        return pltpu.make_async_copy(w_h[i].at[rows], wst_s.at[i, rows], sem)

    def cp_loop(k):
        sem = sem_l.at[k]
        return [cp_xa(4 + 2 * k, 2, sem)] + [cp_w(i, 2 * k + dj, sem) for dj in range(2) for i in range(3)]

    cp_wo = [pltpu.make_async_copy(wob_h.at[pl.ds(c * WOC, WOC)], wost_s.at[pl.ds(c * WOC, WOC)], sem_wo.at[0])
             for c in range(NWO)]

    def cp_outb(g):
        rows = pl.ds(g * 4 * SEG, 4 * SEG)
        return pltpu.make_async_copy(outb_s.at[rows], out_h.at[rows, pl.ds(D, D)], sem_out.at[g])

    cp_x01 = cp_xa(0, 2, sem_a.at[0])
    cp_wqkv = [pltpu.make_async_copy(wqkv_h.at[:, pl.ds(i * D, D)], wqkv_s.at[:, pl.ds(i * D, D)], sem_a.at[1 + i])
               for i in range(3)]
    cp_woa = pltpu.make_async_copy(woa_h, woa_s, sem_a.at[4])
    cp_x23 = cp_xa(2, 2, sem_a.at[5])
    cp_xb = [pltpu.make_async_copy(xb_h.at[pl.ds(r, n)], xb_s.at[pl.ds(r, n)], sem_b.at[0])
             for r, n in ((0, 256), (256, 384))]
    cp_xb2 = [pltpu.make_async_copy(xb_h.at[pl.ds(r, n)], xb_s.at[pl.ds(r, n)], sem_b.at[6])
              for r, n in ((640, 384), (1024, 384), (1408, 384), (1792, 256))]
    cp_mem = pltpu.make_async_copy(mem0_h, mem_s, sem_b.at[1])
    cp_wlast = {j: [cp_w(i, j, sem_b.at[2 + j - 12]) for i in range(3)] for j in range(12, NP)}
    cp_outa = pltpu.make_async_copy(outa_s, out_h.at[:, pl.ds(0, D)], sem_out.at[NG])

    NLOOP = (NB - 4) // 2
    def start_in_order(items):
        def body(i, carry):
            for k, cps in enumerate(items):
                @pl.when(i == k)
                def _(cps=cps):
                    for c in cps:
                        c.start()
            return carry
        lax.fori_loop(0, len(items), body, 0)

    def start_loop(n, fn):
        def body(i, carry):
            for c in fn(i):
                c.start()
            return carry
        lax.fori_loop(0, n, body, 0)

    start_in_order([[cp_wqkv[0]], [cp_x01], [cp_x23], [cp_wqkv[1]], [cp_wqkv[2]], [cp_woa]])
    start_loop(NLOOP, cp_loop)
    for c in cp_xb + [cp_mem]:
        c.start()
    start_loop(NP - 12, lambda j: [cp_w(i, 12 + j, sem_b.at[2 + j]) for i in range(3)])

    lo16, hi16 = jnp.uint32(0xFFFF), jnp.uint32(0xFFFF0000)

    def permute_rows(base, dst_ref):
        for dp in range(DH // 2):
            for hb in range(2):
                for c in range(NT):
                    a = t1_s[c, pl.ds(base + hb * 160 + dp, 8, stride=DH), :]
                    b = t1_s[c, pl.ds(base + hb * 160 + DH // 2 + dp, 8, stride=DH), :]
                    r = (base if dst_ref is wpt_s else 0) + 2 * dp * 16 + hb * 8
                    dst_ref[r:r + 8, c * 128:(c + 1) * 128] = (a & lo16) | (b << 16)
                    dst_ref[r + 16:r + 24, c * 128:(c + 1) * 128] = (a >> 16) | (b & hi16)

    def to_t1(val_u32, base):
        for c in range(NT):
            t1_s[c, base:base + D // 2, :] = val_u32[:, c * 128:(c + 1) * 128]

    scale_a = DH ** (-0.5)

    def store_part(i, y, p):
        for c in range(NT):
            yc = y[:, c * 128:(c + 1) * 128]
            if i == 0:
                qa_s[p, c] = yc * scale_a
            else:
                ref = ka_s if i == 1 else va_s
                ref[p, c, PAD:, :] = yc
                if not ORD:
                    ref[1 - p, c, 0:PAD, :] = yc[RB - PAD:]

    def wpt_part(i):
        return pltpu.bitcast(wpt_s[i * (D // 2):(i + 1) * (D // 2), :], bf16)

    MS = CFG('MS', 128)
    def qkv(b, p):
        for m0 in range(0, RB, MS):
            x = xa_s[pl.ds(pl.multiple_of(b * RB + m0, MS), MS), :]
            for i in range(3):
                y = _dot_nt(x, wpt_part(i))
                for c in range(NT):
                    yc = y[:, c * 128:(c + 1) * 128]
                    if i == 0:
                        qa_s[p, c, m0:m0 + MS, :] = yc * scale_a
                    else:
                        (ka_s if i == 1 else va_s)[p, c, PAD + m0:PAD + m0 + MS, :] = yc

    def attn(p, first=False, hooks=()):
        hooks = list(hooks)
        ngr = RB // GR
        every = ngr // len(hooks) if hooks else 0
        rows = lax.broadcasted_iota(jnp.int32, (GR, 128), 0)
        def stage1(gi):
            r0 = gi * GR
            q = [qa_s[p, c, r0:r0 + GR, :] for c in range(NT)]
            lg = []
            for w in range(WIN):
                o = r0 + PAD - DIL * w
                t = q[0] * ka_s[p, 0, o:o + GR, :]
                for c in range(1, NT):
                    t = t + q[c] * ka_s[p, c, o:o + GR, :]
                lg.append(t)
            return [t + pltpu.roll(t, 64, 1) for t in lg]
        SWP = CFG('SWP', 0)
        nxt = stage1(0) if SWP else None
        for gi in range(ngr):
            r0 = gi * GR
            if SWP:
                lg = nxt
                if gi + 1 < ngr:
                    nxt = stage1(gi + 1)
            else:
                lg = stage1(gi)
            lg = [t + pltpu.roll(t, 32, 1) for t in lg]
            if first:
                lg = [jnp.where(rows + r0 >= DIL * w, t, NEG) if r0 < DIL * w else t for w, t in enumerate(lg)]
            m = functools.reduce(jnp.maximum, lg)
            e = [jnp.exp(t - m) for t in lg]
            rinv = 1.0 / functools.reduce(lambda a, b: a + b, e)
            for c in range(NT):
                a = None
                for w in range(WIN):
                    o = r0 + PAD - DIL * w
                    u = e[w] * va_s[p, c, o:o + GR, :]
                    a = u if a is None else a + u
                oa_s[p, r0:r0 + GR, c * 128:(c + 1) * 128] = a * rinv
            if hooks and (gi + 1) % every == 0:
                hooks.pop(0)()
        for hk in hooks:
            hk()

    def proj(b, p):
        MP = CFG('MP', 128)
        for m0 in range(0, RB, MP):
            y = _dot(oa_s[p, m0:m0 + MP, :].astype(bf16), pltpu.bitcast(wop_s[...], bf16))
            outa_s[pl.ds(pl.multiple_of(b * RB + m0, MP), MP), :] = y.astype(bf16)

    def halo(p):
        for ref in (ka_s, va_s):
            ref[1 - p, :, 0:PAD, :] = ref[p, :, RB:RB + PAD, :]

    def qkv_piece(b, p, i, c0, nc):
        x = xa_s[pl.ds(pl.multiple_of(b * RB, RB), RB), :]
        r0 = i * (D // 2) + c0 * 64
        y = _dot_nt(x, pltpu.bitcast(wpt_s[r0:r0 + nc * 64, :], bf16))
        for cc in range(nc):
            c = c0 + cc
            yc = y[:, cc * 128:(cc + 1) * 128]
            if i == 0:
                qa_s[p, c] = yc * scale_a
            else:
                (ka_s if i == 1 else va_s)[p, c, PAD:, :] = yc

    def proj_piece(b, p, c0, nc):
        y = _dot(oa_s[p].astype(bf16), pltpu.bitcast(wop_s[:, c0 * 128:(c0 + nc) * 128], bf16))
        outa_s[pl.ds(pl.multiple_of(b * RB, RB), RB), c0 * 128:(c0 + nc) * 128] = y.astype(bf16)

    def tick(t, p, hooks=()):
        if ORD >= 4:
            mx = [functools.partial(proj_piece, t - 2, p, c, 1) for c in range(NT)]
            mx += [functools.partial(qkv_piece, t, p, i, c, 1) for i in range(3) for c in range(NT)]
            hooks = list(hooks)
            ngr = RB // GR
            lead = 20 - ngr if ORD == 4 else 2
            for fn in mx[:lead]:
                fn()
            rest = mx[lead:]
            hk = []
            for gi in range(ngr):
                fns = [rest.pop(0)] if rest else []
                if ORD == 5 and gi % 8 == 7 and rest: fns.append(rest.pop(0))
                if hooks and gi % (ngr // 4) == (ngr // 4) - 1:
                    fns.append(hooks.pop(0))
                hk.append(lambda fns=fns: [f() for f in fns])
            attn(1 - p, hooks=hk)
            for fn in rest + hooks: fn()
            halo(p)
            return
        if ORD == 0:
            proj(t - 2, p); attn(1 - p, hooks=hooks); qkv(t, p)
        elif ORD == 1:
            proj(t - 2, p); qkv(t, p); attn(1 - p, hooks=hooks); halo(p)
        elif ORD == 2:
            qkv(t, p); proj(t - 2, p); attn(1 - p, hooks=hooks); halo(p)
        elif ORD == 3:
            qkv(t, p); attn(1 - p, hooks=hooks); proj(t - 2, p); halo(p)

    def transpose_part(j, i):
        r0 = j * PW if isinstance(j, int) else pl.multiple_of(j * PW, PW)
        w_s[j, :, i * PW:(i + 1) * PW] = pltpu.bitcast(wst_s[i, pl.ds(r0, PW), :].T, u32)

    def transposes(j):
        return [functools.partial(transpose_part, j, i) for i in range(3)]

    zpad = jnp.zeros((NT, PAD, 128), f32)
    ka_s[2, :, 0:PAD, :] = zpad
    va_s[2, :, 0:PAD, :] = zpad
    gacc_s[...] = jnp.zeros(gacc_s.shape, f32)
    def prep_part(i):
        to_t1(pltpu.bitcast(wqkv_s[:, i * D:(i + 1) * D].T, u32), i * (D // 2))
        permute_rows(i * (D // 2), wpt_s)

    SETS = (2, 3, 0, 1)

    def first_block(i, b):
        y = _dot_nt(xa_s[b * RB:(b + 1) * RB, :], wpt_part(i))
        p = SETS[b]
        for c in range(NT):
            yc = y[:, c * 128:(c + 1) * 128]
            if i == 0:
                qa_s[p, c] = yc * scale_a
            else:
                ref = ka_s if i == 1 else va_s
                ref[p, c, PAD:, :] = yc
                if b < 3:
                    ref[SETS[b + 1], c, 0:PAD, :] = yc[RB - PAD:]

    with jax.named_scope("s_w0"):
        cp_wqkv[0].wait()
    with jax.named_scope("s_a0"):
        prep_part(0)
        cp_x01.wait()
        first_block(0, 0); first_block(0, 1)
    with jax.named_scope("s_w1"):
        cp_x23.wait()
        cp_wqkv[1].wait()
    with jax.named_scope("s_a1"):
        first_block(0, 2); first_block(0, 3); prep_part(1)
    with jax.named_scope("s_w2"):
        cp_wqkv[2].wait()
    with jax.named_scope("s_a2"):
        first_block(1, 0); first_block(1, 1); prep_part(2)
        first_block(2, 0); first_block(2, 1)
    with jax.named_scope("s_w3"):
        cp_woa.wait()
    with jax.named_scope("s_a3"):
        for c in cp_wo:
            c.start()
        first_block(1, 2); first_block(2, 2)
        attn(SETS[0], first=True)
        to_t1(pltpu.bitcast(woa_s[...], u32), 3 * (D // 2))
        permute_rows(3 * (D // 2), wop_s)
        first_block(1, 3); first_block(2, 3)
        attn(SETS[1])
        proj(0, SETS[0])
        attn(SETS[2])
        proj(1, SETS[1])
        halo(1)

    def a_body(k, carry):
      with jax.named_scope("s_abody"):
        for c in cp_loop(k):
            c.wait()
        t = 4 + 2 * k
        tick(t, 0, transposes(2 * k)); tick(t + 1, 1, transposes(2 * k + 1))
      return carry

    lax.fori_loop(0, NLOOP, a_body, 0)

    def wpair(j):
        return pltpu.bitcast(w_s[j], bf16)

    def deferred_rows(g, n):
        return jnp.concatenate(
            [xb_s[pl.ds(pl.multiple_of((4 * g + i) * SEG, SEG), 8), :] for i in range(4 * n)], axis=0)

    def pre_f(j):
        y = _dot(pltpu.bitcast(pl_s[...], bf16), wpair(j))
        for g in range(NPRE):
            dq_s[g, j] = y[g * 32:(g + 1) * 32]

    def wo_convert(c):
        wo_s[c * (WOC // 2):(c + 1) * (WOC // 2), :] = pltpu.bitcast(wost_s[c * WOC:(c + 1) * WOC, :], u32)

    def interleave(mxu, side):
        side = list(side)
        per = -(-len(side) // len(mxu))
        for fn in mxu:
            fn()
            for sf in side[:per]:
                sf()
            side = side[per:]

    PF = lambda js: [functools.partial(pre_f, j) for j in js]
    N1, N2 = CFG('N1', 4), CFG('N2', 10)
    with jax.named_scope("s_p0"):
        for c in cp_xb + [cp_mem] + cp_wlast[12] + cp_wlast[13]:
            c.wait()
        for c in cp_xb2:
            c.start()
        pl_s[...] = pltpu.bitcast(deferred_rows(0, NPRE), u32)
        proj(NB - 2, 0); pre_f(0); attn(1); pre_f(1)
        proj(NB - 1, 1)
        interleave(PF(range(2, N1)), transposes(12) + transposes(13))
    with jax.named_scope("s_p1"):
        for c in cp_wlast[14] + cp_wlast[15]:
            c.wait()
        interleave(PF(range(N1, N2)), transposes(14) + transposes(15))
        for fn in PF(range(N2, NP)):
            fn()
    with jax.named_scope("s_p2"):
        for c in cp_wo:
            c.wait()

    scale_b = E ** (-0.5)
    ri = lax.broadcasted_iota(jnp.int32, (L, 2 * L), 0)
    ci = lax.broadcasted_iota(jnp.int32, (L, 2 * L), 1)
    is_even = ci < L
    cj = jnp.where(is_even, ci, ci - L)
    pos = lambda r: jnp.where(r < MEM, r, jnp.where(r < 32, r + 8, r - 24))
    mask = (ri < MEM) | (pos(ri) >= pos(cj))
    ev384 = lax.broadcasted_iota(jnp.int32, (L, PW), 1) < E

    def wo_rows(j):
        r0 = j * E if isinstance(j, int) else pl.multiple_of(j * E, 8)
        return pltpu.bitcast(wo_s[pl.ds(r0, E), :], bf16)

    def group(g, with_f, with_g, unroll):
        slot = lax.rem(g, NSLOT)
        fslot = lax.rem(g + NPRE, NSLOT)
        par = lax.rem(g, 2)

        def step(i):
            static = isinstance(i, int)
            r0 = pl.multiple_of((g * 4 + i) * SEG, SEG)
            drow = pl.ds(i * 8 if static else pl.multiple_of(i * 8, 8), 8)
            h = jnp.concatenate([mem_s[...], xb_s[pl.ds(r0 + 8, 24), :]], axis=0)
            fl = deferred_rows(g + NPRE, 1) if with_f else None
            qk, vm, pp, oo, acc = {}, {}, {}, {}, [None]

            def P(j):
                y = _dot(h, wpair(j))
                y = jnp.concatenate([y, dq_s[slot, j, drow, :]], axis=0)
                k, v = y[:, PW:2 * PW], y[:, 2 * PW:]
                blk = lambda a: jnp.concatenate(
                    [jnp.where(ev384, a, 0.0), jnp.where(ev384, 0.0, a)], axis=0).astype(bf16)
                qk[j] = (y[:, :PW].astype(bf16), blk(k))
                vm[j] = blk(v)

            def Sx(j):
                q, km = qk.pop(j)
                sc = jnp.where(mask, _dot_nt(q, km) * scale_b, NEG)
                m_e = jnp.max(jnp.where(is_even, sc, -jnp.inf), axis=1, keepdims=True)
                m_o = jnp.max(jnp.where(is_even, -jnp.inf, sc), axis=1, keepdims=True)
                e = jnp.exp(sc - jnp.where(is_even, m_e, m_o))
                l_e = jnp.sum(jnp.where(is_even, e, 0.0), axis=1, keepdims=True)
                l_o = jnp.sum(jnp.where(is_even, 0.0, e), axis=1, keepdims=True)
                pp[j] = (e * jnp.where(is_even, 1.0 / l_e, 1.0 / l_o)).astype(bf16)

            def V(j):
                o = _dot(pp.pop(j), vm.pop(j))
                do_s[par, drow, j * PW:(j + 1) * PW] = o[32:]
                oo[j] = o[:32].astype(bf16)

            def O(j):
                if with_g:
                    wj = wo_rows(j)
                else:
                    wj = wost_s[j * PW:(j + 1) * PW, :]
                    wo_s[j * E:(j + 1) * E, :] = pltpu.bitcast(wj, u32)
                r = _dot(oo.pop(j), wj)
                acc[0] = r if acc[0] is None else acc[0] + r

            def F(j):
                dq_s[fslot, j] = _dot(fl, wpair(j))

            def G(j):
                c0 = j * PW if static else pl.multiple_of(j * PW, 128)
                gacc_s[...] += _dot(do_s[1 - par, :, pl.ds(c0, PW)].astype(bf16), wo_rows(j))

            fills = [functools.partial(F, i * 4 + t) for t in range(4)] if with_f else []
            if with_g:
                fills += [functools.partial(G, i * 4 + t) for t in range(4)]
            d1, d2, d3 = 1, 2, 1
            seq = []
            for t in range(NP + d1 + d2 + d3):
                if t < NP:
                    seq.append(("P", t))
                items = [("S", t - d1), ("V", t - d1 - d2), ("O", t - d1 - d2 - d3)]
                if CFG('VS', 0):
                    items = [items[1], items[0], items[2]]
                seq += [it for it in items if 0 <= it[1] < NP]
            place = CFG('PLF' if with_f else 'PLN', 'O11,O12,O13,O14' if with_f else 'O13,O14').split(',')
            for nm, j in seq:
                {"P": P, "S": Sx, "V": V, "O": O}[nm](j)
                while place and place[0] == f"{nm}{j}" and fills:
                    place.pop(0)
                    fills.pop(0)()
            for fn in fills:
                fn()
            out = acc[0].astype(bf16)
            mem_s[...] = out[:MEM]
            outb_s[pl.ds(r0 + 8, 24), :] = out[MEM:]

        if unroll == 4:
            for i in range(4):
                step(i)
        else:
            def inner(ii, carry):
                for u in range(unroll):
                    step(ii * unroll + u)
                return carry
            lax.fori_loop(0, 4 // unroll, inner, 0)
        if with_g:
            write_deferred(g - 1, gacc_s[...])
            gacc_s[...] = jnp.zeros(gacc_s.shape, f32)
            cp_outb(g - 1).start()

    def write_deferred(g, val):
        r = val.astype(bf16)
        for i in range(4):
            outb_s[pl.ds(pl.multiple_of((g * 4 + i) * SEG, SEG), 8), :] = r[i * 8:(i + 1) * 8]

    def g_with_f(g, carry):
        with jax.named_scope("s_gF"):
            group(g, True, True, 4)
        return carry

    def g_no_f(g, carry):
        with jax.named_scope("s_gN"):
            group(g, False, True, 2)
        return carry

    cp_outa.start()
    if CFG('SKIPB', 0):
        for c in cp_xb2:
            c.wait()
        outb_s[...] = xb_s[...]
        do_s[...] = jnp.zeros(do_s.shape, f32)
        for g in range(NG - 1):
            cp_outb(g).start()
    else:
        with jax.named_scope("s_g0"):
            group(jnp.int32(0), True, False, 1)
        for c in cp_xb2:
            c.wait()
        lax.fori_loop(1, NG - NPRE, g_with_f, 0)
        lax.fori_loop(NG - NPRE, NG, g_no_f, 0)

    gl = NG - 1
    write_deferred(gl, _dot(do_s[gl % 2].astype(bf16), pltpu.bitcast(wo_s[...], bf16)))
    cp_outb(gl).start()
    cp_outa.wait()
    for g in range(NG):
        cp_outb(g).wait()


@functools.partial(jax.jit, static_argnames=("B_seg_len",))
def pallas_concat_heads__sliding_local_dilated__memory_aug_recurrent_mem_tr__prompt_kernel(
    A_x, A_wqkv, A_wo, B_x, B_mem0, B_Wq, B_Wk, B_Wv, B_Wo, B_seg_len,
):
    assert int(B_seg_len) == SEG
    assert A_x.shape == (1, S, D) and B_x.shape == (1, S, D) and B_mem0.shape == (1, MEM, D)
    assert B_Wq.shape == (D, HB, E) and B_Wo.shape == (HB, E, D)
    wt = lambda w: w.transpose(1, 2, 0).reshape(HB * E, D)
    V = pltpu.VMEM
    scratch = [
        V((S, D), bf16), V((D, 3 * D), bf16), V((D, D), bf16), V((S, D), bf16),
        V((3, HB * E, D), bf16), V((HB * E, D), bf16),
        V((NT, 4 * (D // 2), 128), u32), V((3 * D // 2, D), u32), V((D // 2, D), u32),
        V((4, NT, RB, 128), f32), V((4, NT, PAD + RB, 128), f32), V((4, NT, PAD + RB, 128), f32),
        V((4, RB, D), f32), V((S, D), bf16),
        V((NP, D // 2, 3 * PW), u32), V((HB * E // 2, D), u32), V((MEM, D), bf16),
        V((NSLOT, NP, 32, 3 * PW), f32), V((2, 32, HB * E), f32), V((32, D), f32), V((S, D), bf16), V((NPRE * 16, D), u32),
        pltpu.SemaphoreType.DMA((6,)), pltpu.SemaphoreType.DMA(((NB - 4) // 2,)),
        pltpu.SemaphoreType.DMA((7,)), pltpu.SemaphoreType.DMA((NWO,)), pltpu.SemaphoreType.DMA((NG + 1,)),
    ]
    out = pl.pallas_call(
        _kernel,
        out_shape=jax.ShapeDtypeStruct((S, 2 * D), bf16),
        in_specs=[pl.BlockSpec(memory_space=pl.ANY)] * 9,
        out_specs=pl.BlockSpec(memory_space=pl.ANY),
        scratch_shapes=scratch,
        compiler_params=pltpu.CompilerParams(vmem_limit_bytes=120 * 1024 * 1024),
    )(A_x.reshape(S, D), A_wqkv, A_wo, B_x.reshape(S, D), B_mem0.reshape(MEM, D),
      wt(B_Wq), wt(B_Wk), wt(B_Wv), B_Wo.reshape(HB * E, D))
    return out.reshape(1, S, 2 * D)
```

```python
import functools
CFG = lambda k, d: d

import jax
import jax.numpy as jnp
from jax import lax
import jax.experimental.pallas as pl
import jax.experimental.pallas.tpu as pltpu

f32, bf16, u32 = jnp.float32, jnp.bfloat16, jnp.uint32

S, D = 2048, 640
NT = D // 128
HA, DH, WIN, DIL = 32, 20, 8, 2
PAD = 16
RB = 128
NB = S // RB
ORD = CFG('ORD', 1)
GR = CFG('GR', 8)
HB, E, MEM, SEG = 32, 192, 8, 32
NP = HB // 2
PW = 2 * E
L = MEM + SEG
NG = S // (4 * SEG)
NPRE = 4
NSLOT = NPRE + 2
NWO = 4
WOC = HB * E // NWO
NEG = -1000000000.0


def _rcp(x):
    m = CFG('RCP', 2)
    if m == 0:
        return 1.0 / x
    r = pl.reciprocal(x, approx=True)
    if m == 2:
        r = r * (2.0 - x * r)
    return r


def _dot(a, b):
    return jnp.dot(a, b, preferred_element_type=f32)


def _dot_nt(a, b):
    return lax.dot_general(a, b, (((1,), (1,)), ((), ())), preferred_element_type=f32)


def _kernel(xa_h, wqkv_h, woa_h, xb_h, mem0_h, wq_h, wk_h, wv_h, wob_h, out_h,
            xa_s, wqkv_s, woa_s, xb_s, wst_s, wost_s,
            t1_s, wpt_s, wop_s, qa_s, ka_s, va_s, oa_s, outa_s,
            w_s, wo_s, mem_s, dq_s, kvm_s, gacc_s, outb_s, pl_s, mq_s, mk_s, mv_s, mo_s, cur_s,
            sem_a, sem_l, sem_b, sem_wo, sem_out):
    w_h = (wq_h, wk_h, wv_h)

    def cp_xa(blk, nblk, sem):
        rows = pl.ds(blk * RB, nblk * RB)
        return pltpu.make_async_copy(xa_h.at[rows], xa_s.at[rows], sem)

    def cp_w(i, j, sem):
        rows = pl.ds(j * PW, PW)
        return pltpu.make_async_copy(w_h[i].at[rows], wst_s.at[i, rows], sem)

    def cp_loop(k):
        sem = sem_l.at[k]
        return [cp_xa(4 + 2 * k, 2, sem)] + [cp_w(i, 2 * k + dj, sem) for dj in range(2) for i in range(3)]

    cp_wo = [pltpu.make_async_copy(wob_h.at[pl.ds(c * WOC, WOC)], wost_s.at[pl.ds(c * WOC, WOC)], sem_wo.at[0])
             for c in range(NWO)]

    def cp_outb(g):
        rows = pl.ds(g * 4 * SEG, 4 * SEG)
        return pltpu.make_async_copy(outb_s.at[rows], out_h.at[rows, pl.ds(D, D)], sem_out.at[g])

    cp_x01 = cp_xa(0, 2, sem_a.at[0])
    cp_wqkv = [pltpu.make_async_copy(wqkv_h.at[:, pl.ds(i * D, D)], wqkv_s.at[:, pl.ds(i * D, D)], sem_a.at[1 + i])
               for i in range(3)]
    cp_woa = pltpu.make_async_copy(woa_h, woa_s, sem_a.at[4])
    cp_x23 = cp_xa(2, 2, sem_a.at[5])
    cp_xb = [pltpu.make_async_copy(xb_h.at[pl.ds(r, n)], xb_s.at[pl.ds(r, n)], sem_b.at[0])
             for r, n in ((0, 256), (256, 384))]
    cp_xb2 = [pltpu.make_async_copy(xb_h.at[pl.ds(r, n)], xb_s.at[pl.ds(r, n)], sem_b.at[6])
              for r, n in ((640, 384), (1024, 384), (1408, 384), (1792, 256))]
    cp_mem = pltpu.make_async_copy(mem0_h, mem_s, sem_b.at[1])
    cp_wlast = {j: [cp_w(i, j, sem_b.at[2 + j - 12]) for i in range(3)] for j in range(12, NP)}
    cp_outa = pltpu.make_async_copy(outa_s, out_h.at[:, pl.ds(0, D)], sem_out.at[NG])

    NLOOP = (NB - 4) // 2
    def start_in_order(items):
        def body(i, carry):
            for k, cps in enumerate(items):
                @pl.when(i == k)
                def _(cps=cps):
                    for c in cps:
                        c.start()
            return carry
        lax.fori_loop(0, len(items), body, 0)

    def start_loop(n, fn):
        def body(i, carry):
            for c in fn(i):
                c.start()
            return carry
        lax.fori_loop(0, n, body, 0)

    start_in_order([[cp_wqkv[0]], [cp_x01], [cp_x23], [cp_wqkv[1]], [cp_wqkv[2]], [cp_woa]])
    start_loop(NLOOP, cp_loop)
    for c in cp_xb + [cp_mem]:
        c.start()
    start_loop(NP - 12, lambda j: [cp_w(i, 12 + j, sem_b.at[2 + j]) for i in range(3)])

    lo16, hi16 = jnp.uint32(0xFFFF), jnp.uint32(0xFFFF0000)

    def permute_rows(base, dst_ref):
        for dp in range(DH // 2):
            for hb in range(2):
                for c in range(NT):
                    a = t1_s[c, pl.ds(base + hb * 160 + dp, 8, stride=DH), :]
                    b = t1_s[c, pl.ds(base + hb * 160 + DH // 2 + dp, 8, stride=DH), :]
                    r = (base if dst_ref is wpt_s else 0) + 2 * dp * 16 + hb * 8
                    dst_ref[r:r + 8, c * 128:(c + 1) * 128] = (a & lo16) | (b << 16)
                    dst_ref[r + 16:r + 24, c * 128:(c + 1) * 128] = (a >> 16) | (b & hi16)

    def to_t1(val_u32, base):
        for c in range(NT):
            t1_s[c, base:base + D // 2, :] = val_u32[:, c * 128:(c + 1) * 128]

    scale_a = DH ** (-0.5)

    def store_part(i, y, p):
        for c in range(NT):
            yc = y[:, c * 128:(c + 1) * 128]
            if i == 0:
                qa_s[p, c] = yc * scale_a
            else:
                ref = ka_s if i == 1 else va_s
                ref[p, c, PAD:, :] = yc
                if not ORD:
                    ref[1 - p, c, 0:PAD, :] = yc[RB - PAD:]

    def wpt_part(i):
        return pltpu.bitcast(wpt_s[i * (D // 2):(i + 1) * (D // 2), :], bf16)

    MS = CFG('MS', 128)
    def qkv(b, p):
        for m0 in range(0, RB, MS):
            x = xa_s[pl.ds(pl.multiple_of(b * RB + m0, MS), MS), :]
            for i in range(3):
                y = _dot_nt(x, wpt_part(i))
                for c in range(NT):
                    yc = y[:, c * 128:(c + 1) * 128]
                    if i == 0:
                        qa_s[p, c, m0:m0 + MS, :] = yc * scale_a
                    else:
                        (ka_s if i == 1 else va_s)[p, c, PAD + m0:PAD + m0 + MS, :] = yc

    def attn(p, first=False, hooks=()):
        hooks = list(hooks)
        ngr = RB // GR
        every = ngr // len(hooks) if hooks else 0
        rows = lax.broadcasted_iota(jnp.int32, (GR, 128), 0)
        def stage1(gi):
            r0 = gi * GR
            q = [qa_s[p, c, r0:r0 + GR, :] for c in range(NT)]
            lg = []
            for w in range(WIN):
                o = r0 + PAD - DIL * w
                t = q[0] * ka_s[p, 0, o:o + GR, :]
                for c in range(1, NT):
                    t = t + q[c] * ka_s[p, c, o:o + GR, :]
                lg.append(t)
            return [t + pltpu.roll(t, 64, 1) for t in lg]
        SWP = CFG('SWP', 0)
        nxt = stage1(0) if SWP else None
        for gi in range(ngr):
            r0 = gi * GR
            if SWP:
                lg = nxt
                if gi + 1 < ngr:
                    nxt = stage1(gi + 1)
            else:
                lg = stage1(gi)
            lg = [t + pltpu.roll(t, 32, 1) for t in lg]
            if first:
                lg = [jnp.where(rows + r0 >= DIL * w, t, NEG) if r0 < DIL * w else t for w, t in enumerate(lg)]
            m = functools.reduce(jnp.maximum, lg)
            e = [jnp.exp(t - m) for t in lg]
            rinv = 1.0 / functools.reduce(lambda a, b: a + b, e)
            for c in range(NT):
                a = None
                for w in range(WIN):
                    o = r0 + PAD - DIL * w
                    u = e[w] * va_s[p, c, o:o + GR, :]
                    a = u if a is None else a + u
                oa_s[p, r0:r0 + GR, c * 128:(c + 1) * 128] = a * rinv
            if hooks and (gi + 1) % every == 0:
                hooks.pop(0)()
        for hk in hooks:
            hk()

    def proj(b, p):
        MP = CFG('MP', 128)
        for m0 in range(0, RB, MP):
            y = _dot(oa_s[p, m0:m0 + MP, :].astype(bf16), pltpu.bitcast(wop_s[...], bf16))
            outa_s[pl.ds(pl.multiple_of(b * RB + m0, MP), MP), :] = y.astype(bf16)

    def halo(p):
        for ref in (ka_s, va_s):
            ref[1 - p, :, 0:PAD, :] = ref[p, :, RB:RB + PAD, :]

    def qkv_piece(b, p, i, c0, nc):
        x = xa_s[pl.ds(pl.multiple_of(b * RB, RB), RB), :]
        r0 = i * (D // 2) + c0 * 64
        y = _dot_nt(x, pltpu.bitcast(wpt_s[r0:r0 + nc * 64, :], bf16))
        for cc in range(nc):
            c = c0 + cc
            yc = y[:, cc * 128:(cc + 1) * 128]
            if i == 0:
                qa_s[p, c] = yc * scale_a
            else:
                (ka_s if i == 1 else va_s)[p, c, PAD:, :] = yc

    def proj_piece(b, p, c0, nc):
        y = _dot(oa_s[p].astype(bf16), pltpu.bitcast(wop_s[:, c0 * 128:(c0 + nc) * 128], bf16))
        outa_s[pl.ds(pl.multiple_of(b * RB, RB), RB), c0 * 128:(c0 + nc) * 128] = y.astype(bf16)

    def tick(t, p, hooks=()):
        if ORD >= 4:
            mx = [functools.partial(proj_piece, t - 2, p, c, 1) for c in range(NT)]
            mx += [functools.partial(qkv_piece, t, p, i, c, 1) for i in range(3) for c in range(NT)]
            hooks = list(hooks)
            ngr = RB // GR
            lead = 20 - ngr if ORD == 4 else 2
            for fn in mx[:lead]:
                fn()
            rest = mx[lead:]
            hk = []
            for gi in range(ngr):
                fns = [rest.pop(0)] if rest else []
                if ORD == 5 and gi % 8 == 7 and rest: fns.append(rest.pop(0))
                if hooks and gi % (ngr // 4) == (ngr // 4) - 1:
                    fns.append(hooks.pop(0))
                hk.append(lambda fns=fns: [f() for f in fns])
            attn(1 - p, hooks=hk)
            for fn in rest + hooks: fn()
            halo(p)
            return
        if ORD == 0:
            proj(t - 2, p); attn(1 - p, hooks=hooks); qkv(t, p)
        elif ORD == 1:
            proj(t - 2, p); qkv(t, p); attn(1 - p, hooks=hooks); halo(p)
        elif ORD == 2:
            qkv(t, p); proj(t - 2, p); attn(1 - p, hooks=hooks); halo(p)
        elif ORD == 3:
            qkv(t, p); attn(1 - p, hooks=hooks); proj(t - 2, p); halo(p)

    def transpose_part(j, i):
        r0 = j * PW if isinstance(j, int) else pl.multiple_of(j * PW, PW)
        w_s[j, :, i * PW:(i + 1) * PW] = pltpu.bitcast(wst_s[i, pl.ds(r0, PW), :].T, u32)

    def transposes(j):
        return [functools.partial(transpose_part, j, i) for i in range(3)]

    zpad = jnp.zeros((NT, PAD, 128), f32)
    ka_s[2, :, 0:PAD, :] = zpad
    va_s[2, :, 0:PAD, :] = zpad
    gacc_s[...] = jnp.zeros(gacc_s.shape, f32)
    def prep_part(i):
        to_t1(pltpu.bitcast(wqkv_s[:, i * D:(i + 1) * D].T, u32), i * (D // 2))
        permute_rows(i * (D // 2), wpt_s)

    SETS = (2, 3, 0, 1)

    def first_block(i, b):
        y = _dot_nt(xa_s[b * RB:(b + 1) * RB, :], wpt_part(i))
        p = SETS[b]
        for c in range(NT):
            yc = y[:, c * 128:(c + 1) * 128]
            if i == 0:
                qa_s[p, c] = yc * scale_a
            else:
                ref = ka_s if i == 1 else va_s
                ref[p, c, PAD:, :] = yc
                if b < 3:
                    ref[SETS[b + 1], c, 0:PAD, :] = yc[RB - PAD:]

    EXP = CFG('EXP', 0)
    def phase_a():
        with jax.named_scope("s_w0"):
            cp_wqkv[0].wait()
        with jax.named_scope("s_a0"):
            prep_part(0)
            cp_x01.wait()
            first_block(0, 0); first_block(0, 1)
        with jax.named_scope("s_w1"):
            cp_x23.wait()
            cp_wqkv[1].wait()
        with jax.named_scope("s_a1"):
            first_block(0, 2); first_block(0, 3); prep_part(1)
        with jax.named_scope("s_w2"):
            cp_wqkv[2].wait()
        with jax.named_scope("s_a2"):
            first_block(1, 0); first_block(1, 1); prep_part(2)
            first_block(2, 0); first_block(2, 1)
        with jax.named_scope("s_w3"):
            cp_woa.wait()
        with jax.named_scope("s_a3"):
            for c in cp_wo:
                c.start()
            first_block(1, 2); first_block(2, 2)
            attn(SETS[0], first=True)
            to_t1(pltpu.bitcast(woa_s[...], u32), 3 * (D // 2))
            permute_rows(3 * (D // 2), wop_s)
            first_block(1, 3); first_block(2, 3)
            attn(SETS[1])
            proj(0, SETS[0])
            attn(SETS[2])
            proj(1, SETS[1])
            halo(1)

        def a_body(k, carry):
          with jax.named_scope("s_abody"):
            for c in cp_loop(k):
                c.wait()
            t = 4 + 2 * k
            tick(t, 0, transposes(2 * k)); tick(t + 1, 1, transposes(2 * k + 1))
          return carry

        lax.fori_loop(0, NLOOP, a_body, 0)

    if EXP:
        for c in [cp_wqkv[0], cp_x01, cp_x23, cp_wqkv[1], cp_wqkv[2], cp_woa]:
            c.wait()
        for c in cp_wo:
            c.start()
        for k in range(NLOOP):
            for c in cp_loop(k):
                c.wait()
    else:
        phase_a()

    def wpair(j):
        return pltpu.bitcast(w_s[j], bf16)

    def deferred_rows(g, n):
        return jnp.concatenate(
            [xb_s[pl.ds(pl.multiple_of((4 * g + i) * SEG, SEG), 8), :] for i in range(4 * n)], axis=0)

    def pre_f(j):
        y = _dot(pltpu.bitcast(pl_s[...], bf16), wpair(j))
        for g in range(NPRE):
            dq_s[g, j] = y[g * 32:(g + 1) * 32]

    def wo_convert(c):
        wo_s[c * (WOC // 2):(c + 1) * (WOC // 2), :] = pltpu.bitcast(wost_s[c * WOC:(c + 1) * WOC, :], u32)

    def interleave(mxu, side):
        side = list(side)
        per = -(-len(side) // len(mxu))
        for fn in mxu:
            fn()
            for sf in side[:per]:
                sf()
            side = side[per:]

    PF = lambda js: [functools.partial(pre_f, j) for j in js]
    N1, N2 = CFG('N1', 4), CFG('N2', 10)
    def phase_p():
        with jax.named_scope("s_p0"):
            for c in cp_xb + [cp_mem] + cp_wlast[12] + cp_wlast[13]:
                c.wait()
            for c in cp_xb2:
                c.start()
            pl_s[...] = pltpu.bitcast(deferred_rows(0, NPRE), u32)
            proj(NB - 2, 0); pre_f(0); attn(1); pre_f(1)
            proj(NB - 1, 1)
            interleave(PF(range(2, N1)), transposes(12) + transposes(13))
        with jax.named_scope("s_p1"):
            for c in cp_wlast[14] + cp_wlast[15]:
                c.wait()
            interleave(PF(range(N1, N2)), transposes(14) + transposes(15))
            for fn in PF(range(N2, NP)):
                fn()
        with jax.named_scope("s_p2"):
            for c in cp_wo:
                c.wait()

    if EXP:
        for c in cp_xb + [cp_mem] + sum(cp_wlast.values(), []) + cp_wo:
            c.wait()
        for c in cp_xb2:
            c.start()
    else:
        phase_p()

    scale_b = E ** (-0.5)
    ri = lax.broadcasted_iota(jnp.int32, (32, 2 * L), 0)
    ci = lax.broadcasted_iota(jnp.int32, (32, 2 * L), 1)
    is_even = ci < L
    cj = jnp.where(is_even, ci, ci - L)
    mask = (ri < MEM) | (ri >= cj) | (cj >= 32)
    rd = lax.broadcasted_iota(jnp.int32, (32, 64), 0)
    cd = lax.broadcasted_iota(jnp.int32, (32, 64), 1)
    same_seg = (rd >> 3) == ((cd & 31) >> 3)
    causal_d = (cd < 32) | ((cd & 31) <= rd)

    def blk(a):
        ev = lax.broadcasted_iota(jnp.int32, a.shape, 1) < E
        return jnp.concatenate([jnp.where(ev, a, 0.0), jnp.where(ev, 0.0, a)], axis=0).astype(bf16)

    def wo_rows(j):
        r0 = j * E if isinstance(j, int) else pl.multiple_of(j * E, 8)
        return pltpu.bitcast(wo_s[pl.ds(r0, E), :], bf16)

    def deferred_scores_packed(pslot, ppar, j):
        q = dq_s[pslot, j, :, 0:PW].astype(bf16)
        k = jnp.concatenate([kvm_s[ppar, j, :, 0:PW], dq_s[pslot, j, :, PW:2 * PW]], axis=0)
        r2 = lax.broadcasted_iota(jnp.int32, (32, 128), 0)
        c2 = lax.broadcasted_iota(jnp.int32, (32, 128), 1)
        ev = c2 < 64
        same = (r2 >> 3) == ((c2 & 31) >> 3)
        caus = ((c2 & 63) < 32) | ((c2 & 31) <= r2)
        sc = _dot_nt(q, blk(k)) * scale_b
        sc = jnp.where(same, jnp.where(caus, sc, NEG), -jnp.inf)
        m_e = jnp.max(jnp.where(ev, sc, -jnp.inf), axis=1, keepdims=True)
        m_o = jnp.max(jnp.where(ev, -jnp.inf, sc), axis=1, keepdims=True)
        e = jnp.exp(sc - jnp.where(ev, m_e, m_o))
        l_e = jnp.sum(jnp.where(ev, e, 0.0), axis=1, keepdims=True)
        l_o = jnp.sum(jnp.where(ev, 0.0, e), axis=1, keepdims=True)
        return (e * jnp.where(ev, _rcp(l_e), _rcp(l_o))).astype(bf16)

    def deferred_scores(pslot, ppar, j):
        if CFG('DPACK', 0):
            return deferred_scores_packed(pslot, ppar, j)
        q = dq_s[pslot, j, :, 0:PW].astype(bf16)
        k = jnp.concatenate([kvm_s[ppar, j, :, 0:PW], dq_s[pslot, j, :, PW:2 * PW]], axis=0)
        lane = lax.broadcasted_iota(jnp.int32, (64, 256), 1)
        ps = []
        for qh, kh in ((q[:, 0:256], jnp.where(lane < E, k[:, 0:256], 0.0)),
                       (q[:, 128:PW], jnp.where(lane >= 64, k[:, 128:PW], 0.0))):
            sc = _dot_nt(qh, kh.astype(bf16)) * scale_b
            sc = jnp.where(same_seg, jnp.where(causal_d, sc, NEG), -jnp.inf)
            e = jnp.exp(sc - jnp.max(sc, axis=1, keepdims=True))
            ps.append(e * _rcp(jnp.sum(e, axis=1, keepdims=True)))
        return jnp.concatenate(ps, axis=1).astype(bf16)

    def dstage1(pslot, ppar, j):
        q = dq_s[pslot, j, :, 0:PW].astype(bf16)
        k = jnp.concatenate([kvm_s[ppar, j, :, 0:PW], dq_s[pslot, j, :, PW:2 * PW]], axis=0)
        lane = lax.broadcasted_iota(jnp.int32, (64, 256), 1)
        out = []
        for qh, kh in ((q[:, 0:256], jnp.where(lane < E, k[:, 0:256], 0.0)),
                       (q[:, 128:PW], jnp.where(lane >= 64, k[:, 128:PW], 0.0))):
            sc = _dot_nt(qh, kh.astype(bf16)) * scale_b
            out.append(jnp.where(same_seg, jnp.where(causal_d, sc, NEG), -jnp.inf))
        return out

    def dstage2(scs):
        return [jnp.exp(sc - jnp.max(sc, axis=1, keepdims=True)) for sc in scs]

    def dstage3(es):
        return [e * _rcp(jnp.sum(e, axis=1, keepdims=True)) for e in es]

    def dstage4(ps):
        return jnp.concatenate(ps, axis=1).astype(bf16)

    def deferred_values(pslot, ppar, j, p):
        v = jnp.concatenate([kvm_s[ppar, j, :, PW:2 * PW], dq_s[pslot, j, :, 2 * PW:]], axis=0)
        return _dot(p, blk(v)).astype(bf16)

    def group(g, with_f, with_g, unroll):
        slot = lax.rem(g, NSLOT)
        pslot = lax.rem(g + NSLOT - 1, NSLOT)
        fslot = lax.rem(g + NPRE, NSLOT)
        par = lax.rem(g, 2)

        def step(i):
            static = isinstance(i, int)
            r0 = pl.multiple_of((g * 4 + i) * SEG, SEG)
            drow = pl.ds(i * 8 if static else pl.multiple_of(i * 8, 8), 8)
            h = jnp.concatenate([mem_s[...], xb_s[pl.ds(r0 + 8, 24), :]], axis=0)
            fl = deferred_rows(jnp.minimum(g + NPRE, NG - 1) if EXP else g + NPRE, 1) if with_f else None
            qq, qk, vm, pp, oo, dp, do, acc = {}, {}, {}, {}, {}, {}, {}, [None]
            gl = [None]

            MAT = CFG('MAT', 0)
            def pk(a):
                return pltpu.bitcast(a.astype(bf16), u32)
            def unpk(a):
                return pltpu.bitcast(a, bf16)

            def blk_store(ref, j, y):
                z8 = jnp.zeros((8, 128), f32)
                lo = lax.broadcasted_iota(jnp.int32, (L, 128), 1) < 64
                y1 = y[:, 128:256]
                ref[j, 0:24, :] = pk(jnp.concatenate([y[:, 0:128], z8], axis=0))
                ref[j, 24:64, :] = pk(jnp.concatenate([jnp.where(lo, y1, 0.0), jnp.where(lo, 0.0, y1)], axis=0))
                ref[j, 64:88, :] = pk(jnp.concatenate([z8, y[:, 256:]], axis=0))

            def blk_load(ref, j):
                z = jnp.zeros((32, 128), bf16)
                return jnp.concatenate([jnp.concatenate([unpk(ref[j, 0:24, :]), z], axis=0),
                                        unpk(ref[j, 24:64, :]),
                                        jnp.concatenate([z, unpk(ref[j, 64:88, :])], axis=0)], axis=1)

            def Ppart(j, c):
                y = _dot(h, pltpu.bitcast(w_s[j, :, c * PW:(c + 1) * PW], bf16))
                if c == 0:
                    if MAT & 1:
                        mq_s[j] = pk(y)
                    else:
                        qq[j] = y.astype(bf16)
                    return
                if CFG('KST', 1):
                    cur_s[j, :, (c - 1) * PW:c * PW] = y[:MEM]
                else:
                    kvm_s[par, j, drow, (c - 1) * PW:c * PW] = y[:MEM]
                if MAT & 2:
                    blk_store(mk_s if c == 1 else mv_s, j, jnp.concatenate([y, dq_s[slot, j, drow, c * PW:(c + 1) * PW]], axis=0))
                    return
                y = blk(jnp.concatenate([y, dq_s[slot, j, drow, c * PW:(c + 1) * PW]], axis=0))
                if c == 1:
                    qk[j] = y
                else:
                    vm[j] = y

            def Sx(j):
                q = unpk(mq_s[j]) if MAT & 1 else qq.pop(j)
                km = blk_load(mk_s, j) if MAT & 2 else qk.pop(j)
                sc = jnp.where(mask, _dot_nt(q, km) * scale_b, NEG)
                m_e = jnp.max(jnp.where(is_even, sc, -jnp.inf), axis=1, keepdims=True)
                m_o = jnp.max(jnp.where(is_even, -jnp.inf, sc), axis=1, keepdims=True)
                pp[j] = jnp.exp(sc - jnp.where(is_even, m_e, m_o))
                if "N" not in pat:
                    Nx(j)

            def Nx(j):
                e = pp[j]
                l_e = jnp.sum(jnp.where(is_even, e, 0.0), axis=1, keepdims=True)
                l_o = jnp.sum(jnp.where(is_even, 0.0, e), axis=1, keepdims=True)
                pp[j] = (e * jnp.where(is_even, _rcp(l_e), _rcp(l_o))).astype(bf16)

            def V(j):
                o = _dot(pp.pop(j), blk_load(mv_s, j) if MAT & 2 else vm.pop(j))
                if MAT & 4:
                    mo_s[j] = pk(o)
                else:
                    oo[j] = o.astype(bf16)

            def O(j):
                if with_g:
                    wj = wo_rows(j)
                else:
                    wj = wost_s[j * PW:(j + 1) * PW, :]
                    wo_s[j * E:(j + 1) * E, :] = pltpu.bitcast(wj, u32)
                if CFG('O2', 0) and with_g:
                    if j % 2 == 0:
                        return
                    wj = pltpu.bitcast(wo_s[(j - 1) * E:(j + 1) * E, :], bf16)
                    r = _dot(jnp.concatenate([oo.pop(j - 1), oo.pop(j)], axis=1), wj)
                else:
                    r = _dot(unpk(mo_s[j]) if MAT & 4 else oo.pop(j), wj)
                acc[0] = r if acc[0] is None else acc[0] + r

            def F(t):
                dq_s[fslot, i * 4 + t] = _dot(fl, wpair(i * 4 + t))

            def DS(t):
                dp[t] = deferred_scores(pslot, 1 - par, i * 4 + t)

            def D1(t):
                dp[t] = dstage1(pslot, 1 - par, i * 4 + t)

            def D2(_):
                for t in range(4):
                    dp[t] = dstage2(dp[t])

            def D3(_):
                for t in range(4):
                    dp[t] = dstage3(dp[t])

            def D4(_):
                for t in range(4):
                    dp[t] = dstage4(dp[t])

            def DV(t):
                do[t] = deferred_values(pslot, 1 - par, i * 4 + t, dp.pop(t))

            def G(t):
                r = _dot(do.pop(t), wo_rows(i * 4 + t))
                if CFG('GREG', 0):
                    gl[0] = r if gl[0] is None else gl[0] + r
                    if t == 3:
                        gacc_s[...] += gl[0]
                else:
                    gacc_s[...] += r

            d1, d2, d3 = [int(v) for v in CFG('DIST', '1,2,1').split(',')]
            seq = []
            pat = CFG('PAT', 'q,k,V,S,O,v').split(',')
            for t in range(NP + d1 + d2 + d3):
                idx = {"q": t, "k": t, "v": t - CFG('LV', 0), "S": t - d1, "N": t - d1 - 1, "V": t - d1 - d2, "O": t - d1 - d2 - d3}
                seq += [(nm, idx[nm]) for nm in pat if 0 <= idx[nm] < NP]
            fns = {"q": lambda j: Ppart(j, 0), "k": lambda j: Ppart(j, 1), "v": lambda j: Ppart(j, 2),
                   "S": Sx, "N": Nx, "V": V, "O": O}
            if with_f:
                place = CFG('PLD', 'a0@Z0,a1@Z0,a2@Z0,a3@Z0,b0@k1,c0@k2,d0@k3,B0@v3,B1@v3,B2@v4,B3@v4') + ',' + CFG('PLF', 'F0@O11,F1@O12,F2@O13,F3@O14,G0@O15,G1@O15,G2@O15,G3@O15')
            else:
                place = CFG('PLDN', 'a0@Z0,a1@Z0,a2@Z0,a3@Z0,b0@k1,c0@k2,d0@k3,B0@v3,B1@v3,B2@v4,B3@v4') + ',' + CFG('PLN', 'G0@O13,G1@O13,G2@O14,G3@O15')
            ffn = {"A": DS, "B": DV, "F": F, "G": G, "a": D1, "b": D2, "c": D3, "d": D4}
            place = [x.split('@') for x in place.split(',')]
            place = [(f, at) for f, at in place if with_g or f[0] == "F"]
            for nm, j in [("Z", 0)] + seq:
                if nm != "Z":
                    fns[nm](j)
                while place and place[0][1] == f"{nm}{j}":
                    f = place.pop(0)[0]
                    ffn[f[0]](int(f[1:]))
            assert not place
            if CFG('KST', 1):
                kvm_s[par, :, drow, :] = cur_s[...]
            out = acc[0].astype(bf16)
            mem_s[...] = out[:MEM]
            outb_s[pl.ds(r0 + 8, 24), :] = out[MEM:]

        if unroll == 4:
            for i in range(4):
                step(i)
        else:
            def inner(ii, carry):
                for u in range(unroll):
                    step(ii * unroll + u)
                return carry
            lax.fori_loop(0, 4 // unroll, inner, 0)
        if with_g:
            write_deferred(g - 1, gacc_s[...])
            gacc_s[...] = jnp.zeros(gacc_s.shape, f32)
            cp_outb(g - 1).start()

    def write_deferred(g, val):
        r = val.astype(bf16)
        for i in range(4):
            outb_s[pl.ds(pl.multiple_of((g * 4 + i) * SEG, SEG), 8), :] = r[i * 8:(i + 1) * 8]

    def g_with_f(g, carry):
        with jax.named_scope("s_gF"):
            group(g, True, True, 4)
        return carry

    def g_no_f(g, carry):
        with jax.named_scope("s_gN"):
            group(g, False, True, 2)
        return carry

    cp_outa.start()
    if not EXP:
      with jax.named_scope("s_g0"):
        group(jnp.int32(0), True, False, 1)
    for c in cp_xb2:
        c.wait()
    if EXP == 1:
        lax.fori_loop(1, NG, g_with_f, 0)
    elif EXP == 2:
        lax.fori_loop(1, NG, g_no_f, 0)
    else:
        lax.fori_loop(1, NG - NPRE, g_with_f, 0)
        lax.fori_loop(NG - NPRE, NG, g_no_f, 0)

    gl = NG - 1
    r_last = gl * 4 * SEG
    cp_main = [pltpu.make_async_copy(outb_s.at[pl.ds(r_last + i * SEG + 8, 24)],
                                     out_h.at[pl.ds(r_last + i * SEG + 8, 24), pl.ds(D, D)], sem_out.at[gl])
               for i in range(4)]
    cp_def = [pltpu.make_async_copy(outb_s.at[pl.ds(r_last + i * SEG, 8)],
                                    out_h.at[pl.ds(r_last + i * SEG, 8), pl.ds(D, D)], sem_out.at[NG + 1])
              for i in range(4)]
    for c in cp_main:
        c.start()
    dp, do, acc = {}, {}, [None]
    js = lambda b: range(4 * b, 4 * b + 4)

    def e_a(b):
        for j in js(b):
            dp[j] = dstage1(gl % NSLOT, gl % 2, j)

    def e_st(fn):
        def run(b):
            for j in js(b):
                dp[j] = fn(dp[j])
        return run

    def e_B(b):
        for j in js(b):
            do[j] = deferred_values(gl % NSLOT, gl % 2, j, dp.pop(j))

    def e_G(b):
        for j in js(b):
            r = _dot(do.pop(j), wo_rows(j))
            acc[0] = r if acc[0] is None else acc[0] + r

    efn = {"a": e_a, "b": e_st(dstage2), "c": e_st(dstage3), "d": e_st(dstage4), "B": e_B, "G": e_G}
    for it in CFG('EPI', 'a0,a1,b0,a2,b1,c0,a3,b2,c1,d0,b3,B0,c2,d1,B1,c3,d2,G0,B2,d3,G1,B3,G2,G3').split(','):
        efn[it[0]](int(it[1:]))
    write_deferred(gl, acc[0])
    for c in cp_def:
        c.start()
    cp_outa.wait()
    for g in range(NG - 1):
        cp_outb(g).wait()
    for c in cp_main + cp_def:
        c.wait()


@functools.partial(jax.jit, static_argnames=("B_seg_len",))
def pallas_concat_heads__sliding_local_dilated__memory_aug_recurrent_mem_tr__prompt_kernel(
    A_x, A_wqkv, A_wo, B_x, B_mem0, B_Wq, B_Wk, B_Wv, B_Wo, B_seg_len,
):
    assert int(B_seg_len) == SEG
    assert A_x.shape == (1, S, D) and B_x.shape == (1, S, D) and B_mem0.shape == (1, MEM, D)
    assert B_Wq.shape == (D, HB, E) and B_Wo.shape == (HB, E, D)
    wt = lambda w: w.transpose(1, 2, 0).reshape(HB * E, D)
    V = pltpu.VMEM
    scratch = [
        V((S, D), bf16), V((D, 3 * D), bf16), V((D, D), bf16), V((S, D), bf16),
        V((3, HB * E, D), bf16), V((HB * E, D), bf16),
        V((NT, 4 * (D // 2), 128), u32), V((3 * D // 2, D), u32), V((D // 2, D), u32),
        V((4, NT, RB, 128), f32), V((4, NT, PAD + RB, 128), f32), V((4, NT, PAD + RB, 128), f32),
        V((4, RB, D), f32), V((S, D), bf16),
        V((NP, D // 2, 3 * PW), u32), V((HB * E // 2, D), u32), V((MEM, D), bf16),
        V((NSLOT, NP, 32, 3 * PW), f32), V((2, NP, 32, 2 * PW), f32), V((32, D), f32), V((S, D), bf16), V((NPRE * 16, D), u32),
        V((NP, 16, PW), u32), V((NP, 88, 128), u32), V((NP, 88, 128), u32), V((NP, 16, PW), u32), V((NP, MEM, 2 * PW), f32),
        pltpu.SemaphoreType.DMA((6,)), pltpu.SemaphoreType.DMA(((NB - 4) // 2,)),
        pltpu.SemaphoreType.DMA((7,)), pltpu.SemaphoreType.DMA((NWO,)), pltpu.SemaphoreType.DMA((NG + 2,)),
    ]
    out = pl.pallas_call(
        _kernel,
        out_shape=jax.ShapeDtypeStruct((S, 2 * D), bf16),
        in_specs=[pl.BlockSpec(memory_space=pl.ANY)] * 9,
        out_specs=pl.BlockSpec(memory_space=pl.ANY),
        scratch_shapes=scratch,
        compiler_params=pltpu.CompilerParams(vmem_limit_bytes=120 * 1024 * 1024),
    )(A_x.reshape(S, D), A_wqkv, A_wo, B_x.reshape(S, D), B_mem0.reshape(MEM, D),
      wt(B_Wq), wt(B_Wk), wt(B_Wv), B_Wo.reshape(HB * E, D))
    return out.reshape(1, S, 2 * D)
```

```python
import functools
CFG = lambda k, d: d

import jax
import jax.numpy as jnp
from jax import lax
import jax.experimental.pallas as pl
import jax.experimental.pallas.tpu as pltpu

f32, bf16, u32 = jnp.float32, jnp.bfloat16, jnp.uint32

S, D = 2048, 640
NT = D // 128
HD = D // 2
LOG2E = 1.4426950408889634
NEG = -1000000000.0 * LOG2E
HA, DH, WIN, DIL = 32, 20, 8, 2
PAD = 16
RB = 128
NB = S // RB
NGR = RB // 8
SCALE_A = DH ** (-0.5) * LOG2E
HB, E, MEM, SEG = 32, 192, 8, 32
NP = HB // 2
PW = 2 * E
L = MEM + SEG
NG = S // (4 * SEG)
NPRE = 4
NSLOT = NPRE + 2
XB1 = (NPRE + 1) * 4 * SEG
SCALE_B = E ** (-0.5) * LOG2E


def _dot(a, b):
    return jnp.dot(a, b, preferred_element_type=f32)


def _dot_nt(a, b):
    return lax.dot_general(a, b, (((1,), (1,)), ((), ())), preferred_element_type=f32)


def _rcp(x):
    r = pl.reciprocal(x, approx=True)
    return r * (2.0 - x * r)


def _pack(x):
    return pltpu.bitcast(x, u32)


def _unpack(x):
    return pltpu.bitcast(x, bf16)


def _kernel(xa_h, wqkv_h, woa_h, xb_h, mem0_h, wq_h, wk_h, wv_h, wob_h, out_h,
            xa_s, wqkv_s, woa_s, xb_s, wst_s, wost_s,
            t1_s, wpt_s, wop_s, qa_s, ka_s, va_s, oa_s, outa_s, zero_s,
            w_s, wo_s, mem_s, pl_s, dq_s, cur_s, kvm_s, gacc_s, outb_s,
            sem_in, sem_out):
    EXP = CFG('EXP', 0)
    TL = CFG('TL', 0)
    NLOOP = (NB - 4) // 3
    def rows_copy(src, dst, r0, n, k):
        return pltpu.make_async_copy(src.at[pl.ds(r0, n)], dst.at[pl.ds(r0, n)], sem_in.at[k])

    def w_copies(j0, j1, k):
        return [rows_copy(w, wst_s.at[i], j0 * PW, (j1 - j0) * PW, k) for i, w in enumerate((wq_h, wk_h, wv_h))]

    cp_wqkv = [pltpu.make_async_copy(wqkv_h.at[:, pl.ds(i * D, D)], wqkv_s.at[:, pl.ds(i * D, D)], sem_in.at[i])
               for i in range(3)]
    cp_x01 = rows_copy(xa_h, xa_s, 0, 2 * RB, 3)
    cp_x23 = rows_copy(xa_h, xa_s, 2 * RB, 2 * RB, 4)
    cp_woa = pltpu.make_async_copy(woa_h, woa_s, sem_in.at[5])
    cp_xa = rows_copy(xa_h, xa_s, 4 * RB, S - 4 * RB, 6)
    cp_xb1 = [rows_copy(xb_h, xb_s, 0, XB1, 7), pltpu.make_async_copy(mem0_h, mem_s, sem_in.at[7])]
    NW0 = NLOOP * TL
    cp_w1 = w_copies(NW0, 12, 8)
    cp_w2 = w_copies(12, NP, 9)
    cp_wo = pltpu.make_async_copy(wob_h, wost_s, sem_in.at[10])
    cp_xb2 = rows_copy(xb_h, xb_s, XB1, S - XB1, 11)
    cp_w0 = lambda k: [rows_copy(w, wst_s.at[i], k * PW, PW, 12 + k) for i, w in enumerate((wq_h, wk_h, wv_h))]

    def out_copy(src, r0, n, col, k):
        return pltpu.make_async_copy(src.at[pl.ds(r0, n)], out_h.at[pl.ds(r0, n), pl.ds(col, D)], sem_out.at[k])

    cp_outa = out_copy(outa_s, 0, S, 0, NG + 1)
    cp_outb = lambda g: out_copy(outb_s, g * 4 * SEG, 4 * SEG, D, g)

    order = [[cp_wqkv[0]], [cp_x01], [cp_x23], [cp_wqkv[1]], [cp_wqkv[2]], [cp_woa], [cp_xa]]
    order += [cp_w0(k) for k in range(NW0)]
    order += [cp_xb1, cp_w1, cp_w2, [cp_wo], [cp_xb2]]

    def start_item(i, carry):
        for k, cps in enumerate(order):
            @pl.when(i == k)
            def _(cps=cps):
                for c in cps:
                    c.start()
        return carry

    lax.fori_loop(0, len(order), start_item, 0)

    def wait(*cps):
        for c in cps:
            c.wait()

    def permute_rows(val, base, dst_ref, dst_base):
        lo16, hi16 = jnp.uint32(0xFFFF), jnp.uint32(0xFFFF0000)
        for c in range(NT):
            t1_s[c, base:base + HD, :] = val[:, c * 128:(c + 1) * 128]
        for dp in range(DH // 2):
            for hb in range(2):
                for c in range(NT):
                    a = t1_s[c, pl.ds(base + hb * 160 + dp, 8, stride=DH), :]
                    b = t1_s[c, pl.ds(base + hb * 160 + DH // 2 + dp, 8, stride=DH), :]
                    r = dst_base + 2 * dp * 16 + hb * 8
                    dst_ref[r:r + 8, c * 128:(c + 1) * 128] = (a & lo16) | (b << 16)
                    dst_ref[r + 16:r + 24, c * 128:(c + 1) * 128] = (a >> 16) | (b & hi16)

    def prep_wqkv(i):
        permute_rows(_pack(wqkv_s[:, i * D:(i + 1) * D].T), i * HD, wpt_s, i * HD)

    def token(y):
        return pltpu.bitcast(y[RB - 8:, 0:128], u32) & zero_s[...]

    def qkv_piece(x, p, i, c, halo_set=None):
        r0 = i * HD + c * 64
        y = _dot_nt(x, _unpack(wpt_s[r0:r0 + 64, :]))
        if i == 0:
            qa_s[p, c] = y * SCALE_A
        else:
            ref = ka_s if i == 1 else va_s
            ref[p, c, PAD:, :] = y
            if halo_set is not None:
                ref[halo_set, c, 0:PAD, :] = y[RB - PAD:]
        return y

    def xa_block(b):
        return xa_s[pl.ds(b * RB if isinstance(b, int) else pl.multiple_of(b * RB, RB), RB), :]

    def proj_pieces(b, p):
        o = oa_s[p].astype(bf16)
        rows = pl.ds(b * RB if isinstance(b, int) else pl.multiple_of(b * RB, RB), RB)
        ys = []
        for c in range(NT):
            y = _dot(o, _unpack(wop_s[:, c * 128:(c + 1) * 128]))
            outa_s[rows, c * 128:(c + 1) * 128] = y.astype(bf16)
            ys.append(y)
        return ys

    def attn(p, toks, start, span, first=False, hooks=()):
        hooks = list(hooks)
        rows = lax.broadcasted_iota(jnp.int32, (8, 128), 0)

        def logits(gi):
            r0 = gi * 8
            q = [qa_s[p, c, r0:r0 + 8, :] for c in range(NT)]
            ti = start + (gi * span) // NGR
            if 0 <= ti < len(toks):
                q = [pltpu.bitcast(pltpu.bitcast(a, u32) | toks[ti], f32) for a in q]
            lg = []
            for w in range(WIN):
                o = r0 + PAD - DIL * w
                t = q[0] * ka_s[p, 0, o:o + 8, :]
                for c in range(1, NT):
                    t = t + q[c] * ka_s[p, c, o:o + 8, :]
                lg.append(t)
            return [t + pltpu.roll(t, 64, 1) for t in lg]

        nxt = logits(0)
        for gi in range(NGR):
            r0 = gi * 8
            lg = nxt
            if gi + 1 < NGR:
                nxt = logits(gi + 1)
            lg = [t + pltpu.roll(t, 32, 1) for t in lg]
            if first:
                lg = [jnp.where(rows + r0 >= DIL * w, t, NEG) if r0 < DIL * w else t for w, t in enumerate(lg)]
            m = functools.reduce(jnp.maximum, lg)
            e = [jnp.exp2(t - m) for t in lg]
            rinv = _rcp(functools.reduce(lambda a, b: a + b, e))
            for c in range(NT):
                a = None
                for w in range(WIN):
                    o = r0 + PAD - DIL * w
                    u = e[w] * va_s[p, c, o:o + 8, :]
                    a = u if a is None else a + u
                oa_s[p, r0:r0 + 8, c * 128:(c + 1) * 128] = a * rinv
            if hooks and gi == NGR // 2:
                for hk in hooks:
                    hk()

    def halo(p, pn):
        for ref in (ka_s, va_s):
            ref[pn, :, 0:PAD, :] = ref[p, :, RB:RB + PAD, :]

    def transpose_part(j, i):
        r0 = j * PW if isinstance(j, int) else pl.multiple_of(j * PW, PW)
        w_s[j, :, i * PW:(i + 1) * PW] = _pack(wst_s[i, pl.ds(r0, PW), :].T)

    SETS = (3, 1, 2, 0)
    zpad = jnp.zeros((NT, PAD, 128), f32)
    ka_s[SETS[0], :, 0:PAD, :] = zpad
    va_s[SETS[0], :, 0:PAD, :] = zpad
    zero_s[...] = jnp.zeros(zero_s.shape, u32)
    gacc_s[...] = jnp.zeros(gacc_s.shape, f32)

    def first(i, b):
        x = xa_block(b)
        return [qkv_piece(x, SETS[b], i, c, SETS[b + 1] if b < 3 else None) for c in range(NT)]

    def phase_a():
        with jax.named_scope("s_a0"):
            wait(cp_wqkv[0])
            prep_wqkv(0)
            wait(cp_x01)
            first(0, 0); first(0, 1)
        with jax.named_scope("s_a1"):
            wait(cp_x23, cp_wqkv[1])
            first(0, 2); first(0, 3); prep_wqkv(1)
        with jax.named_scope("s_a2"):
            wait(cp_wqkv[2])
            first(1, 0); first(1, 1); prep_wqkv(2)
            first(2, 0); first(2, 1)
        with jax.named_scope("s_a3"):
            wait(cp_woa)
            g = [int(v) for v in CFG('G3P', '-1,11,10,12').split(',')]
            toks = [token(y) for b in (2, 3) for i in (1, 2) for y in first(i, b)]
            permute_rows(_pack(woa_s[...]), 3 * HD, wop_s, 0)
            attn(SETS[0], toks, g[0], g[1], first=True)
            toks += [token(y) for y in proj_pieces(0, SETS[0])]
            attn(SETS[1], toks, g[2], g[3])
            halo(SETS[3], 1)
            wait(cp_xa)

        def a_body(k, carry):
            with jax.named_scope("s_abody"):
                if TL:
                    wait(*cp_w0(k))
                for u in range(3):
                    t = 4 + 3 * k + u
                    p = (4 + u) % 3
                    x = xa_block(t)
                    ys = proj_pieces(t - 3, p) + [qkv_piece(x, p, i, c) for i in range(3) for c in range(NT)]
                    attn((p + 1) % 3, [token(y) for y in ys], CFG('TOFF', -2), CFG('TNUM', 18),
                         hooks=[functools.partial(transpose_part, k, u)] if TL else [])
                    halo(p, (p + 1) % 3)
            return carry

        lax.fori_loop(0, NLOOP, a_body, 0)

    def wpair(j):
        return _unpack(w_s[j])

    def deferred_rows(g, n):
        return jnp.concatenate(
            [xb_s[pl.ds(pl.multiple_of((4 * g + i) * SEG, SEG), 8), :] for i in range(4 * n)], axis=0)

    def pre_f(j):
        ys = []
        for i in range(3):
            y = _dot(_unpack(pl_s[...]), _unpack(w_s[j, :, i * PW:(i + 1) * PW]))
            for g in range(NPRE):
                dq_s[g, j, :, i * PW:(i + 1) * PW] = y[g * 32:(g + 1) * 32]
            ys.append(y)
        return ys

    def transposes(j):
        for i in range(3):
            transpose_part(j, i)

    def phase_p():
        N1 = CFG('N1', 4)
        with jax.named_scope("s_p0"):
            wait(*cp_xb1, *cp_w1)
            pl_s[...] = _pack(deferred_rows(0, NPRE))
            for j in range(NW0, 2):
                transposes(j)
            g = [int(v) for v in CFG('GP', '-1,6,6,5').split(',')]
            toks = [token(y) for y in proj_pieces(NB - 3, (NB - 3) % 3)]
            toks += [token(y) for y in pre_f(0)]
            attn((NB - 2) % 3, toks, g[0], g[1])
            if NW0 <= 2:
                transposes(2)
            toks += [token(y) for y in pre_f(1)]
            toks += [token(y) for y in proj_pieces(NB - 2, (NB - 2) % 3)]
            attn((NB - 1) % 3, toks, g[2], g[3])
            for j in range(2, N1):
                if j + 1 >= NW0:
                    transposes(j + 1)
                pre_f(j)
                if j == 2:
                    proj_pieces(NB - 1, (NB - 1) % 3)
        with jax.named_scope("s_p1"):
            wait(*cp_w2)
            for j in range(N1, NP):
                if j + 1 < NP:
                    transposes(j + 1)
                pre_f(j)
        wait(cp_wo)

    if EXP in (1, 2):
        wait(*cp_wqkv, cp_x01, cp_x23, cp_woa, cp_xa, *cp_xb1, *cp_w1, *cp_w2, cp_wo)
        for k in range(NW0):
            wait(*cp_w0(k))
    else:
        phase_a()
        phase_p()
    cp_outa.start()

    ri = lax.broadcasted_iota(jnp.int32, (32, 2 * L), 0)
    ci = lax.broadcasted_iota(jnp.int32, (32, 2 * L), 1)
    is_even = ci < L
    cj = jnp.where(is_even, ci, ci - L)
    mask = (ri < MEM) | (ri >= cj) | (cj >= 32)
    rd = lax.broadcasted_iota(jnp.int32, (32, 64), 0)
    cd = lax.broadcasted_iota(jnp.int32, (32, 64), 1)
    same_seg = (rd >> 3) == ((cd & 31) >> 3)
    causal_d = (cd < 32) | ((cd & 31) <= rd)

    def blockdiag(a):
        ev = lax.broadcasted_iota(jnp.int32, a.shape, 1) < E
        return jnp.concatenate([jnp.where(ev, a, 0.0), jnp.where(ev, 0.0, a)], axis=0).astype(bf16)

    def wo_rows(j):
        r0 = j * E if isinstance(j, int) else pl.multiple_of(j * E, 8)
        return _unpack(wo_s[pl.ds(r0, E), :])

    def d_scores(slot, par, j):
        q = dq_s[slot, j, :, 0:PW].astype(bf16)
        k = jnp.concatenate([kvm_s[par, j, :, 0:PW], dq_s[slot, j, :, PW:2 * PW]], axis=0)
        lane = lax.broadcasted_iota(jnp.int32, (64, 256), 1)
        out = []
        for qh, kh in ((q[:, 0:256], jnp.where(lane < E, k[:, 0:256], 0.0)),
                       (q[:, 128:PW], jnp.where(lane >= 64, k[:, 128:PW], 0.0))):
            sc = _dot_nt(qh, kh.astype(bf16)) * SCALE_B
            out.append(jnp.where(same_seg, jnp.where(causal_d, sc, NEG), -jnp.inf))
        return out

    d_exp = lambda scs: [jnp.exp2(sc - jnp.max(sc, axis=1, keepdims=True)) for sc in scs]
    d_norm = lambda es: [e * _rcp(jnp.sum(e, axis=1, keepdims=True)) for e in es]
    d_join = lambda ps: jnp.concatenate(ps, axis=1).astype(bf16)

    def d_values(slot, par, j, p):
        v = jnp.concatenate([kvm_s[par, j, :, PW:2 * PW], dq_s[slot, j, :, 2 * PW:]], axis=0)
        return _dot(p, blockdiag(v)).astype(bf16)

    def write_deferred(g, val):
        r = val.astype(bf16)
        for i in range(4):
            outb_s[pl.ds(pl.multiple_of((g * 4 + i) * SEG, SEG), 8), :] = r[i * 8:(i + 1) * 8]

    def group(g, with_f, with_d, unroll):
        slot = lax.rem(g, NSLOT)
        pslot = lax.rem(g + NSLOT - 1, NSLOT)
        fslot = lax.rem(g + NPRE, NSLOT)
        par = lax.rem(g, 2)

        def step(i):
            r0 = pl.multiple_of((g * 4 + i) * SEG, SEG)
            drow = pl.ds(i * 8 if isinstance(i, int) else pl.multiple_of(i * 8, 8), 8)
            h = jnp.concatenate([mem_s[...], xb_s[pl.ds(r0 + 8, 24), :]], axis=0)
            fl = deferred_rows(jnp.minimum(g + NPRE, NG - 1) if EXP else g + NPRE, 1) if with_f else None
            qq, kk, vv, pp, oo, dp, do, acc = {}, {}, {}, {}, {}, {}, {}, [None]

            def proj(c, j):
                y = _dot(h, _unpack(w_s[j, :, c * PW:(c + 1) * PW]))
                if c == 0:
                    qq[j] = y.astype(bf16)
                else:
                    cur_s[j, :, (c - 1) * PW:c * PW] = y[:MEM]
                    y = jnp.concatenate([y, dq_s[slot, j, drow, c * PW:(c + 1) * PW]], axis=0)
                    (kk if c == 1 else vv)[j] = blockdiag(y)

            def softmax(j):
                sc = jnp.where(mask, _dot_nt(qq.pop(j), kk.pop(j)) * SCALE_B, NEG)
                m_e = jnp.max(jnp.where(is_even, sc, -jnp.inf), axis=1, keepdims=True)
                m_o = jnp.max(jnp.where(is_even, -jnp.inf, sc), axis=1, keepdims=True)
                e = jnp.exp2(sc - jnp.where(is_even, m_e, m_o))
                l_e = jnp.sum(jnp.where(is_even, e, 0.0), axis=1, keepdims=True)
                l_o = jnp.sum(jnp.where(is_even, 0.0, e), axis=1, keepdims=True)
                pp[j] = (e * jnp.where(is_even, _rcp(l_e), _rcp(l_o))).astype(bf16)

            def values(j):
                oo[j] = _dot(pp.pop(j), vv.pop(j)).astype(bf16)

            def oproj(j):
                if with_d:
                    wj = wo_rows(j)
                else:
                    wj = wost_s[j * PW:(j + 1) * PW, :]
                    wo_s[j * E:(j + 1) * E, :] = _pack(wj)
                r = _dot(oo.pop(j), wj)
                acc[0] = r if acc[0] is None else acc[0] + r

            def F(t):
                dq_s[fslot, i * 4 + t] = _dot(fl, wpair(i * 4 + t))

            def Ds(t):
                dp[t] = d_scores(pslot, 1 - par, i * 4 + t)

            def Dstage(fn):
                def run(_):
                    for t in range(4):
                        dp[t] = fn(dp[t])
                return run

            def Dv(t):
                do[t] = d_values(pslot, 1 - par, i * 4 + t, dp.pop(t))

            def G(t):
                gacc_s[...] += _dot(do.pop(t), wo_rows(i * 4 + t))

            main = {"q": (functools.partial(proj, 0), 0), "k": (functools.partial(proj, 1), 0),
                    "V": (values, 3), "S": (softmax, 1), "O": (oproj, 4), "v": (functools.partial(proj, 2), 0)}
            fill = {"a": Ds, "b": Dstage(d_exp), "c": Dstage(d_norm), "d": Dstage(d_join), "B": Dv, "F": F, "G": G}
            place = []
            if with_d:
                place += CFG('PLD', "a0@-,a1@-,a2@-,a3@-,b0@k1,c0@k2,d0@k3,B0@v3,B1@v3,B2@v4,B3@v4").split(",")
            if with_f:
                place += CFG('PLF', "F0@O11,F1@O12,F2@O13,F3@O14").split(",")
            if with_d:
                place += (CFG('PLG', "G0@O15,G1@O15,G2@O15,G3@O15") if with_f
                          else CFG('PLGN', "G0@O13,G1@O13,G2@O14,G3@O15")).split(",")

            def fillers(tag):
                while place and place[0].endswith("@" + tag):
                    f = place.pop(0)
                    fill[f[0]](int(f[1]))

            fillers("-")
            for t in range(NP + 4):
                for name, (fn, lag) in main.items():
                    if 0 <= t - lag < NP:
                        fn(t - lag)
                        fillers(f"{name}{t - lag}")
            assert not place
            kvm_s[par, :, drow, :] = cur_s[...]
            out = acc[0].astype(bf16)
            mem_s[...] = out[:MEM]
            outb_s[pl.ds(r0 + 8, 24), :] = out[MEM:]

        if unroll == 4:
            for i in range(4):
                step(i)
        else:
            def inner(ii, carry):
                for u in range(unroll):
                    step(ii * unroll + u)
                return carry
            lax.fori_loop(0, 4 // unroll, inner, 0)
        if with_d:
            write_deferred(g - 1, gacc_s[...])
            gacc_s[...] = jnp.zeros(gacc_s.shape, f32)
            cp_outb(g - 1).start()

    def run_groups(lo, hi, name, *cfg):
        def body(g, carry):
            with jax.named_scope(name):
                group(g, *cfg)
            return carry
        lax.fori_loop(lo, hi, body, 0)

    if not EXP:
        with jax.named_scope("s_g0"):
            group(jnp.int32(0), True, False, 1)
    wait(cp_xb2)
    if EXP == 1:
        run_groups(1, NG, "s_gF", True, True, 4)
    elif EXP == 2:
        run_groups(1, NG, "s_gN", False, True, 2)
    elif EXP == 3:
        for g in range(NG - 1):
            cp_outb(g).start()
    else:
        run_groups(1, NG - NPRE, "s_gF", True, True, 4)
        run_groups(NG - NPRE, NG, "s_gN", False, True, 2)

    gl = NG - 1
    cp_main = [out_copy(outb_s, (4 * gl + i) * SEG + 8, 24, D, gl) for i in range(4)]
    cp_def = [out_copy(outb_s, (4 * gl + i) * SEG, 8, D, NG) for i in range(4)]
    for c in cp_main:
        c.start()
    dp = [d_scores(gl % NSLOT, gl % 2, j) for j in range(NP)]
    for fn in (d_exp, d_norm, d_join):
        dp = [fn(x) for x in dp]
    do, acc = {}, None
    for b in range(6):
        for j in range(4 * b - 8, 4 * b - 4):
            if j >= 0:
                r = _dot(do.pop(j), wo_rows(j))
                acc = r if acc is None else acc + r
        for j in range(4 * b, min(4 * b + 4, NP)):
            do[j] = d_values(gl % NSLOT, gl % 2, j, dp[j])
    write_deferred(gl, acc)
    for c in cp_def:
        c.start()
    wait(cp_outa, *cp_main, *cp_def)
    for g in range(NG - 1):
        cp_outb(g).wait()


@jax.jit
def _run(A_x, A_wqkv, A_wo, B_x, B_mem0, B_Wq, B_Wk, B_Wv, B_Wo):
    wt = lambda w: w.transpose(1, 2, 0).reshape(HB * E, D)
    V = pltpu.VMEM
    scratch = [
        V((S, D), bf16), V((D, 3 * D), bf16), V((D, D), bf16), V((S, D), bf16),
        V((3, HB * E, D), bf16), V((HB * E, D), bf16),
        V((NT, 4 * HD + 24, 128), u32), V((3 * HD, D), u32), V((HD, D), u32),
        V((4, NT, RB, 128), f32), V((4, NT, PAD + RB, 128), f32), V((4, NT, PAD + RB, 128), f32),
        V((4, RB, D), f32), V((S, D), bf16), V((8, 128), u32),
        V((NP, HD, 3 * PW), u32), V((HB * E // 2, D), u32), V((MEM, D), bf16),
        V((NPRE * 16, D), u32), V((NSLOT, NP, 32, 3 * PW), f32),
        V((NP, MEM, 2 * PW), f32), V((2, NP, 32, 2 * PW), f32),
        V((32, D), f32), V((S, D), bf16),
        pltpu.SemaphoreType.DMA((16,)), pltpu.SemaphoreType.DMA((NG + 2,)),
    ]
    out = pl.pallas_call(
        _kernel,
        out_shape=jax.ShapeDtypeStruct((S, 2 * D), bf16),
        in_specs=[pl.BlockSpec(memory_space=pl.ANY)] * 9,
        out_specs=pl.BlockSpec(memory_space=pl.ANY),
        scratch_shapes=scratch,
        compiler_params=pltpu.CompilerParams(vmem_limit_bytes=120 * 1024 * 1024),
    )(A_x.reshape(S, D), A_wqkv, A_wo, B_x.reshape(S, D), B_mem0.reshape(MEM, D),
      wt(B_Wq), wt(B_Wk), wt(B_Wv), B_Wo.reshape(HB * E, D))
    return out.reshape(1, S, 2 * D)


def pallas_concat_heads__sliding_local_dilated__memory_aug_recurrent_mem_tr__prompt_kernel(
    A_x, A_wqkv, A_wo, B_x, B_mem0, B_Wq, B_Wk, B_Wv, B_Wo, B_seg_len,
):
    if isinstance(B_seg_len, int):
        assert B_seg_len == SEG
    assert A_x.shape == (1, S, D) and B_x.shape == (1, S, D) and B_mem0.shape == (1, MEM, D)
    assert B_Wq.shape == (D, HB, E) and B_Wo.shape == (HB, E, D)
    return _run(A_x, A_wqkv, A_wo, B_x, B_mem0, B_Wq, B_Wk, B_Wv, B_Wo)
```

```python
import functools

import jax
import jax.numpy as jnp
from jax import lax
import jax.experimental.pallas as pl
import jax.experimental.pallas.tpu as pltpu

f32, bf16, u32 = jnp.float32, jnp.bfloat16, jnp.uint32

S, D = 2048, 640
NT = D // 128
HD = D // 2
LOG2E = 1.4426950408889634
NEG = -1000000000.0 * LOG2E
HA, DH, WIN, DIL = 32, 20, 8, 2
PAD = 16
RB = 128
NB = S // RB
NGR = RB // 8
SCALE_A = DH ** (-0.5) * LOG2E
HB, E, MEM, SEG = 32, 192, 8, 32
NP = HB // 2
PW = 2 * E
L = MEM + SEG
NG = S // (4 * SEG)
NPRE = 4
NSLOT = NPRE + 2
XB1 = (NPRE + 1) * 4 * SEG
SCALE_B = E ** (-0.5) * LOG2E


def _dot(a, b):
    return jnp.dot(a, b, preferred_element_type=f32)


def _dot_nt(a, b):
    return lax.dot_general(a, b, (((1,), (1,)), ((), ())), preferred_element_type=f32)


def _rcp(x):
    r = pl.reciprocal(x, approx=True)
    return r * (2.0 - x * r)


def _pack(x):
    return pltpu.bitcast(x, u32)


def _unpack(x):
    return pltpu.bitcast(x, bf16)


def _kernel(xa_h, wqkv_h, woa_h, xb_h, mem0_h, wq_h, wk_h, wv_h, wob_h, out_h,
            xa_s, wqkv_s, woa_s, xb_s, wst_s, wost_s,
            t1_s, wpt_s, wop_s, qa_s, ka_s, va_s, oa_s, outa_s, zero_s,
            w_s, wo_s, mem_s, pl_s, dq_s, cur_s, kvm_s, gacc_s, outb_s,
            sem_in, sem_out):
    def rows_copy(src, dst, r0, n, k):
        return pltpu.make_async_copy(src.at[pl.ds(r0, n)], dst.at[pl.ds(r0, n)], sem_in.at[k])

    def w_copies(j0, j1, k):
        return [rows_copy(w, wst_s.at[i], j0 * PW, (j1 - j0) * PW, k) for i, w in enumerate((wq_h, wk_h, wv_h))]

    cp_wqkv = [pltpu.make_async_copy(wqkv_h.at[:, pl.ds(i * D, D)], wqkv_s.at[:, pl.ds(i * D, D)], sem_in.at[i])
               for i in range(3)]
    cp_x01 = rows_copy(xa_h, xa_s, 0, 2 * RB, 3)
    cp_x23 = rows_copy(xa_h, xa_s, 2 * RB, 2 * RB, 4)
    cp_woa = pltpu.make_async_copy(woa_h, woa_s, sem_in.at[5])
    cp_xa = rows_copy(xa_h, xa_s, 4 * RB, S - 4 * RB, 6)
    cp_xb1 = [rows_copy(xb_h, xb_s, 0, XB1, 7), pltpu.make_async_copy(mem0_h, mem_s, sem_in.at[7])]
    cp_w1 = w_copies(0, 12, 8)
    cp_w2 = w_copies(12, NP, 9)
    cp_wo = pltpu.make_async_copy(wob_h, wost_s, sem_in.at[10])
    cp_xb2 = rows_copy(xb_h, xb_s, XB1, S - XB1, 11)

    def out_copy(src, r0, n, col, k):
        return pltpu.make_async_copy(src.at[pl.ds(r0, n)], out_h.at[pl.ds(r0, n), pl.ds(col, D)], sem_out.at[k])

    cp_outa = out_copy(outa_s, 0, S, 0, NG + 1)
    cp_outb = lambda g: out_copy(outb_s, g * 4 * SEG, 4 * SEG, D, g)

    order = [[cp_wqkv[0]], [cp_x01], [cp_x23], [cp_wqkv[1]], [cp_wqkv[2]], [cp_woa], [cp_xa],
             cp_xb1, cp_w1, cp_w2, [cp_wo], [cp_xb2]]

    def start_item(i, carry):
        for k, cps in enumerate(order):
            @pl.when(i == k)
            def _(cps=cps):
                for c in cps:
                    c.start()
        return carry

    lax.fori_loop(0, len(order), start_item, 0)

    def wait(*cps):
        for c in cps:
            c.wait()

    def permute_rows(val, base, dst_ref, dst_base):
        lo16, hi16 = jnp.uint32(0xFFFF), jnp.uint32(0xFFFF0000)
        for c in range(NT):
            t1_s[c, base:base + HD, :] = val[:, c * 128:(c + 1) * 128]
        for dp in range(DH // 2):
            for hb in range(2):
                for c in range(NT):
                    a = t1_s[c, pl.ds(base + hb * 160 + dp, 8, stride=DH), :]
                    b = t1_s[c, pl.ds(base + hb * 160 + DH // 2 + dp, 8, stride=DH), :]
                    r = dst_base + 2 * dp * 16 + hb * 8
                    dst_ref[r:r + 8, c * 128:(c + 1) * 128] = (a & lo16) | (b << 16)
                    dst_ref[r + 16:r + 24, c * 128:(c + 1) * 128] = (a >> 16) | (b & hi16)

    def prep_wqkv(i):
        permute_rows(_pack(wqkv_s[:, i * D:(i + 1) * D].T), i * HD, wpt_s, i * HD)

    def token(y):
        return pltpu.bitcast(y[RB - 8:, 0:128], u32) & zero_s[...]

    def qkv_piece(x, p, i, c, halo_set=None):
        r0 = i * HD + c * 64
        y = _dot_nt(x, _unpack(wpt_s[r0:r0 + 64, :]))
        if i == 0:
            qa_s[p, c] = y * SCALE_A
        else:
            ref = ka_s if i == 1 else va_s
            ref[p, c, PAD:, :] = y
            if halo_set is not None:
                ref[halo_set, c, 0:PAD, :] = y[RB - PAD:]
        return y

    def xa_block(b):
        return xa_s[pl.ds(b * RB if isinstance(b, int) else pl.multiple_of(b * RB, RB), RB), :]

    def proj_pieces(b, p):
        o = oa_s[p].astype(bf16)
        rows = pl.ds(b * RB if isinstance(b, int) else pl.multiple_of(b * RB, RB), RB)
        ys = []
        for c in range(NT):
            y = _dot(o, _unpack(wop_s[:, c * 128:(c + 1) * 128]))
            outa_s[rows, c * 128:(c + 1) * 128] = y.astype(bf16)
            ys.append(y)
        return ys

    def attn(p, toks, start, span, first=False):
        rows = lax.broadcasted_iota(jnp.int32, (8, 128), 0)

        def logits(gi):
            r0 = gi * 8
            q = [qa_s[p, c, r0:r0 + 8, :] for c in range(NT)]
            ti = start + (gi * span) // NGR
            if 0 <= ti < len(toks):
                q = [pltpu.bitcast(pltpu.bitcast(a, u32) | toks[ti], f32) for a in q]
            lg = []
            for w in range(WIN):
                o = r0 + PAD - DIL * w
                t = q[0] * ka_s[p, 0, o:o + 8, :]
                for c in range(1, NT):
                    t = t + q[c] * ka_s[p, c, o:o + 8, :]
                lg.append(t)
            return [t + pltpu.roll(t, 64, 1) for t in lg]

        nxt = logits(0)
        for gi in range(NGR):
            r0 = gi * 8
            lg = nxt
            if gi + 1 < NGR:
                nxt = logits(gi + 1)
            lg = [t + pltpu.roll(t, 32, 1) for t in lg]
            if first:
                lg = [jnp.where(rows + r0 >= DIL * w, t, NEG) if r0 < DIL * w else t for w, t in enumerate(lg)]
            m = functools.reduce(jnp.maximum, lg)
            e = [jnp.exp2(t - m) for t in lg]
            rinv = _rcp(functools.reduce(lambda a, b: a + b, e))
            for c in range(NT):
                a = None
                for w in range(WIN):
                    o = r0 + PAD - DIL * w
                    u = e[w] * va_s[p, c, o:o + 8, :]
                    a = u if a is None else a + u
                oa_s[p, r0:r0 + 8, c * 128:(c + 1) * 128] = a * rinv

    def halo(p, pn):
        for ref in (ka_s, va_s):
            ref[pn, :, 0:PAD, :] = ref[p, :, RB:RB + PAD, :]

    SETS = (3, 1, 2, 0)
    zpad = jnp.zeros((NT, PAD, 128), f32)
    ka_s[SETS[0], :, 0:PAD, :] = zpad
    va_s[SETS[0], :, 0:PAD, :] = zpad
    zero_s[...] = jnp.zeros(zero_s.shape, u32)
    gacc_s[...] = jnp.zeros(gacc_s.shape, f32)

    def first(i, b):
        x = xa_block(b)
        return [qkv_piece(x, SETS[b], i, c, SETS[b + 1] if b < 3 else None) for c in range(NT)]

    wait(cp_wqkv[0])
    prep_wqkv(0)
    wait(cp_x01)
    first(0, 0); first(0, 1)
    wait(cp_x23, cp_wqkv[1])
    first(0, 2); first(0, 3); prep_wqkv(1)
    wait(cp_wqkv[2])
    first(1, 0); first(1, 1); prep_wqkv(2)
    first(2, 0); first(2, 1)
    wait(cp_woa)
    toks = [token(y) for b in (2, 3) for i in (1, 2) for y in first(i, b)]
    permute_rows(_pack(woa_s[...]), 3 * HD, wop_s, 0)
    attn(SETS[0], toks, -1, 11, first=True)
    toks += [token(y) for y in proj_pieces(0, SETS[0])]
    attn(SETS[1], toks, 10, 12)
    halo(SETS[3], 1)
    wait(cp_xa)

    def a_body(k, carry):
        for u in range(3):
            t = 4 + 3 * k + u
            p = (4 + u) % 3
            x = xa_block(t)
            ys = proj_pieces(t - 3, p) + [qkv_piece(x, p, i, c) for i in range(3) for c in range(NT)]
            attn((p + 1) % 3, [token(y) for y in ys], -2, 19)
            halo(p, (p + 1) % 3)
        return carry

    lax.fori_loop(0, (NB - 4) // 3, a_body, 0)

    def wpair(j):
        return _unpack(w_s[j])

    def deferred_rows(g, n):
        return jnp.concatenate(
            [xb_s[pl.ds(pl.multiple_of((4 * g + i) * SEG, SEG), 8), :] for i in range(4 * n)], axis=0)

    def pre_f(j):
        ys = []
        for i in range(3):
            y = _dot(_unpack(pl_s[...]), _unpack(w_s[j, :, i * PW:(i + 1) * PW]))
            for g in range(NPRE):
                dq_s[g, j, :, i * PW:(i + 1) * PW] = y[g * 32:(g + 1) * 32]
            ys.append(y)
        return ys

    def transposes(j):
        for i in range(3):
            w_s[j, :, i * PW:(i + 1) * PW] = _pack(wst_s[i, j * PW:(j + 1) * PW, :].T)

    wait(*cp_xb1, *cp_w1)
    pl_s[...] = _pack(deferred_rows(0, NPRE))
    transposes(0); transposes(1)
    toks = [token(y) for y in proj_pieces(NB - 3, (NB - 3) % 3) + pre_f(0)]
    attn((NB - 2) % 3, toks, -1, 6)
    transposes(2)
    toks += [token(y) for y in pre_f(1) + proj_pieces(NB - 2, (NB - 2) % 3)]
    attn((NB - 1) % 3, toks, 6, 5)
    for j in range(2, NP):
        if j == 4:
            wait(*cp_w2)
        if j + 1 < NP:
            transposes(j + 1)
        pre_f(j)
        if j == 2:
            proj_pieces(NB - 1, (NB - 1) % 3)
    wait(cp_wo)
    cp_outa.start()

    ri = lax.broadcasted_iota(jnp.int32, (32, 2 * L), 0)
    ci = lax.broadcasted_iota(jnp.int32, (32, 2 * L), 1)
    is_even = ci < L
    cj = jnp.where(is_even, ci, ci - L)
    mask = (ri < MEM) | (ri >= cj) | (cj >= 32)
    rd = lax.broadcasted_iota(jnp.int32, (32, 64), 0)
    cd = lax.broadcasted_iota(jnp.int32, (32, 64), 1)
    same_seg = (rd >> 3) == ((cd & 31) >> 3)
    causal_d = (cd < 32) | ((cd & 31) <= rd)

    def blockdiag(a):
        ev = lax.broadcasted_iota(jnp.int32, a.shape, 1) < E
        return jnp.concatenate([jnp.where(ev, a, 0.0), jnp.where(ev, 0.0, a)], axis=0).astype(bf16)

    def wo_rows(j):
        r0 = j * E if isinstance(j, int) else pl.multiple_of(j * E, 8)
        return _unpack(wo_s[pl.ds(r0, E), :])

    def d_scores(slot, par, j):
        q = dq_s[slot, j, :, 0:PW].astype(bf16)
        k = jnp.concatenate([kvm_s[par, j, :, 0:PW], dq_s[slot, j, :, PW:2 * PW]], axis=0)
        lane = lax.broadcasted_iota(jnp.int32, (64, 256), 1)
        out = []
        for qh, kh in ((q[:, 0:256], jnp.where(lane < E, k[:, 0:256], 0.0)),
                       (q[:, 128:PW], jnp.where(lane >= 64, k[:, 128:PW], 0.0))):
            sc = _dot_nt(qh, kh.astype(bf16)) * SCALE_B
            out.append(jnp.where(same_seg, jnp.where(causal_d, sc, NEG), -jnp.inf))
        return out

    d_exp = lambda scs: [jnp.exp2(sc - jnp.max(sc, axis=1, keepdims=True)) for sc in scs]
    d_norm = lambda es: [e * _rcp(jnp.sum(e, axis=1, keepdims=True)) for e in es]
    d_join = lambda ps: jnp.concatenate(ps, axis=1).astype(bf16)

    def d_values(slot, par, j, p):
        v = jnp.concatenate([kvm_s[par, j, :, PW:2 * PW], dq_s[slot, j, :, 2 * PW:]], axis=0)
        return _dot(p, blockdiag(v)).astype(bf16)

    def write_deferred(g, val):
        r = val.astype(bf16)
        for i in range(4):
            outb_s[pl.ds(pl.multiple_of((g * 4 + i) * SEG, SEG), 8), :] = r[i * 8:(i + 1) * 8]

    def group(g, with_f, with_d, unroll):
        slot = lax.rem(g, NSLOT)
        pslot = lax.rem(g + NSLOT - 1, NSLOT)
        fslot = lax.rem(g + NPRE, NSLOT)
        par = lax.rem(g, 2)

        def step(i):
            r0 = pl.multiple_of((g * 4 + i) * SEG, SEG)
            drow = pl.ds(i * 8 if isinstance(i, int) else pl.multiple_of(i * 8, 8), 8)
            h = jnp.concatenate([mem_s[...], xb_s[pl.ds(r0 + 8, 24), :]], axis=0)
            fl = deferred_rows(g + NPRE, 1) if with_f else None
            qq, kk, vv, pp, oo, dp, do, acc = {}, {}, {}, {}, {}, {}, {}, [None]

            def proj(c, j):
                y = _dot(h, _unpack(w_s[j, :, c * PW:(c + 1) * PW]))
                if c == 0:
                    qq[j] = y.astype(bf16)
                else:
                    cur_s[j, :, (c - 1) * PW:c * PW] = y[:MEM]
                    y = jnp.concatenate([y, dq_s[slot, j, drow, c * PW:(c + 1) * PW]], axis=0)
                    (kk if c == 1 else vv)[j] = blockdiag(y)

            def softmax(j):
                sc = jnp.where(mask, _dot_nt(qq.pop(j), kk.pop(j)) * SCALE_B, NEG)
                m_e = jnp.max(jnp.where(is_even, sc, -jnp.inf), axis=1, keepdims=True)
                m_o = jnp.max(jnp.where(is_even, -jnp.inf, sc), axis=1, keepdims=True)
                e = jnp.exp2(sc - jnp.where(is_even, m_e, m_o))
                l_e = jnp.sum(jnp.where(is_even, e, 0.0), axis=1, keepdims=True)
                l_o = jnp.sum(jnp.where(is_even, 0.0, e), axis=1, keepdims=True)
                pp[j] = (e * jnp.where(is_even, _rcp(l_e), _rcp(l_o))).astype(bf16)

            def values(j):
                oo[j] = _dot(pp.pop(j), vv.pop(j)).astype(bf16)

            def oproj(j):
                if with_d:
                    wj = wo_rows(j)
                else:
                    wj = wost_s[j * PW:(j + 1) * PW, :]
                    wo_s[j * E:(j + 1) * E, :] = _pack(wj)
                r = _dot(oo.pop(j), wj)
                acc[0] = r if acc[0] is None else acc[0] + r

            def F(t):
                dq_s[fslot, i * 4 + t] = _dot(fl, wpair(i * 4 + t))

            def Ds(t):
                dp[t] = d_scores(pslot, 1 - par, i * 4 + t)

            def Dstage(fn):
                def run(_):
                    for t in range(4):
                        dp[t] = fn(dp[t])
                return run

            def Dv(t):
                do[t] = d_values(pslot, 1 - par, i * 4 + t, dp.pop(t))

            def G(t):
                gacc_s[...] += _dot(do.pop(t), wo_rows(i * 4 + t))

            main = {"k": (functools.partial(proj, 1), 0), "q": (functools.partial(proj, 0), 0),
                    "V": (values, 3), "S": (softmax, 1), "O": (oproj, 4), "v": (functools.partial(proj, 2), 0)}
            fill = {"a": Ds, "b": Dstage(d_exp), "c": Dstage(d_norm), "d": Dstage(d_join), "B": Dv, "F": F, "G": G}
            place = []
            if with_d:
                place += "a0@- a1@- a2@- a3@- b0@k1 c0@k2 d0@k3 B0@v3 B1@v3 B2@v4 B3@v4".split()
            if with_f:
                place += ("F0@O11" if with_d else "F0@v15", "F1@O12", "F2@O13", "F3@O14")
            if with_d:
                place += ("G0@O15 G1@O15 G2@O15 G3@O15" if with_f else "G0@O13 G1@O13 G2@O14 G3@O15").split()

            def fillers(tag):
                for f in [f for f in place if f.endswith("@" + tag)]:
                    place.remove(f)
                    fill[f[0]](int(f[1]))

            fillers("-")
            for t in range(NP + 4):
                for name, (fn, lag) in main.items():
                    if 0 <= t - lag < NP:
                        fn(t - lag)
                        fillers(f"{name}{t - lag}")
            assert not place
            kvm_s[par, :, drow, :] = cur_s[...]
            out = acc[0].astype(bf16)
            mem_s[...] = out[:MEM]
            outb_s[pl.ds(r0 + 8, 24), :] = out[MEM:]

        if unroll == 4:
            for i in range(4):
                step(i)
        else:
            def inner(ii, carry):
                for u in range(unroll):
                    step(ii * unroll + u)
                return carry
            lax.fori_loop(0, 4 // unroll, inner, 0)
        if with_d:
            write_deferred(g - 1, gacc_s[...])
            gacc_s[...] = jnp.zeros(gacc_s.shape, f32)
            cp_outb(g - 1).start()

    def run_groups(lo, hi, *cfg):
        def body(g, carry):
            group(g, *cfg)
            return carry
        lax.fori_loop(lo, hi, body, 0)

    group(jnp.int32(0), True, False, 1)
    wait(cp_xb2)
    run_groups(1, NG - NPRE, True, True, 4)
    run_groups(NG - NPRE, NG, False, True, 2)

    gl = NG - 1
    cp_main = [out_copy(outb_s, (4 * gl + i) * SEG + 8, 24, D, gl) for i in range(4)]
    cp_def = [out_copy(outb_s, (4 * gl + i) * SEG, 8, D, NG) for i in range(4)]
    for c in cp_main:
        c.start()
    dp = [d_scores(gl % NSLOT, gl % 2, j) for j in range(NP)]
    for fn in (d_exp, d_norm, d_join):
        dp = [fn(x) for x in dp]
    do, acc = {}, None
    for b in range(6):
        for j in range(4 * b - 8, 4 * b - 4):
            if j >= 0:
                r = _dot(do.pop(j), wo_rows(j))
                acc = r if acc is None else acc + r
        for j in range(4 * b, min(4 * b + 4, NP)):
            do[j] = d_values(gl % NSLOT, gl % 2, j, dp[j])
    write_deferred(gl, acc)
    for c in cp_def:
        c.start()
    wait(cp_outa, *cp_main, *cp_def)
    for g in range(NG - 1):
        cp_outb(g).wait()


@jax.jit
def _run(A_x, A_wqkv, A_wo, B_x, B_mem0, B_Wq, B_Wk, B_Wv, B_Wo):
    wt = lambda w: w.transpose(1, 2, 0).reshape(HB * E, D)
    V = pltpu.VMEM
    scratch = [
        V((S, D), bf16), V((D, 3 * D), bf16), V((D, D), bf16), V((S, D), bf16),
        V((3, HB * E, D), bf16), V((HB * E, D), bf16),
        V((NT, 4 * HD + 24, 128), u32), V((3 * HD, D), u32), V((HD, D), u32),
        V((4, NT, RB, 128), f32), V((4, NT, PAD + RB, 128), f32), V((4, NT, PAD + RB, 128), f32),
        V((4, RB, D), f32), V((S, D), bf16), V((8, 128), u32),
        V((NP, HD, 3 * PW), u32), V((HB * E // 2, D), u32), V((MEM, D), bf16),
        V((NPRE * 16, D), u32), V((NSLOT, NP, 32, 3 * PW), f32),
        V((NP, MEM, 2 * PW), f32), V((2, NP, 32, 2 * PW), f32),
        V((32, D), f32), V((S, D), bf16),
        pltpu.SemaphoreType.DMA((12,)), pltpu.SemaphoreType.DMA((NG + 2,)),
    ]
    out = pl.pallas_call(
        _kernel,
        out_shape=jax.ShapeDtypeStruct((S, 2 * D), bf16),
        in_specs=[pl.BlockSpec(memory_space=pl.ANY)] * 9,
        out_specs=pl.BlockSpec(memory_space=pl.ANY),
        scratch_shapes=scratch,
        compiler_params=pltpu.CompilerParams(vmem_limit_bytes=120 * 1024 * 1024),
    )(A_x.reshape(S, D), A_wqkv, A_wo, B_x.reshape(S, D), B_mem0.reshape(MEM, D),
      wt(B_Wq), wt(B_Wk), wt(B_Wv), B_Wo.reshape(HB * E, D))
    return out.reshape(1, S, 2 * D)


def pallas_concat_heads__sliding_local_dilated__memory_aug_recurrent_mem_tr__prompt_kernel(
    A_x, A_wqkv, A_wo, B_x, B_mem0, B_Wq, B_Wk, B_Wv, B_Wo, B_seg_len,
):
    if isinstance(B_seg_len, int):
        assert B_seg_len == SEG
    assert A_x.shape == (1, S, D) and B_x.shape == (1, S, D) and B_mem0.shape == (1, MEM, D)
    assert B_Wq.shape == (D, HB, E) and B_Wo.shape == (HB, E, D)
    return _run(A_x, A_wqkv, A_wo, B_x, B_mem0, B_Wq, B_Wk, B_Wv, B_Wo)
```

```python
import functools

import jax
import jax.numpy as jnp
from jax import lax
import jax.experimental.pallas as pl
import jax.experimental.pallas.tpu as pltpu

f32, bf16, u32 = jnp.float32, jnp.bfloat16, jnp.uint32

S, D = 2048, 640
NT = D // 128
HD = D // 2
LOG2E = 1.4426950408889634
NEG = -1000000000.0 * LOG2E
HA, DH, WIN, DIL = 32, 20, 8, 2
PAD = 16
RB = 128
NB = S // RB
NGR = RB // 8
SCALE_A = DH ** (-0.5) * LOG2E
HB, E, MEM, SEG = 32, 192, 8, 32
NP = HB // 2
PW = 2 * E
L = MEM + SEG
NG = S // (4 * SEG)
NPRE = 4
NSLOT = NPRE + 2
XB1 = (NPRE + 1) * 4 * SEG
SCALE_B = E ** (-0.5) * LOG2E


def _dot(a, b):
    return jnp.dot(a, b, preferred_element_type=f32)


def _dot_nt(a, b):
    return lax.dot_general(a, b, (((1,), (1,)), ((), ())), preferred_element_type=f32)


def _rcp(x):
    r = pl.reciprocal(x, approx=True)
    return r * (2.0 - x * r)


def _pack(x):
    return pltpu.bitcast(x, u32)


def _unpack(x):
    return pltpu.bitcast(x, bf16)


def _kernel(xa_h, wqkv_h, woa_h, xb_h, mem0_h, wq_h, wk_h, wv_h, wob_h, out_h,
            xa_s, wqkv_s, woa_s, xb_s, wst_s, wost_s,
            t1_s, wpt_s, wop_s, qa_s, ka_s, va_s, oa_s, outa_s, zero_s,
            w_s, wo_s, mem_s, pl_s, dq_s, cur_s, kvm_s, gacc_s, outb_s,
            one_s, sem_in, sem_out):
    def rows_copy(src, dst, r0, n, k):
        return pltpu.make_async_copy(src.at[pl.ds(r0, n)], dst.at[pl.ds(r0, n)], sem_in.at[k])

    def w_copies(j0, j1, k):
        return [rows_copy(w, wst_s.at[i], j0 * PW, (j1 - j0) * PW, k) for i, w in enumerate((wq_h, wk_h, wv_h))]

    cp_wqkv = [pltpu.make_async_copy(wqkv_h.at[:, pl.ds(i * D, D)], wqkv_s.at[:, pl.ds(i * D, D)], sem_in.at[i])
               for i in range(3)]
    cp_x01 = rows_copy(xa_h, xa_s, 0, 2 * RB, 3)
    cp_x23 = rows_copy(xa_h, xa_s, 2 * RB, 2 * RB, 4)
    cp_woa = pltpu.make_async_copy(woa_h, woa_s, sem_in.at[5])
    cp_xa = rows_copy(xa_h, xa_s, 4 * RB, S - 4 * RB, 6)
    cp_xb1 = [rows_copy(xb_h, xb_s, 0, XB1, 7), pltpu.make_async_copy(mem0_h, mem_s, sem_in.at[7])]
    cp_w1 = w_copies(0, 12, 8)
    cp_w2 = w_copies(12, NP, 9)
    cp_wo = pltpu.make_async_copy(wob_h, wost_s, sem_in.at[10])
    cp_xb2 = rows_copy(xb_h, xb_s, XB1, S - XB1, 11)

    def out_copy(src, r0, n, col, k):
        return pltpu.make_async_copy(src.at[pl.ds(r0, n)], out_h.at[pl.ds(r0, n), pl.ds(col, D)], sem_out.at[k])

    cp_outa = out_copy(outa_s, 0, S, 0, NG + 1)
    cp_outb = lambda g: out_copy(outb_s, g * 4 * SEG, 4 * SEG, D, g)

    order = [[cp_wqkv[0]], [cp_x01], [cp_x23], [cp_wqkv[1]], [cp_wqkv[2]], [cp_woa], [cp_xa],
             cp_xb1, cp_w1, cp_w2, [cp_wo], [cp_xb2]]

    def start_item(i, carry):
        for k, cps in enumerate(order):
            @pl.when(i == k)
            def _(cps=cps):
                for c in cps:
                    c.start()
        return carry

    def wait(*cps):
        for c in cps:
            c.wait()

    def permute_rows(val, base, dst_ref, dst_base):
        lo16, hi16 = jnp.uint32(0xFFFF), jnp.uint32(0xFFFF0000)
        for c in range(NT):
            t1_s[c, base:base + HD, :] = val[:, c * 128:(c + 1) * 128]
        for dp in range(DH // 2):
            for hb in range(2):
                for c in range(NT):
                    a = t1_s[c, pl.ds(base + hb * 160 + dp, 8, stride=DH), :]
                    b = t1_s[c, pl.ds(base + hb * 160 + DH // 2 + dp, 8, stride=DH), :]
                    r = dst_base + 2 * dp * 16 + hb * 8
                    dst_ref[r:r + 8, c * 128:(c + 1) * 128] = (a & lo16) | (b << 16)
                    dst_ref[r + 16:r + 24, c * 128:(c + 1) * 128] = (a >> 16) | (b & hi16)

    def prep_wqkv(i):
        permute_rows(_pack(wqkv_s[:, i * D:(i + 1) * D].T), i * HD, wpt_s, i * HD)

    def token(y):
        return pltpu.bitcast(y[RB - 8:, 0:128], u32) & zero_s[...]

    def qkv_piece(x, p, i, c, halo_set=None):
        r0 = i * HD + c * 64
        y = _dot_nt(x, _unpack(wpt_s[r0:r0 + 64, :]))
        if i == 0:
            qa_s[p, c] = y * SCALE_A
        else:
            ref = ka_s if i == 1 else va_s
            ref[p, c, PAD:, :] = y
            if halo_set is not None:
                ref[halo_set, c, 0:PAD, :] = y[RB - PAD:]
        return y

    def xa_block(b):
        return xa_s[pl.ds(b * RB if isinstance(b, int) else pl.multiple_of(b * RB, RB), RB), :]

    def proj_pieces(b, p):
        o = oa_s[p].astype(bf16)
        rows = pl.ds(b * RB if isinstance(b, int) else pl.multiple_of(b * RB, RB), RB)
        ys = []
        for c in range(NT):
            y = _dot(o, _unpack(wop_s[:, c * 128:(c + 1) * 128]))
            outa_s[rows, c * 128:(c + 1) * 128] = y.astype(bf16)
            ys.append(y)
        return ys

    def attn(p, toks, start, span, first=False):
        rows = lax.broadcasted_iota(jnp.int32, (8, 128), 0)

        def logits(gi):
            r0 = gi * 8
            q = [qa_s[p, c, r0:r0 + 8, :] for c in range(NT)]
            ti = start + (gi * span) // NGR
            if 0 <= ti < len(toks):
                q = [pltpu.bitcast(pltpu.bitcast(a, u32) | toks[ti], f32) for a in q]
            lg = []
            for w in range(WIN):
                o = r0 + PAD - DIL * w
                t = q[0] * ka_s[p, 0, o:o + 8, :]
                for c in range(1, NT):
                    t = t + q[c] * ka_s[p, c, o:o + 8, :]
                lg.append(t)
            return [t + pltpu.roll(t, 64, 1) for t in lg]

        nxt = logits(0)
        for gi in range(NGR):
            r0 = gi * 8
            lg = nxt
            if gi + 1 < NGR:
                nxt = logits(gi + 1)
            lg = [t + pltpu.roll(t, 32, 1) for t in lg]
            if first:
                lg = [jnp.where(rows + r0 >= DIL * w, t, NEG) if r0 < DIL * w else t for w, t in enumerate(lg)]
            m = functools.reduce(jnp.maximum, lg)
            e = [jnp.exp2(t - m) for t in lg]
            rinv = _rcp(functools.reduce(lambda a, b: a + b, e))
            for c in range(NT):
                a = None
                for w in range(WIN):
                    o = r0 + PAD - DIL * w
                    u = e[w] * va_s[p, c, o:o + 8, :]
                    a = u if a is None else a + u
                oa_s[p, r0:r0 + 8, c * 128:(c + 1) * 128] = a * rinv

    def halo(p, pn):
        for ref in (ka_s, va_s):
            ref[pn, :, 0:PAD, :] = ref[p, :, RB:RB + PAD, :]

    SETS = (3, 1, 2, 0)
    def first(i, b):
        x = xa_block(b)
        return [qkv_piece(x, SETS[b], i, c, SETS[b + 1] if b < 3 else None) for c in range(NT)]

    def phase_a():
        lax.fori_loop(0, len(order), start_item, 0)
        zpad = jnp.zeros((NT, PAD, 128), f32)
        ka_s[SETS[0], :, 0:PAD, :] = zpad
        va_s[SETS[0], :, 0:PAD, :] = zpad
        zero_s[...] = jnp.zeros(zero_s.shape, u32)
        gacc_s[...] = jnp.zeros(gacc_s.shape, f32)

        wait(cp_wqkv[0])
        prep_wqkv(0)
        wait(cp_x01)
        first(0, 0); first(0, 1)
        wait(cp_x23, cp_wqkv[1])
        first(0, 2); first(0, 3); prep_wqkv(1)
        wait(cp_wqkv[2])
        first(1, 0); first(1, 1); prep_wqkv(2)
        first(2, 0); first(2, 1)
        wait(cp_woa)
        toks = [token(y) for b in (2, 3) for i in (1, 2) for y in first(i, b)]
        permute_rows(_pack(woa_s[...]), 3 * HD, wop_s, 0)
        attn(SETS[0], toks, -1, 11, first=True)
        toks += [token(y) for y in proj_pieces(0, SETS[0])]
        attn(SETS[1], toks, 10, 12)
        halo(SETS[3], 1)
        wait(cp_xa)

        def a_body(k, carry):
            for u in range(3):
                t = 4 + 3 * k + u
                p = (4 + u) % 3
                x = xa_block(t)
                ys = proj_pieces(t - 3, p) + [qkv_piece(x, p, i, c) for i in range(3) for c in range(NT)]
                attn((p + 1) % 3, [token(y) for y in ys], -2, 19)
                halo(p, (p + 1) % 3)
            return carry

        lax.fori_loop(0, (NB - 4) // 3, a_body, 0)

    def wpair(j):
        return _unpack(w_s[j])

    def deferred_rows(g, n):
        return jnp.concatenate(
            [xb_s[pl.ds(pl.multiple_of((4 * g + i) * SEG, SEG), 8), :] for i in range(4 * n)], axis=0)

    def pre_f(j):
        ys = []
        for i in range(3):
            y = _dot(_unpack(pl_s[...]), _unpack(w_s[j, :, i * PW:(i + 1) * PW]))
            for g in range(NPRE):
                dq_s[g, j, :, i * PW:(i + 1) * PW] = y[g * 32:(g + 1) * 32]
            ys.append(y)
        return ys

    def transposes(j):
        for i in range(3):
            w_s[j, :, i * PW:(i + 1) * PW] = _pack(wst_s[i, j * PW:(j + 1) * PW, :].T)

    def phase_p():
        wait(*cp_xb1, *cp_w1)
        pl_s[...] = _pack(deferred_rows(0, NPRE))
        transposes(0); transposes(1)
        toks = [token(y) for y in proj_pieces(NB - 3, (NB - 3) % 3) + pre_f(0)]
        attn((NB - 2) % 3, toks, -1, 6)
        transposes(2)
        toks += [token(y) for y in pre_f(1) + proj_pieces(NB - 2, (NB - 2) % 3)]
        attn((NB - 1) % 3, toks, 6, 5)
        for j in range(2, NP):
            if j == 4:
                wait(*cp_w2)
            if j + 1 < NP:
                transposes(j + 1)
            pre_f(j)
            if j == 2:
                proj_pieces(NB - 1, (NB - 1) % 3)
        wait(cp_wo)

    def prologue(_, carry):
        phase_a()
        phase_p()
        return carry

    one_s[0] = jnp.int32(1)
    lax.fori_loop(0, one_s[0], prologue, 0)
    cp_outa.start()

    ri = lax.broadcasted_iota(jnp.int32, (32, 2 * L), 0)
    ci = lax.broadcasted_iota(jnp.int32, (32, 2 * L), 1)
    is_even = ci < L
    cj = jnp.where(is_even, ci, ci - L)
    mask = (ri < MEM) | (ri >= cj) | (cj >= 32)
    rd = lax.broadcasted_iota(jnp.int32, (32, 64), 0)
    cd = lax.broadcasted_iota(jnp.int32, (32, 64), 1)
    same_seg = (rd >> 3) == ((cd & 31) >> 3)
    causal_d = (cd < 32) | ((cd & 31) <= rd)

    def blockdiag(a):
        ev = lax.broadcasted_iota(jnp.int32, a.shape, 1) < E
        return jnp.concatenate([jnp.where(ev, a, 0.0), jnp.where(ev, 0.0, a)], axis=0).astype(bf16)

    def wo_rows(j):
        r0 = j * E if isinstance(j, int) else pl.multiple_of(j * E, 8)
        return _unpack(wo_s[pl.ds(r0, E), :])

    def d_scores(slot, par, j):
        q = dq_s[slot, j, :, 0:PW].astype(bf16)
        k = jnp.concatenate([kvm_s[par, j, :, 0:PW], dq_s[slot, j, :, PW:2 * PW]], axis=0)
        lane = lax.broadcasted_iota(jnp.int32, (64, 256), 1)
        out = []
        for qh, kh in ((q[:, 0:256], jnp.where(lane < E, k[:, 0:256], 0.0)),
                       (q[:, 128:PW], jnp.where(lane >= 64, k[:, 128:PW], 0.0))):
            sc = _dot_nt(qh, kh.astype(bf16)) * SCALE_B
            out.append(jnp.where(same_seg, jnp.where(causal_d, sc, NEG), -jnp.inf))
        return out

    d_exp = lambda scs: [jnp.exp2(sc - jnp.max(sc, axis=1, keepdims=True)) for sc in scs]
    d_norm = lambda es: [e * _rcp(jnp.sum(e, axis=1, keepdims=True)) for e in es]
    d_join = lambda ps: jnp.concatenate(ps, axis=1).astype(bf16)

    def d_values(slot, par, j, p):
        v = jnp.concatenate([kvm_s[par, j, :, PW:2 * PW], dq_s[slot, j, :, 2 * PW:]], axis=0)
        return _dot(p, blockdiag(v)).astype(bf16)

    def write_deferred(g, val):
        r = val.astype(bf16)
        for i in range(4):
            outb_s[pl.ds(pl.multiple_of((g * 4 + i) * SEG, SEG), 8), :] = r[i * 8:(i + 1) * 8]

    def group(g, with_f, with_d, unroll):
        slot = lax.rem(g, NSLOT)
        pslot = lax.rem(g + NSLOT - 1, NSLOT)
        fslot = lax.rem(g + NPRE, NSLOT)
        par = lax.rem(g, 2)

        def step(i):
            r0 = pl.multiple_of((g * 4 + i) * SEG, SEG)
            drow = pl.ds(i * 8 if isinstance(i, int) else pl.multiple_of(i * 8, 8), 8)
            h = jnp.concatenate([mem_s[...], xb_s[pl.ds(r0 + 8, 24), :]], axis=0)
            fl = deferred_rows(g + NPRE, 1) if with_f else None
            qq, kk, vv, pp, oo, dp, do, acc = {}, {}, {}, {}, {}, {}, {}, [None]

            def proj(c, j):
                y = _dot(h, _unpack(w_s[j, :, c * PW:(c + 1) * PW]))
                if c == 0:
                    qq[j] = y.astype(bf16)
                else:
                    cur_s[j, :, (c - 1) * PW:c * PW] = y[:MEM]
                    y = jnp.concatenate([y, dq_s[slot, j, drow, c * PW:(c + 1) * PW]], axis=0)
                    (kk if c == 1 else vv)[j] = blockdiag(y)

            def softmax(j):
                sc = jnp.where(mask, _dot_nt(qq.pop(j), kk.pop(j)) * SCALE_B, NEG)
                m_e = jnp.max(jnp.where(is_even, sc, -jnp.inf), axis=1, keepdims=True)
                m_o = jnp.max(jnp.where(is_even, -jnp.inf, sc), axis=1, keepdims=True)
                e = jnp.exp2(sc - jnp.where(is_even, m_e, m_o))
                l_e = jnp.sum(jnp.where(is_even, e, 0.0), axis=1, keepdims=True)
                l_o = jnp.sum(jnp.where(is_even, 0.0, e), axis=1, keepdims=True)
                pp[j] = (e * jnp.where(is_even, _rcp(l_e), _rcp(l_o))).astype(bf16)

            def values(j):
                oo[j] = _dot(pp.pop(j), vv.pop(j)).astype(bf16)

            def oproj(j):
                if with_d:
                    wj = wo_rows(j)
                else:
                    wj = wost_s[j * PW:(j + 1) * PW, :]
                    wo_s[j * E:(j + 1) * E, :] = _pack(wj)
                r = _dot(oo.pop(j), wj)
                acc[0] = r if acc[0] is None else acc[0] + r

            def F(t):
                dq_s[fslot, i * 4 + t] = _dot(fl, wpair(i * 4 + t))

            def Ds(t):
                dp[t] = d_scores(pslot, 1 - par, i * 4 + t)

            def Dstage(fn):
                def run(_):
                    for t in range(4):
                        dp[t] = fn(dp[t])
                return run

            def Dv(t):
                do[t] = d_values(pslot, 1 - par, i * 4 + t, dp.pop(t))

            def G(t):
                gacc_s[...] += _dot(do.pop(t), wo_rows(i * 4 + t))

            main = {"k": (functools.partial(proj, 1), 0), "q": (functools.partial(proj, 0), 0),
                    "V": (values, 3), "S": (softmax, 1), "O": (oproj, 4), "v": (functools.partial(proj, 2), 0)}
            fill = {"a": Ds, "b": Dstage(d_exp), "c": Dstage(d_norm), "d": Dstage(d_join), "B": Dv, "F": F, "G": G}
            place = []
            if with_d:
                place += "a0@- a1@- a2@- a3@- b0@k1 c0@k2 d0@k3 B0@v3 B1@v3 B2@v4 B3@v4".split()
            if with_f:
                place += ("F0@O11" if with_d else "F0@v15", "F1@O12", "F2@O13", "F3@O14")
            if with_d:
                place += ("G0@O15 G1@O15 G2@O15 G3@O15" if with_f else "G0@O13 G1@O13 G2@O14 G3@O15").split()

            def fillers(tag):
                for f in [f for f in place if f.endswith("@" + tag)]:
                    place.remove(f)
                    fill[f[0]](int(f[1]))

            fillers("-")
            for t in range(NP + 4):
                for name, (fn, lag) in main.items():
                    if 0 <= t - lag < NP:
                        fn(t - lag)
                        fillers(f"{name}{t - lag}")
            assert not place
            kvm_s[par, :, drow, :] = cur_s[...]
            out = acc[0].astype(bf16)
            mem_s[...] = out[:MEM]
            outb_s[pl.ds(r0 + 8, 24), :] = out[MEM:]

        if unroll == 4:
            for i in range(4):
                step(i)
        else:
            def inner(ii, carry):
                for u in range(unroll):
                    step(ii * unroll + u)
                return carry
            lax.fori_loop(0, 4 // unroll, inner, 0)
        if with_d:
            write_deferred(g - 1, gacc_s[...])
            gacc_s[...] = jnp.zeros(gacc_s.shape, f32)
            cp_outb(g - 1).start()

    def run_groups(lo, hi, *cfg):
        def body(g, carry):
            group(g, *cfg)
            return carry
        lax.fori_loop(lo, hi, body, 0)

    group(jnp.int32(0), True, False, 1)
    wait(cp_xb2)
    run_groups(1, NG - NPRE, True, True, 4)
    run_groups(NG - NPRE, NG, False, True, 2)

    gl = NG - 1
    cp_main = [out_copy(outb_s, (4 * gl + i) * SEG + 8, 24, D, gl) for i in range(4)]
    cp_def = [out_copy(outb_s, (4 * gl + i) * SEG, 8, D, NG) for i in range(4)]
    for c in cp_main:
        c.start()
    dp = [d_scores(gl % NSLOT, gl % 2, j) for j in range(NP)]
    for fn in (d_exp, d_norm, d_join):
        dp = [fn(x) for x in dp]
    do, acc = {}, None
    for b in range(6):
        for j in range(4 * b - 8, 4 * b - 4):
            if j >= 0:
                r = _dot(do.pop(j), wo_rows(j))
                acc = r if acc is None else acc + r
        for j in range(4 * b, min(4 * b + 4, NP)):
            do[j] = d_values(gl % NSLOT, gl % 2, j, dp[j])
    write_deferred(gl, acc)
    for c in cp_def:
        c.start()
    wait(cp_outa, *cp_main, *cp_def)
    for g in range(NG - 1):
        cp_outb(g).wait()


@jax.jit
def _run(A_x, A_wqkv, A_wo, B_x, B_mem0, B_Wq, B_Wk, B_Wv, B_Wo):
    wt = lambda w: w.transpose(1, 2, 0).reshape(HB * E, D)
    V = pltpu.VMEM
    scratch = [
        V((S, D), bf16), V((D, 3 * D), bf16), V((D, D), bf16), V((S, D), bf16),
        V((3, HB * E, D), bf16), V((HB * E, D), bf16),
        V((NT, 4 * HD + 24, 128), u32), V((3 * HD, D), u32), V((HD, D), u32),
        V((4, NT, RB, 128), f32), V((4, NT, PAD + RB, 128), f32), V((4, NT, PAD + RB, 128), f32),
        V((4, RB, D), f32), V((S, D), bf16), V((8, 128), u32),
        V((NP, HD, 3 * PW), u32), V((HB * E // 2, D), u32), V((MEM, D), bf16),
        V((NPRE * 16, D), u32), V((NSLOT, NP, 32, 3 * PW), f32),
        V((NP, MEM, 2 * PW), f32), V((2, NP, 32, 2 * PW), f32),
        V((32, D), f32), V((S, D), bf16),
        pltpu.SMEM((1,), jnp.int32), pltpu.SemaphoreType.DMA((12,)), pltpu.SemaphoreType.DMA((NG + 2,)),
    ]
    out = pl.pallas_call(
        _kernel,
        out_shape=jax.ShapeDtypeStruct((S, 2 * D), bf16),
        in_specs=[pl.BlockSpec(memory_space=pl.ANY)] * 9,
        out_specs=pl.BlockSpec(memory_space=pl.ANY),
        scratch_shapes=scratch,
        compiler_params=pltpu.CompilerParams(vmem_limit_bytes=120 * 1024 * 1024),
    )(A_x.reshape(S, D), A_wqkv, A_wo, B_x.reshape(S, D), B_mem0.reshape(MEM, D),
      wt(B_Wq), wt(B_Wk), wt(B_Wv), B_Wo.reshape(HB * E, D))
    return out.reshape(1, S, 2 * D)


def pallas_concat_heads__sliding_local_dilated__memory_aug_recurrent_mem_tr__prompt_kernel(
    A_x, A_wqkv, A_wo, B_x, B_mem0, B_Wq, B_Wk, B_Wv, B_Wo, B_seg_len,
):
    if isinstance(B_seg_len, int):
        assert B_seg_len == SEG
    assert A_x.shape == (1, S, D) and B_x.shape == (1, S, D) and B_mem0.shape == (1, MEM, D)
    assert B_Wq.shape == (D, HB, E) and B_Wo.shape == (HB, E, D)
    return _run(A_x, A_wqkv, A_wo, B_x, B_mem0, B_Wq, B_Wk, B_Wv, B_Wo)
```

```python
import functools

import jax
import jax.numpy as jnp
from jax import lax
import jax.experimental.pallas as pl
import jax.experimental.pallas.tpu as pltpu

f32, bf16, u32 = jnp.float32, jnp.bfloat16, jnp.uint32

S, D = 2048, 640
NT = D // 128
HD = D // 2
LOG2E = 1.4426950408889634
NEG = -1000000000.0 * LOG2E
HA, DH, WIN, DIL = 32, 20, 8, 2
PAD = 16
RB = 128
NB = S // RB
NGR = RB // 8
SCALE_A = DH ** (-0.5) * LOG2E
HB, E, MEM, SEG = 32, 192, 8, 32
NP = HB // 2
PW = 2 * E
L = MEM + SEG
NG = S // (4 * SEG)
NPRE = 4
NSLOT = NPRE + 2
XB1 = (NPRE + 1) * 4 * SEG
SCALE_B = E ** (-0.5) * LOG2E


def _dot(a, b):
    return jnp.dot(a, b, preferred_element_type=f32)


def _dot_nt(a, b):
    return lax.dot_general(a, b, (((1,), (1,)), ((), ())), preferred_element_type=f32)


def _rcp(x):
    r = pl.reciprocal(x, approx=True)
    return r * (2.0 - x * r)


def _pack(x):
    return pltpu.bitcast(x, u32)


def _unpack(x):
    return pltpu.bitcast(x, bf16)


def _kernel(xa_h, wqkv_h, woa_h, xb_h, mem0_h, wq_h, wk_h, wv_h, wob_h, out_h,
            xa_s, wqkv_s, woa_s, xb_s, wst_s, wost_s,
            t1_s, wpt_s, wop_s, qa_s, ka_s, va_s, oa_s, outa_s, zero_s,
            w_s, wo_s, mem_s, pl_s, dq_s, cur_s, kvm_s, gacc_s, outb_s,
            one_s, sem_in, sem_out):
    def rows_copy(src, dst, r0, n, k):
        return pltpu.make_async_copy(src.at[pl.ds(r0, n)], dst.at[pl.ds(r0, n)], sem_in.at[k])

    def w_copies(j0, j1, k):
        return [rows_copy(w, wst_s.at[i], j0 * PW, (j1 - j0) * PW, k) for i, w in enumerate((wq_h, wk_h, wv_h))]

    cp_wqkv = [pltpu.make_async_copy(wqkv_h.at[:, pl.ds(i * D, D)], wqkv_s.at[:, pl.ds(i * D, D)], sem_in.at[i])
               for i in range(3)]
    cp_x01 = rows_copy(xa_h, xa_s, 0, 2 * RB, 3)
    cp_x23 = rows_copy(xa_h, xa_s, 2 * RB, 2 * RB, 4)
    cp_woa = pltpu.make_async_copy(woa_h, woa_s, sem_in.at[5])
    cp_xa = rows_copy(xa_h, xa_s, 4 * RB, S - 4 * RB, 6)
    cp_xb1 = [rows_copy(xb_h, xb_s, 0, XB1, 7), pltpu.make_async_copy(mem0_h, mem_s, sem_in.at[7])]
    cp_w1 = w_copies(0, 12, 8)
    cp_w2 = w_copies(12, NP, 9)
    cp_wo = pltpu.make_async_copy(wob_h, wost_s, sem_in.at[10])
    cp_xb2 = rows_copy(xb_h, xb_s, XB1, S - XB1, 11)

    def out_copy(src, r0, n, col, k):
        return pltpu.make_async_copy(src.at[pl.ds(r0, n)], out_h.at[pl.ds(r0, n), pl.ds(col, D)], sem_out.at[k])

    R1, R2 = (NG - NPRE - 1) * 4 * SEG, (NG - 1) * 4 * SEG
    cp_outa = out_copy(outa_s, 0, S, 0, 0)
    cp_outb1 = out_copy(outb_s, 0, R1, D, 1)
    cp_outb2 = [out_copy(outb_s, R1, R2 - R1, D, 2)] + [out_copy(outb_s, R2 + i * SEG + 8, 24, D, 2) for i in range(4)]
    cp_outb3 = [out_copy(outb_s, R2 + i * SEG, 8, D, 3) for i in range(4)]

    order = [[cp_wqkv[0]], [cp_x01], [cp_x23], [cp_wqkv[1]], [cp_wqkv[2]], [cp_woa], [cp_xa],
             cp_xb1, cp_w1, cp_w2, [cp_wo], [cp_xb2]]

    def start_item(i, carry):
        for k, cps in enumerate(order):
            @pl.when(i == k)
            def _(cps=cps):
                for c in cps:
                    c.start()
        return carry

    def wait(*cps):
        for c in cps:
            c.wait()

    def permute_rows(val, base, dst_ref, dst_base):
        lo16, hi16 = jnp.uint32(0xFFFF), jnp.uint32(0xFFFF0000)
        for c in range(NT):
            t1_s[c, base:base + HD, :] = val[:, c * 128:(c + 1) * 128]
        for dp in range(DH // 2):
            for hb in range(2):
                for c in range(NT):
                    a = t1_s[c, pl.ds(base + hb * 160 + dp, 8, stride=DH), :]
                    b = t1_s[c, pl.ds(base + hb * 160 + DH // 2 + dp, 8, stride=DH), :]
                    r = dst_base + 2 * dp * 16 + hb * 8
                    dst_ref[r:r + 8, c * 128:(c + 1) * 128] = (a & lo16) | (b << 16)
                    dst_ref[r + 16:r + 24, c * 128:(c + 1) * 128] = (a >> 16) | (b & hi16)

    def prep_wqkv(i):
        permute_rows(_pack(wqkv_s[:, i * D:(i + 1) * D].T), i * HD, wpt_s, i * HD)

    def token(y):
        return pltpu.bitcast(y[RB - 8:, 0:128], u32) & zero_s[...]

    def qkv_piece(x, p, i, c, halo_set=None):
        r0 = i * HD + c * 64
        y = _dot_nt(x, _unpack(wpt_s[r0:r0 + 64, :]))
        if i == 0:
            qa_s[p, c] = y * SCALE_A
        else:
            ref = ka_s if i == 1 else va_s
            ref[p, c, PAD:, :] = y
            if halo_set is not None:
                ref[halo_set, c, 0:PAD, :] = y[RB - PAD:]
        return y

    def xa_block(b):
        return xa_s[pl.ds(b * RB if isinstance(b, int) else pl.multiple_of(b * RB, RB), RB), :]

    def proj_pieces(b, p):
        o = oa_s[p].astype(bf16)
        rows = pl.ds(b * RB if isinstance(b, int) else pl.multiple_of(b * RB, RB), RB)
        ys = []
        for c in range(NT):
            y = _dot(o, _unpack(wop_s[:, c * 128:(c + 1) * 128]))
            outa_s[rows, c * 128:(c + 1) * 128] = y.astype(bf16)
            ys.append(y)
        return ys

    def attn(p, toks, start, span, first=False):
        rows = lax.broadcasted_iota(jnp.int32, (8, 128), 0)

        def logits(gi):
            r0 = gi * 8
            q = [qa_s[p, c, r0:r0 + 8, :] for c in range(NT)]
            ti = start + (gi * span) // NGR
            if 0 <= ti < len(toks):
                q = [pltpu.bitcast(pltpu.bitcast(a, u32) | toks[ti], f32) for a in q]
            lg = []
            for w in range(WIN):
                o = r0 + PAD - DIL * w
                t = q[0] * ka_s[p, 0, o:o + 8, :]
                for c in range(1, NT):
                    t = t + q[c] * ka_s[p, c, o:o + 8, :]
                lg.append(t)
            return [t + pltpu.roll(t, 64, 1) for t in lg]

        nxt = logits(0)
        for gi in range(NGR):
            r0 = gi * 8
            lg = nxt
            if gi + 1 < NGR:
                nxt = logits(gi + 1)
            lg = [t + pltpu.roll(t, 32, 1) for t in lg]
            if first:
                lg = [jnp.where(rows + r0 >= DIL * w, t, NEG) if r0 < DIL * w else t for w, t in enumerate(lg)]
            m = functools.reduce(jnp.maximum, lg)
            e = [jnp.exp2(t - m) for t in lg]
            rinv = _rcp(functools.reduce(lambda a, b: a + b, e))
            for c in range(NT):
                a = None
                for w in range(WIN):
                    o = r0 + PAD - DIL * w
                    u = e[w] * va_s[p, c, o:o + 8, :]
                    a = u if a is None else a + u
                oa_s[p, r0:r0 + 8, c * 128:(c + 1) * 128] = a * rinv

    def halo(p, pn):
        for ref in (ka_s, va_s):
            ref[pn, :, 0:PAD, :] = ref[p, :, RB:RB + PAD, :]

    SETS = (3, 1, 2, 0)

    def first(i, b):
        x = xa_block(b)
        return [qkv_piece(x, SETS[b], i, c, SETS[b + 1] if b < 3 else None) for c in range(NT)]

    def phase_a():
        lax.fori_loop(0, len(order), start_item, 0)
        zpad = jnp.zeros((NT, PAD, 128), f32)
        ka_s[SETS[0], :, 0:PAD, :] = zpad
        va_s[SETS[0], :, 0:PAD, :] = zpad
        zero_s[...] = jnp.zeros(zero_s.shape, u32)
        gacc_s[...] = jnp.zeros(gacc_s.shape, f32)

        wait(cp_wqkv[0])
        prep_wqkv(0)
        wait(cp_x01)
        first(0, 0); first(0, 1)
        wait(cp_x23, cp_wqkv[1])
        first(0, 2); first(0, 3); prep_wqkv(1)
        wait(cp_wqkv[2])
        first(1, 0); first(1, 1); prep_wqkv(2)
        first(2, 0); first(2, 1)
        wait(cp_woa)
        toks = [token(y) for b in (2, 3) for i in (1, 2) for y in first(i, b)]
        permute_rows(_pack(woa_s[...]), 3 * HD, wop_s, 0)
        attn(SETS[0], toks, -1, 11, first=True)
        toks += [token(y) for y in proj_pieces(0, SETS[0])]
        attn(SETS[1], toks, 10, 12)
        halo(SETS[3], 1)
        wait(cp_xa)

        def a_body(k, carry):
            for u in range(3):
                t = 4 + 3 * k + u
                p = (4 + u) % 3
                x = xa_block(t)
                ys = proj_pieces(t - 3, p) + [qkv_piece(x, p, i, c) for i in range(3) for c in range(NT)]
                attn((p + 1) % 3, [token(y) for y in ys], -2, 19)
                halo(p, (p + 1) % 3)
            return carry

        lax.fori_loop(0, (NB - 4) // 3, a_body, 0)

    def wpair(j):
        return _unpack(w_s[j])

    def deferred_rows(g, n):
        return jnp.concatenate(
            [xb_s[pl.ds(pl.multiple_of((4 * g + i) * SEG, SEG), 8), :] for i in range(4 * n)], axis=0)

    def pre_f(j):
        ys = []
        for i in range(3):
            y = _dot(_unpack(pl_s[...]), _unpack(w_s[j, :, i * PW:(i + 1) * PW]))
            for g in range(NPRE):
                dq_s[g, j, :, i * PW:(i + 1) * PW] = y[g * 32:(g + 1) * 32]
            ys.append(y)
        return ys

    def transposes(j):
        for i in range(3):
            w_s[j, :, i * PW:(i + 1) * PW] = _pack(wst_s[i, j * PW:(j + 1) * PW, :].T)

    def phase_p():
        wait(*cp_xb1, *cp_w1)
        pl_s[...] = _pack(deferred_rows(0, NPRE))
        transposes(0); transposes(1)
        toks = [token(y) for y in proj_pieces(NB - 3, (NB - 3) % 3) + pre_f(0)]
        attn((NB - 2) % 3, toks, -1, 6)
        transposes(2)
        toks += [token(y) for y in pre_f(1) + proj_pieces(NB - 2, (NB - 2) % 3)]
        attn((NB - 1) % 3, toks, 6, 5)
        for j in range(2, NP):
            if j == 4:
                wait(*cp_w2)
            if j + 1 < NP:
                transposes(j + 1)
            pre_f(j)
            if j == 2:
                proj_pieces(NB - 1, (NB - 1) % 3)
        wait(cp_wo)

    def prologue(_, carry):
        phase_a()
        phase_p()
        return carry

    one_s[0] = jnp.int32(1)
    lax.fori_loop(0, one_s[0], prologue, 0)
    cp_outa.start()

    ri = lax.broadcasted_iota(jnp.int32, (32, 2 * L), 0)
    ci = lax.broadcasted_iota(jnp.int32, (32, 2 * L), 1)
    is_even = ci < L
    cj = jnp.where(is_even, ci, ci - L)
    mask = (ri < MEM) | (ri >= cj) | (cj >= 32)
    rd = lax.broadcasted_iota(jnp.int32, (32, 64), 0)
    cd = lax.broadcasted_iota(jnp.int32, (32, 64), 1)
    same_seg = (rd >> 3) == ((cd & 31) >> 3)
    causal_d = (cd < 32) | ((cd & 31) <= rd)

    def blockdiag(a):
        ev = lax.broadcasted_iota(jnp.int32, a.shape, 1) < E
        return jnp.concatenate([jnp.where(ev, a, 0.0), jnp.where(ev, 0.0, a)], axis=0).astype(bf16)

    def wo_rows(j):
        r0 = j * E if isinstance(j, int) else pl.multiple_of(j * E, 8)
        return _unpack(wo_s[pl.ds(r0, E), :])

    def d_scores(slot, par, j):
        q = dq_s[slot, j, :, 0:PW].astype(bf16)
        k = jnp.concatenate([kvm_s[par, j, :, 0:PW], dq_s[slot, j, :, PW:2 * PW]], axis=0)
        lane = lax.broadcasted_iota(jnp.int32, (64, 256), 1)
        out = []
        for qh, kh in ((q[:, 0:256], jnp.where(lane < E, k[:, 0:256], 0.0)),
                       (q[:, 128:PW], jnp.where(lane >= 64, k[:, 128:PW], 0.0))):
            sc = _dot_nt(qh, kh.astype(bf16)) * SCALE_B
            out.append(jnp.where(same_seg, jnp.where(causal_d, sc, NEG), -jnp.inf))
        return out

    d_exp = lambda scs: [jnp.exp2(sc - jnp.max(sc, axis=1, keepdims=True)) for sc in scs]
    d_norm = lambda es: [e * _rcp(jnp.sum(e, axis=1, keepdims=True)) for e in es]
    d_join = lambda ps: jnp.concatenate(ps, axis=1).astype(bf16)

    def d_values(slot, par, j, p):
        v = jnp.concatenate([kvm_s[par, j, :, PW:2 * PW], dq_s[slot, j, :, 2 * PW:]], axis=0)
        return _dot(p, blockdiag(v)).astype(bf16)

    def write_deferred(g, val):
        r = val.astype(bf16)
        for i in range(4):
            outb_s[pl.ds(pl.multiple_of((g * 4 + i) * SEG, SEG), 8), :] = r[i * 8:(i + 1) * 8]

    def group(g, with_f, with_d, unroll):
        slot = lax.rem(g, NSLOT)
        pslot = lax.rem(g + NSLOT - 1, NSLOT)
        fslot = lax.rem(g + NPRE, NSLOT)
        par = lax.rem(g, 2)

        def step(i):
            r0 = pl.multiple_of((g * 4 + i) * SEG, SEG)
            drow = pl.ds(i * 8 if isinstance(i, int) else pl.multiple_of(i * 8, 8), 8)
            h = jnp.concatenate([mem_s[...], xb_s[pl.ds(r0 + 8, 24), :]], axis=0)
            fl = deferred_rows(g + NPRE, 1) if with_f else None
            qq, kk, vv, pp, oo, dp, do, acc = {}, {}, {}, {}, {}, {}, {}, [None]

            def proj(c, j):
                y = _dot(h, _unpack(w_s[j, :, c * PW:(c + 1) * PW]))
                if c == 0:
                    qq[j] = y.astype(bf16)
                else:
                    cur_s[j, :, (c - 1) * PW:c * PW] = y[:MEM]
                    y = jnp.concatenate([y, dq_s[slot, j, drow, c * PW:(c + 1) * PW]], axis=0)
                    (kk if c == 1 else vv)[j] = blockdiag(y)

            def softmax(j):
                sc = jnp.where(mask, _dot_nt(qq.pop(j), kk.pop(j)) * SCALE_B, NEG)
                m_e = jnp.max(jnp.where(is_even, sc, -jnp.inf), axis=1, keepdims=True)
                m_o = jnp.max(jnp.where(is_even, -jnp.inf, sc), axis=1, keepdims=True)
                e = jnp.exp2(sc - jnp.where(is_even, m_e, m_o))
                l_e = jnp.sum(jnp.where(is_even, e, 0.0), axis=1, keepdims=True)
                l_o = jnp.sum(jnp.where(is_even, 0.0, e), axis=1, keepdims=True)
                pp[j] = (e * jnp.where(is_even, _rcp(l_e), _rcp(l_o))).astype(bf16)

            def values(j):
                oo[j] = _dot(pp.pop(j), vv.pop(j)).astype(bf16)

            def oproj(j):
                if with_d:
                    wj = wo_rows(j)
                else:
                    wj = wost_s[j * PW:(j + 1) * PW, :]
                    wo_s[j * E:(j + 1) * E, :] = _pack(wj)
                r = _dot(oo.pop(j), wj)
                acc[0] = r if acc[0] is None else acc[0] + r

            def F(t):
                dq_s[fslot, i * 4 + t] = _dot(fl, wpair(i * 4 + t))

            def Ds(t):
                dp[t] = d_scores(pslot, 1 - par, i * 4 + t)

            def Dstage(fn):
                def run(_):
                    for t in range(4):
                        dp[t] = fn(dp[t])
                return run

            def Dv(t):
                do[t] = d_values(pslot, 1 - par, i * 4 + t, dp.pop(t))

            def G(t):
                gacc_s[...] += _dot(do.pop(t), wo_rows(i * 4 + t))

            main = {"k": (functools.partial(proj, 1), 0), "q": (functools.partial(proj, 0), 0),
                    "V": (values, 3), "S": (softmax, 1), "O": (oproj, 4), "v": (functools.partial(proj, 2), 0)}
            fill = {"a": Ds, "b": Dstage(d_exp), "c": Dstage(d_norm), "d": Dstage(d_join), "B": Dv, "F": F, "G": G}
            place = []
            if with_d:
                place += "a0@- a1@- a2@- a3@- b0@k1 c0@k2 d0@k3 B0@v3 B1@v3 B2@v4 B3@v4".split()
            if with_f:
                place += ("F0@O11" if with_d else "F0@v15", "F1@O12", "F2@O13", "F3@O14")
            if with_d:
                place += ("G0@O15 G1@O15 G2@O15 G3@O15" if with_f else "G0@O13 G1@O13 G2@O14 G3@O15").split()

            def fillers(tag):
                for f in [f for f in place if f.endswith("@" + tag)]:
                    place.remove(f)
                    fill[f[0]](int(f[1]))

            fillers("-")
            for t in range(NP + 4):
                for name, (fn, lag) in main.items():
                    if 0 <= t - lag < NP:
                        fn(t - lag)
                        fillers(f"{name}{t - lag}")
            assert not place
            kvm_s[par, :, drow, :] = cur_s[...]
            out = acc[0].astype(bf16)
            mem_s[...] = out[:MEM]
            outb_s[pl.ds(r0 + 8, 24), :] = out[MEM:]

        if unroll == 4:
            for i in range(4):
                step(i)
        else:
            def inner(ii, carry):
                for u in range(unroll):
                    step(ii * unroll + u)
                return carry
            lax.fori_loop(0, 4 // unroll, inner, 0)
        if with_d:
            write_deferred(g - 1, gacc_s[...])
            gacc_s[...] = jnp.zeros(gacc_s.shape, f32)

    def run_groups(lo, hi, *cfg):
        def body(g, carry):
            group(g, *cfg)
            return carry
        lax.fori_loop(lo, hi, body, 0)

    group(jnp.int32(0), True, False, 1)
    wait(cp_xb2)
    run_groups(1, NG - NPRE, True, True, 4)
    cp_outb1.start()
    run_groups(NG - NPRE, NG, False, True, 2)

    gl = NG - 1
    for c in cp_outb2:
        c.start()
    dp = [d_scores(gl % NSLOT, gl % 2, j) for j in range(NP)]
    for fn in (d_exp, d_norm, d_join):
        dp = [fn(x) for x in dp]
    do, acc = {}, None
    for b in range(6):
        for j in range(4 * b - 8, 4 * b - 4):
            if j >= 0:
                r = _dot(do.pop(j), wo_rows(j))
                acc = r if acc is None else acc + r
        for j in range(4 * b, min(4 * b + 4, NP)):
            do[j] = d_values(gl % NSLOT, gl % 2, j, dp[j])
    write_deferred(gl, acc)
    for c in cp_outb3:
        c.start()
    wait(cp_outa, cp_outb1, *cp_outb2, *cp_outb3)


@jax.jit
def _run(A_x, A_wqkv, A_wo, B_x, B_mem0, B_Wq, B_Wk, B_Wv, B_Wo):
    wt = lambda w: w.transpose(1, 2, 0).reshape(HB * E, D)
    V = pltpu.VMEM
    scratch = [
        V((S, D), bf16), V((D, 3 * D), bf16), V((D, D), bf16), V((S, D), bf16),
        V((3, HB * E, D), bf16), V((HB * E, D), bf16),
        V((NT, 4 * HD + 24, 128), u32), V((3 * HD, D), u32), V((HD, D), u32),
        V((4, NT, RB, 128), f32), V((4, NT, PAD + RB, 128), f32), V((4, NT, PAD + RB, 128), f32),
        V((4, RB, D), f32), V((S, D), bf16), V((8, 128), u32),
        V((NP, HD, 3 * PW), u32), V((HB * E // 2, D), u32), V((MEM, D), bf16),
        V((NPRE * 16, D), u32), V((NSLOT, NP, 32, 3 * PW), f32),
        V((NP, MEM, 2 * PW), f32), V((2, NP, 32, 2 * PW), f32),
        V((32, D), f32), V((S, D), bf16),
        pltpu.SMEM((1,), jnp.int32), pltpu.SemaphoreType.DMA((12,)), pltpu.SemaphoreType.DMA((4,)),
    ]
    out = pl.pallas_call(
        _kernel,
        out_shape=jax.ShapeDtypeStruct((S, 2 * D), bf16),
        in_specs=[pl.BlockSpec(memory_space=pl.ANY)] * 9,
        out_specs=pl.BlockSpec(memory_space=pl.ANY),
        scratch_shapes=scratch,
        compiler_params=pltpu.CompilerParams(vmem_limit_bytes=120 * 1024 * 1024),
    )(A_x.reshape(S, D), A_wqkv, A_wo, B_x.reshape(S, D), B_mem0.reshape(MEM, D),
      wt(B_Wq), wt(B_Wk), wt(B_Wv), B_Wo.reshape(HB * E, D))
    return out.reshape(1, S, 2 * D)


def pallas_concat_heads__sliding_local_dilated__memory_aug_recurrent_mem_tr__prompt_kernel(
    A_x, A_wqkv, A_wo, B_x, B_mem0, B_Wq, B_Wk, B_Wv, B_Wo, B_seg_len,
):
    if isinstance(B_seg_len, int):
        assert B_seg_len == SEG
    assert A_x.shape == (1, S, D) and B_x.shape == (1, S, D) and B_mem0.shape == (1, MEM, D)
    assert B_Wq.shape == (D, HB, E) and B_Wo.shape == (HB, E, D)
    return _run(A_x, A_wqkv, A_wo, B_x, B_mem0, B_Wq, B_Wk, B_Wv, B_Wo)
```

```python
import functools

import jax
import jax.numpy as jnp
from jax import lax
import jax.experimental.pallas as pl
import jax.experimental.pallas.tpu as pltpu

f32, bf16, u32 = jnp.float32, jnp.bfloat16, jnp.uint32

S, D = 2048, 640
NT = D // 128
HD = D // 2
LOG2E = 1.4426950408889634
NEG = -1000000000.0 * LOG2E
HA, DH, WIN, DIL = 32, 20, 8, 2
PAD = 16
RB = 128
NB = S // RB
NGR = RB // 8
SCALE_A = DH ** (-0.5) * LOG2E
HB, E, MEM, SEG = 32, 192, 8, 32
NP = HB // 2
PW = 2 * E
L = MEM + SEG
NG = S // (4 * SEG)
NPRE = 4
NSLOT = NPRE + 2
XB1 = (NPRE + 1) * 4 * SEG
SCALE_B = E ** (-0.5) * LOG2E


def _dot(a, b):
    return jnp.dot(a, b, preferred_element_type=f32)


def _dot_nt(a, b):
    return lax.dot_general(a, b, (((1,), (1,)), ((), ())), preferred_element_type=f32)


def _rcp(x):
    r = pl.reciprocal(x, approx=True)
    return r * (2.0 - x * r)


def _pack(x):
    return pltpu.bitcast(x, u32)


def _unpack(x):
    return pltpu.bitcast(x, bf16)


def _kernel(xa_h, wqkv_h, woa_h, xb_h, mem0_h, wq_h, wk_h, wv_h, wob_h, out_h,
            xa_s, wqkv_s, woa_s, xb_s, wst_s, wost_s,
            t1_s, wpt_s, wop_s, qa_s, ka_s, va_s, oa_s, outa_s, zero_s,
            w_s, wo_s, mem_s, pl_s, dq_s, cur_s, kvm_s, gacc_s, outb_s,
            sem_in, sem_out):
    def rows_copy(src, dst, r0, n, k):
        return pltpu.make_async_copy(src.at[pl.ds(r0, n)], dst.at[pl.ds(r0, n)], sem_in.at[k])

    def w_copies(j0, j1, k):
        return [rows_copy(w, wst_s.at[i], j0 * PW, (j1 - j0) * PW, k) for i, w in enumerate((wq_h, wk_h, wv_h))]

    cp_wqkv = [pltpu.make_async_copy(wqkv_h.at[:, pl.ds(i * D, D)], wqkv_s.at[:, pl.ds(i * D, D)], sem_in.at[i])
               for i in range(3)]
    cp_x01 = rows_copy(xa_h, xa_s, 0, 2 * RB, 3)
    cp_x23 = rows_copy(xa_h, xa_s, 2 * RB, 2 * RB, 4)
    cp_woa = pltpu.make_async_copy(woa_h, woa_s, sem_in.at[5])
    cp_xa = rows_copy(xa_h, xa_s, 4 * RB, S - 4 * RB, 6)
    cp_xb1 = [rows_copy(xb_h, xb_s, 0, XB1, 7), pltpu.make_async_copy(mem0_h, mem_s, sem_in.at[7])]
    cp_w1 = w_copies(0, 12, 8)
    cp_w2 = w_copies(12, NP, 9)
    cp_wo = pltpu.make_async_copy(wob_h, wost_s, sem_in.at[10])
    cp_xb2 = rows_copy(xb_h, xb_s, XB1, S - XB1, 11)

    def out_copy(src, r0, n, col, k):
        return pltpu.make_async_copy(src.at[pl.ds(r0, n)], out_h.at[pl.ds(r0, n), pl.ds(col, D)], sem_out.at[k])

    R1, R2 = (NG - NPRE - 1) * 4 * SEG, (NG - 1) * 4 * SEG
    cp_outa = out_copy(outa_s, 0, S, 0, 0)
    cp_outb1 = out_copy(outb_s, 0, R1, D, 1)
    cp_outb2 = [out_copy(outb_s, R1, R2 - R1, D, 2)] + [out_copy(outb_s, R2 + i * SEG + 8, 24, D, 2) for i in range(4)]
    cp_outb3 = [out_copy(outb_s, R2 + i * SEG, 8, D, 3) for i in range(4)]

    order = [[cp_wqkv[0]], [cp_x01], [cp_x23], [cp_wqkv[1]], [cp_wqkv[2]], [cp_woa], [cp_xa],
             cp_xb1, cp_w1, cp_w2, [cp_wo], [cp_xb2]]

    def start_item(i, carry):
        for k, cps in enumerate(order):
            @pl.when(i == k)
            def _(cps=cps):
                for c in cps:
                    c.start()
        return carry

    def wait(*cps):
        for c in cps:
            c.wait()

    def permute_rows(val, base, dst_ref, dst_base):
        lo16, hi16 = jnp.uint32(0xFFFF), jnp.uint32(0xFFFF0000)
        for c in range(NT):
            t1_s[c, base:base + HD, :] = val[:, c * 128:(c + 1) * 128]
        for dp in range(DH // 2):
            for hb in range(2):
                for c in range(NT):
                    a = t1_s[c, pl.ds(base + hb * 160 + dp, 8, stride=DH), :]
                    b = t1_s[c, pl.ds(base + hb * 160 + DH // 2 + dp, 8, stride=DH), :]
                    r = dst_base + 2 * dp * 16 + hb * 8
                    dst_ref[r:r + 8, c * 128:(c + 1) * 128] = (a & lo16) | (b << 16)
                    dst_ref[r + 16:r + 24, c * 128:(c + 1) * 128] = (a >> 16) | (b & hi16)

    def prep_wqkv(i):
        permute_rows(_pack(wqkv_s[:, i * D:(i + 1) * D].T), i * HD, wpt_s, i * HD)

    def token(y):
        return pltpu.bitcast(y[RB - 8:, 0:128], u32) & zero_s[...]

    def qkv_piece(x, p, i, c, halo_set=None):
        r0 = i * HD + c * 64
        y = _dot_nt(x, _unpack(wpt_s[r0:r0 + 64, :]))
        if i == 0:
            qa_s[p, c] = y * SCALE_A
        else:
            ref = ka_s if i == 1 else va_s
            ref[p, c, PAD:, :] = y
            if halo_set is not None:
                ref[halo_set, c, 0:PAD, :] = y[RB - PAD:]
        return y

    def xa_block(b):
        return xa_s[pl.ds(b * RB if isinstance(b, int) else pl.multiple_of(b * RB, RB), RB), :]

    def proj_pieces(b, p):
        o = oa_s[p].astype(bf16)
        rows = pl.ds(b * RB if isinstance(b, int) else pl.multiple_of(b * RB, RB), RB)
        ys = []
        for c in range(NT):
            y = _dot(o, _unpack(wop_s[:, c * 128:(c + 1) * 128]))
            outa_s[rows, c * 128:(c + 1) * 128] = y.astype(bf16)
            ys.append(y)
        return ys

    def attn(p, toks, start, span, first=False):
        rows = lax.broadcasted_iota(jnp.int32, (8, 128), 0)

        def logits(gi):
            r0 = gi * 8
            q = [qa_s[p, c, r0:r0 + 8, :] for c in range(NT)]
            ti = start + (gi * span) // NGR
            if 0 <= ti < len(toks):
                q = [pltpu.bitcast(pltpu.bitcast(a, u32) | toks[ti], f32) for a in q]
            lg = []
            for w in range(WIN):
                o = r0 + PAD - DIL * w
                t = q[0] * ka_s[p, 0, o:o + 8, :]
                for c in range(1, NT):
                    t = t + q[c] * ka_s[p, c, o:o + 8, :]
                lg.append(t)
            return [t + pltpu.roll(t, 64, 1) for t in lg]

        nxt = logits(0)
        for gi in range(NGR):
            r0 = gi * 8
            lg = nxt
            if gi + 1 < NGR:
                nxt = logits(gi + 1)
            lg = [t + pltpu.roll(t, 32, 1) for t in lg]
            if first:
                lg = [jnp.where(rows + r0 >= DIL * w, t, NEG) if r0 < DIL * w else t for w, t in enumerate(lg)]
            m = functools.reduce(jnp.maximum, lg)
            e = [jnp.exp2(t - m) for t in lg]
            rinv = _rcp(functools.reduce(lambda a, b: a + b, e))
            for c in range(NT):
                a = None
                for w in range(WIN):
                    o = r0 + PAD - DIL * w
                    u = e[w] * va_s[p, c, o:o + 8, :]
                    a = u if a is None else a + u
                oa_s[p, r0:r0 + 8, c * 128:(c + 1) * 128] = a * rinv

    def halo(p, pn):
        for ref in (ka_s, va_s):
            ref[pn, :, 0:PAD, :] = ref[p, :, RB:RB + PAD, :]

    SETS = (3, 1, 2, 0)

    def first(i, b):
        x = xa_block(b)
        return [qkv_piece(x, SETS[b], i, c, SETS[b + 1] if b < 3 else None) for c in range(NT)]

    def phase_a():
        lax.fori_loop(0, len(order), start_item, 0)
        zpad = jnp.zeros((NT, PAD, 128), f32)
        ka_s[SETS[0], :, 0:PAD, :] = zpad
        va_s[SETS[0], :, 0:PAD, :] = zpad
        zero_s[...] = jnp.zeros(zero_s.shape, u32)
        gacc_s[...] = jnp.zeros(gacc_s.shape, f32)

        wait(cp_wqkv[0])
        prep_wqkv(0)
        wait(cp_x01)
        first(0, 0); first(0, 1)
        wait(cp_x23, cp_wqkv[1])
        first(0, 2); first(0, 3); prep_wqkv(1)
        wait(cp_wqkv[2])
        first(1, 0); first(1, 1); prep_wqkv(2)
        first(2, 0); first(2, 1)
        wait(cp_woa)
        toks = [token(y) for b in (2, 3) for i in (1, 2) for y in first(i, b)]
        permute_rows(_pack(woa_s[...]), 3 * HD, wop_s, 0)
        attn(SETS[0], toks, -1, 11, first=True)
        toks += [token(y) for y in proj_pieces(0, SETS[0])]
        attn(SETS[1], toks, 10, 12)
        halo(SETS[3], 1)
        wait(cp_xa)

        def a_body(k, carry):
            for u in range(3):
                t = 4 + 3 * k + u
                p = (4 + u) % 3
                x = xa_block(t)
                ys = proj_pieces(t - 3, p) + [qkv_piece(x, p, i, c) for i in range(3) for c in range(NT)]
                attn((p + 1) % 3, [token(y) for y in ys], -2, 19)
                halo(p, (p + 1) % 3)
            return carry

        lax.fori_loop(0, (NB - 4) // 3, a_body, 0)

    def wpair(j):
        return _unpack(w_s[j])

    def deferred_rows(g, n):
        return jnp.concatenate(
            [xb_s[pl.ds(pl.multiple_of((4 * g + i) * SEG, SEG), 8), :] for i in range(4 * n)], axis=0)

    def pre_f(j):
        ys = []
        for i in range(3):
            y = _dot(_unpack(pl_s[...]), _unpack(w_s[j, :, i * PW:(i + 1) * PW]))
            for g in range(NPRE):
                dq_s[g, j, :, i * PW:(i + 1) * PW] = y[g * 32:(g + 1) * 32]
            ys.append(y)
        return ys

    def transposes(j):
        for i in range(3):
            w_s[j, :, i * PW:(i + 1) * PW] = _pack(wst_s[i, j * PW:(j + 1) * PW, :].T)

    def phase_p():
        wait(*cp_xb1, *cp_w1)
        pl_s[...] = _pack(deferred_rows(0, NPRE))
        transposes(0); transposes(1)
        toks = [token(y) for y in proj_pieces(NB - 3, (NB - 3) % 3) + pre_f(0)]
        attn((NB - 2) % 3, toks, -1, 6)
        transposes(2)
        toks += [token(y) for y in pre_f(1) + proj_pieces(NB - 2, (NB - 2) % 3)]
        attn((NB - 1) % 3, toks, 6, 5)
        for j in range(2, NP):
            if j == 4:
                wait(*cp_w2)
            if j + 1 < NP:
                transposes(j + 1)
            pre_f(j)
            if j == 2:
                proj_pieces(NB - 1, (NB - 1) % 3)
        wait(cp_wo)

    phase_a()
    phase_p()
    cp_outa.start()

    ri = lax.broadcasted_iota(jnp.int32, (32, 2 * L), 0)
    ci = lax.broadcasted_iota(jnp.int32, (32, 2 * L), 1)
    is_even = ci < L
    cj = jnp.where(is_even, ci, ci - L)
    mask = (ri < MEM) | (ri >= cj) | (cj >= 32)
    rd = lax.broadcasted_iota(jnp.int32, (32, 64), 0)
    cd = lax.broadcasted_iota(jnp.int32, (32, 64), 1)
    same_seg = (rd >> 3) == ((cd & 31) >> 3)
    causal_d = (cd < 32) | ((cd & 31) <= rd)

    def blockdiag(a):
        ev = lax.broadcasted_iota(jnp.int32, a.shape, 1) < E
        return jnp.concatenate([jnp.where(ev, a, 0.0), jnp.where(ev, 0.0, a)], axis=0).astype(bf16)

    def wo_rows(j):
        r0 = j * E if isinstance(j, int) else pl.multiple_of(j * E, 8)
        return _unpack(wo_s[pl.ds(r0, E), :])

    def d_scores(slot, par, j):
        q = dq_s[slot, j, :, 0:PW].astype(bf16)
        k = jnp.concatenate([kvm_s[par, j, :, 0:PW], dq_s[slot, j, :, PW:2 * PW]], axis=0)
        lane = lax.broadcasted_iota(jnp.int32, (64, 256), 1)
        out = []
        for qh, kh in ((q[:, 0:256], jnp.where(lane < E, k[:, 0:256], 0.0)),
                       (q[:, 128:PW], jnp.where(lane >= 64, k[:, 128:PW], 0.0))):
            sc = _dot_nt(qh, kh.astype(bf16)) * SCALE_B
            out.append(jnp.where(same_seg, jnp.where(causal_d, sc, NEG), -jnp.inf))
        return out

    d_exp = lambda scs: [jnp.exp2(sc - jnp.max(sc, axis=1, keepdims=True)) for sc in scs]
    d_norm = lambda es: [e * _rcp(jnp.sum(e, axis=1, keepdims=True)) for e in es]
    d_join = lambda ps: jnp.concatenate(ps, axis=1).astype(bf16)

    def d_values(slot, par, j, p):
        v = jnp.concatenate([kvm_s[par, j, :, PW:2 * PW], dq_s[slot, j, :, 2 * PW:]], axis=0)
        return _dot(p, blockdiag(v)).astype(bf16)

    def write_deferred(g, val):
        r = val.astype(bf16)
        for i in range(4):
            outb_s[pl.ds(pl.multiple_of((g * 4 + i) * SEG, SEG), 8), :] = r[i * 8:(i + 1) * 8]

    def group(g, with_f, with_d, unroll):
        slot = lax.rem(g, NSLOT)
        pslot = lax.rem(g + NSLOT - 1, NSLOT)
        fslot = lax.rem(g + NPRE, NSLOT)
        par = lax.rem(g, 2)

        def step(i):
            r0 = pl.multiple_of((g * 4 + i) * SEG, SEG)
            drow = pl.ds(i * 8 if isinstance(i, int) else pl.multiple_of(i * 8, 8), 8)
            h = jnp.concatenate([mem_s[...], xb_s[pl.ds(r0 + 8, 24), :]], axis=0)
            fl = deferred_rows(g + NPRE, 1) if with_f else None
            qq, kk, vv, pp, oo, dp, do, acc = {}, {}, {}, {}, {}, {}, {}, [None]

            def proj(c, j):
                y = _dot(h, _unpack(w_s[j, :, c * PW:(c + 1) * PW]))
                if c == 0:
                    qq[j] = y.astype(bf16)
                else:
                    cur_s[j, :, (c - 1) * PW:c * PW] = y[:MEM]
                    y = jnp.concatenate([y, dq_s[slot, j, drow, c * PW:(c + 1) * PW]], axis=0)
                    (kk if c == 1 else vv)[j] = blockdiag(y)

            def softmax(j):
                sc = jnp.where(mask, _dot_nt(qq.pop(j), kk.pop(j)) * SCALE_B, NEG)
                m_e = jnp.max(jnp.where(is_even, sc, -jnp.inf), axis=1, keepdims=True)
                m_o = jnp.max(jnp.where(is_even, -jnp.inf, sc), axis=1, keepdims=True)
                e = jnp.exp2(sc - jnp.where(is_even, m_e, m_o))
                l_e = jnp.sum(jnp.where(is_even, e, 0.0), axis=1, keepdims=True)
                l_o = jnp.sum(jnp.where(is_even, 0.0, e), axis=1, keepdims=True)
                pp[j] = (e * jnp.where(is_even, _rcp(l_e), _rcp(l_o))).astype(bf16)

            def values(j):
                oo[j] = _dot(pp.pop(j), vv.pop(j)).astype(bf16)

            def oproj(j):
                if with_d:
                    wj = wo_rows(j)
                else:
                    wj = wost_s[j * PW:(j + 1) * PW, :]
                    wo_s[j * E:(j + 1) * E, :] = _pack(wj)
                r = _dot(oo.pop(j), wj)
                acc[0] = r if acc[0] is None else acc[0] + r

            def F(t):
                dq_s[fslot, i * 4 + t] = _dot(fl, wpair(i * 4 + t))

            def Ds(t):
                dp[t] = d_scores(pslot, 1 - par, i * 4 + t)

            def Dstage(fn):
                def run(_):
                    for t in range(4):
                        dp[t] = fn(dp[t])
                return run

            def Dv(t):
                do[t] = d_values(pslot, 1 - par, i * 4 + t, dp.pop(t))

            def G(t):
                gacc_s[...] += _dot(do.pop(t), wo_rows(i * 4 + t))

            main = {"k": (functools.partial(proj, 1), 0), "q": (functools.partial(proj, 0), 0),
                    "V": (values, 3), "S": (softmax, 1), "O": (oproj, 4), "v": (functools.partial(proj, 2), 0)}
            fill = {"a": Ds, "b": Dstage(d_exp), "c": Dstage(d_norm), "d": Dstage(d_join), "B": Dv, "F": F, "G": G}
            place = []
            if with_d:
                place += "a0@- a1@- a2@- a3@- b0@k1 c0@k2 d0@k3 B0@v3 B1@v3 B2@v4 B3@v4".split()
            if with_f:
                place += ("F0@O11" if with_d else "F0@v15", "F1@O12", "F2@O13", "F3@O14")
            if with_d:
                place += ("G0@O15 G1@O15 G2@O15 G3@O15" if with_f else "G0@O13 G1@O13 G2@O14 G3@O15").split()

            def fillers(tag):
                for f in [f for f in place if f.endswith("@" + tag)]:
                    place.remove(f)
                    fill[f[0]](int(f[1]))

            fillers("-")
            for t in range(NP + 4):
                for name, (fn, lag) in main.items():
                    if 0 <= t - lag < NP:
                        fn(t - lag)
                        fillers(f"{name}{t - lag}")
            assert not place
            kvm_s[par, :, drow, :] = cur_s[...]
            out = acc[0].astype(bf16)
            mem_s[...] = out[:MEM]
            outb_s[pl.ds(r0 + 8, 24), :] = out[MEM:]

        if unroll == 4:
            for i in range(4):
                step(i)
        else:
            def inner(ii, carry):
                for u in range(unroll):
                    step(ii * unroll + u)
                return carry
            lax.fori_loop(0, 4 // unroll, inner, 0)
        if with_d:
            write_deferred(g - 1, gacc_s[...])
            gacc_s[...] = jnp.zeros(gacc_s.shape, f32)

    def run_groups(lo, hi, *cfg):
        def body(g, carry):
            group(g, *cfg)
            return carry
        lax.fori_loop(lo, hi, body, 0)

    group(jnp.int32(0), True, False, 1)
    wait(cp_xb2)
    run_groups(1, NG - NPRE, True, True, 4)
    cp_outb1.start()
    run_groups(NG - NPRE, NG, False, True, 2)

    gl = NG - 1
    for c in cp_outb2:
        c.start()
    dp = [d_scores(gl % NSLOT, gl % 2, j) for j in range(NP)]
    for fn in (d_exp, d_norm, d_join):
        dp = [fn(x) for x in dp]
    do, acc = {}, None
    for b in range(6):
        for j in range(4 * b - 8, 4 * b - 4):
            if j >= 0:
                r = _dot(do.pop(j), wo_rows(j))
                acc = r if acc is None else acc + r
        for j in range(4 * b, min(4 * b + 4, NP)):
            do[j] = d_values(gl % NSLOT, gl % 2, j, dp[j])
    write_deferred(gl, acc)
    for c in cp_outb3:
        c.start()
    wait(cp_outa, cp_outb1, *cp_outb2, *cp_outb3)


@jax.jit
def _run(A_x, A_wqkv, A_wo, B_x, B_mem0, B_Wq, B_Wk, B_Wv, B_Wo):
    wt = lambda w: w.transpose(1, 2, 0).reshape(HB * E, D)
    V = pltpu.VMEM
    scratch = [
        V((S, D), bf16), V((D, 3 * D), bf16), V((D, D), bf16), V((S, D), bf16),
        V((3, HB * E, D), bf16), V((HB * E, D), bf16),
        V((NT, 4 * HD + 24, 128), u32), V((3 * HD, D), u32), V((HD, D), u32),
        V((4, NT, RB, 128), f32), V((4, NT, PAD + RB, 128), f32), V((4, NT, PAD + RB, 128), f32),
        V((4, RB, D), f32), V((S, D), bf16), V((8, 128), u32),
        V((NP, HD, 3 * PW), u32), V((HB * E // 2, D), u32), V((MEM, D), bf16),
        V((NPRE * 16, D), u32), V((NSLOT, NP, 32, 3 * PW), f32),
        V((NP, MEM, 2 * PW), f32), V((2, NP, 32, 2 * PW), f32),
        V((32, D), f32), V((S, D), bf16),
        pltpu.SemaphoreType.DMA((12,)), pltpu.SemaphoreType.DMA((4,)),
    ]
    out = pl.pallas_call(
        _kernel,
        out_shape=jax.ShapeDtypeStruct((S, 2 * D), bf16),
        in_specs=[pl.BlockSpec(memory_space=pl.ANY)] * 9,
        out_specs=pl.BlockSpec(memory_space=pl.ANY),
        scratch_shapes=scratch,
        compiler_params=pltpu.CompilerParams(vmem_limit_bytes=120 * 1024 * 1024),
    )(A_x.reshape(S, D), A_wqkv, A_wo, B_x.reshape(S, D), B_mem0.reshape(MEM, D),
      wt(B_Wq), wt(B_Wk), wt(B_Wv), B_Wo.reshape(HB * E, D))
    return out.reshape(1, S, 2 * D)


def pallas_concat_heads__sliding_local_dilated__memory_aug_recurrent_mem_tr__prompt_kernel(
    A_x, A_wqkv, A_wo, B_x, B_mem0, B_Wq, B_Wk, B_Wv, B_Wo, B_seg_len,
):
    if isinstance(B_seg_len, int):
        assert B_seg_len == SEG
    assert A_x.shape == (1, S, D) and B_x.shape == (1, S, D) and B_mem0.shape == (1, MEM, D)
    assert B_Wq.shape == (D, HB, E) and B_Wo.shape == (HB, E, D)
    return _run(A_x, A_wqkv, A_wo, B_x, B_mem0, B_Wq, B_Wk, B_Wv, B_Wo)
```
